```python
import jax
import jax.numpy as jnp

def _softmax(x, axis=-1):
    return jax.nn.softmax(x, axis=axis)
def _gelu(x):
    return jax.nn.gelu(x, approximate=True)
def _silu(x):
    return jax.nn.silu(x)
def _sigmoid(x):
    return jax.nn.sigmoid(x)
def _layernorm(x, axis=-1, eps=1e-5):
    m = jnp.mean(x, axis=axis, keepdims=True)
    v = jnp.var(x, axis=axis, keepdims=True)
    return (x - m) / jnp.sqrt(v + eps)
def _scatter_add(tgt, idx, src, axis=0):
    return tgt.at[idx].add(src)
def _segment_sum(src, seg, n):
    return jax.ops.segment_sum(src, seg, n)
class _Rng:
    def __init__(self, key):
        self._k = key
    def _next(self):
        self._k, sub = jax.random.split(self._k)
        return sub
    def normal(self, shape):
        return jax.random.normal(self._next(), shape, dtype=jnp.bfloat16)
    def randint(self, lo, hi, shape):
        return jax.random.randint(self._next(), shape, lo, hi, dtype=jnp.int32)
    def uniform(self, shape, lo=0.0, hi=1.0):
        return jax.random.uniform(self._next(), shape, jnp.bfloat16, lo, hi)
    def permutation(self, n):
        return jax.random.permutation(self._next(), n)


kernel_name = 'interleave_layers__compressed_kv_cla__moe_arch_mod__decode'

def setup_inputs():
    _rng = _Rng(jax.random.key(int.from_bytes(__import__("os").urandom(4), "little")))
    _w = (lambda a: (lambda t: t.astype(jnp.bfloat16) if jnp.issubdtype(t.dtype, jnp.floating) else t)(jnp.asarray(a)))
    def _A_setup():
        B, H, Sq, Sk, D, M = 1, 32, 1, 4096, 128, 640
        Dc = 4 * D
        return {
            "x": _w((lambda *s: _rng.normal(s) * 0.05)(B, Sq, M)),
            "c_kv": _w((lambda *s: _rng.normal(s) * 0.05)(B, Sk, Dc)),
            "w_q": _w((lambda *s: _rng.normal(s) * 0.05)(M, H, D) * (M ** -0.5)),
            "w_uk": _w((lambda *s: _rng.normal(s) * 0.05)(Dc, H, D) * (Dc ** -0.5)),
            "w_uv": _w((lambda *s: _rng.normal(s) * 0.05)(Dc, H, D) * (Dc ** -0.5)),
            "w_o": _w((lambda *s: _rng.normal(s) * 0.05)(H, D, M) * ((H * D) ** -0.5)),
        }
    _A_in = _A_setup()

    def _B_setup():
        B, S, D, F, C = 1, 1, 640, 1728, 1
        return {
            "x": _w((lambda *s: _rng.normal(s) * 0.05)(B, S, D)),
            "w_r": _w((lambda *s: _rng.normal(s) * 0.05)(D)),
            "w_gate": _w((lambda *s: _rng.normal(s) * 0.05)(D, F)),
            "w_up": _w((lambda *s: _rng.normal(s) * 0.05)(D, F)),
            "w_down": _w((lambda *s: _rng.normal(s) * 0.05)(F, D)),
        }
    _B_in = _B_setup()

    return {
        "A_x": _A_in["x"],
        "A_c_kv": _A_in["c_kv"],
        "A_w_q": _A_in["w_q"],
        "A_w_uk": _A_in["w_uk"],
        "A_w_uv": _A_in["w_uv"],
        "A_w_o": _A_in["w_o"],
        "B_x": _B_in["x"],
        "B_w_r": _B_in["w_r"],
        "B_w_gate": _B_in["w_gate"],
        "B_w_up": _B_in["w_up"],
        "B_w_down": _B_in["w_down"],
    }

def reference(A_x, A_c_kv, A_w_q, A_w_uk, A_w_uv, A_w_o, B_x, B_w_r, B_w_gate, B_w_up, B_w_down):
    def _A_ref(x, c_kv, w_q, w_uk, w_uv, w_o):
        B, Sq, M = x.shape[0], x.shape[1], x.shape[2]
        Sk = c_kv.shape[1]
        H, D = w_q.shape[1], w_q.shape[2]
        q = jnp.einsum("bqm,mhd->bhqd", x, w_q)
        k = jnp.einsum("bkc,chd->bhkd", c_kv, w_uk)
        v = jnp.einsum("bkc,chd->bhkd", c_kv, w_uv)
        scores = jnp.einsum("bhqd,bhkd->bhqk", q, k) * (D ** -0.5)
        off = Sk - Sq
        qi = jnp.arange(Sq)[:, None]
        kj = jnp.arange(Sk)[None, :]
        cmask = kj <= (qi + off)
        scores = jnp.where(cmask[None, None], scores, -1e9)
        p = _softmax(scores, axis=-1)
        ctx = jnp.einsum("bhqk,bhkd->bhqd", p, v)
        return jnp.einsum("bhqd,hdm->bqm", ctx, w_o)

    def _B_ref(x, w_r, w_gate, w_up, w_down):
        B, S, D = x.shape
        C = 1
        r = x @ w_r
        idx = jnp.argsort(-r, axis=-1)[:, :C]
        idx_e = jnp.repeat(idx.reshape(B, C, 1), D, axis=2)
        x_sel = jnp.take_along_axis(x, idx_e, axis=1)
        g = _silu(x_sel @ w_gate)
        u = x_sel @ w_up
        y = (g * u) @ w_down
        r_sel = _sigmoid(jnp.take_along_axis(r, idx, axis=1))
        y = y * r_sel.reshape(B, C, 1)
        b_off = (jnp.arange(B) * S).reshape(B, 1)
        flat_idx = (idx + b_off).reshape(B * C)
        zero = (x * 0.0).reshape(B * S, D)
        upd = _scatter_add(zero, flat_idx, y.reshape(B * C, D), axis=0)
        return x + upd.reshape(B, S, D)

    x = A_x
    x = x + _A_ref(_layernorm(x, axis=-1), A_c_kv, A_w_q, A_w_uk, A_w_uv, A_w_o)
    x = x + _B_ref(_layernorm(x, axis=-1), B_w_r, B_w_gate, B_w_up, B_w_down)
    x = x + _A_ref(_layernorm(x, axis=-1), A_c_kv, A_w_q, A_w_uk, A_w_uv, A_w_o)
    x = x + _B_ref(_layernorm(x, axis=-1), B_w_r, B_w_gate, B_w_up, B_w_down)
    return x
```

```python
import functools
import jax
import jax.numpy as jnp
from jax import lax
from jax.experimental import pallas as pl
from jax.experimental.pallas import tpu as pltpu

M, H, D, C, S, F = 640, 32, 128, 512, 4096, 1728
f32, bf16, u32, i32 = jnp.float32, jnp.bfloat16, jnp.uint32, jnp.int32
EPS = 1e-5


def _iota(shape, dim):
    return lax.broadcasted_iota(i32, shape, dim)


def _dot(a, b):
    return jnp.dot(a, b, preferred_element_type=f32)


def _dot_t(a, b):
    return lax.dot_general(a, b, (((1,), (1,)), ((), ())), preferred_element_type=f32)


def _layernorm(x):
    m = jnp.mean(x, axis=-1, keepdims=True)
    xc = x - m
    v = jnp.mean(xc * xc, axis=-1, keepdims=True)
    return xc * lax.rsqrt(v + EPS)


def _c1(p):
    j = (p + 1) % 16
    ci = ((p - 15 - j) % 128) // 16
    return 8 * j + ci


def _c2(p):
    j = (-p) % 16
    ci = ((p + j) % 128) // 16
    return 8 * j + ci


def make_kernel(T=8):
  def kernel(x_ref, wr_ref, wq_hbm, wuk_hbm, ckv_hbm, wuv_hbm, wg_hbm, wu_hbm, wo_hbm, wd_hbm,
           out_ref,
           wq, wuk, ckv, wuv, wg, wu, wo, wd, wukT, ckvT, wgT, wuT, rp_ref, s_ref, sems):
    srcs = [wq_hbm, wuk_hbm, ckv_hbm, wuv_hbm, wg_hbm, wu_hbm, wo_hbm, wd_hbm]
    dsts = [wq, wuk, ckv, wuv, wg, wu, wo, wd]
    copies = [pltpu.make_async_copy(s, d, sems.at[i]) for i, (s, d) in enumerate(zip(srcs, dsts))]
    for cp in copies:
        cp.start()

    sub = _iota((8, 128), 0)
    lane = _iota((8, 128), 1)
    l16 = lane % 16
    lo, hi = jnp.uint32(0xFFFF), jnp.uint32(0xFFFF0000)
    zero = jnp.uint32(0)
    mask_rev = jnp.where(l16 == 15 - 2 * sub, lo, zero) | jnp.where(l16 == 14 - 2 * sub, hi, zero)
    r16 = _iota((16, 128), 0)
    ln16 = _iota((16, 128), 1)
    diag_nat = (ln16 % 16) == r16
    rr = _iota((128, 128), 0)
    cc = _iota((128, 128), 1)
    eye = (rr == cc).astype(bf16)
    pm1 = (cc == _c1(rr)).astype(bf16)
    p2 = (rr == _c2(cc)).astype(bf16)
    expand = ((rr % 8) == (cc // 16)).astype(bf16)
    amask = (ln16 // 8) == r16
    rev_idx = 7 - sub

    wr = wr_ref[...].reshape(1, M).astype(f32)
    x = x_ref[0].astype(f32)

    def attention(x, first):
        xn = _layernorm(x)
        a = jnp.concatenate(
            [jnp.where(amask, jnp.broadcast_to(xn[:, g * 128:(g + 1) * 128], (16, 128)), 0.0)
             for g in range(5)], axis=0).astype(bf16)
        r = lax.bitcast_convert_type(_dot(a, expand), u32)
        rp_ref[...] = r | (r >> 16)
        if first:
            copies[0].wait()
        acc = [jnp.zeros((16, 128), f32), jnp.zeros((16, 128), f32)]
        for c0 in range(0, 80, T):
            L = jnp.concatenate(
                [pltpu.bitcast(jnp.broadcast_to(rp_ref[t:t + 1, :], (8, 128)) & mask_rev, bf16)
                 for t in range(c0, c0 + T)], axis=1)
            for hf in range(2):
                W = wq[8 * c0:8 * (c0 + T), 16 * hf:16 * hf + 16, :].reshape(128 * T, 128)
                acc[hf] = acc[hf] + _dot(L, W)
        q_rev = [a_.astype(bf16) for a_ in acc]

        if first:
            copies[1].wait()
            for hf in range(2):
                for a0 in range(0, 64, T):
                    W = wuk[8 * a0:8 * (a0 + T), 16 * hf:16 * hf + 16, :].reshape(128 * T, 128)
                    wukT[hf, :, 128 * a0:128 * (a0 + T)] = _dot_t(eye, W).astype(bf16)
        qa = []
        for hf in range(2):
            blocks = []
            for b in range(4):
                accb = jnp.zeros((16, 128), f32)
                for j0 in range(0, 16, T):
                    a0 = 16 * b + j0
                    o = _dot(q_rev[hf], wukT[hf, :, 128 * a0:128 * (a0 + T)])
                    for jj in range(T):
                        j = j0 + jj
                        v = pltpu.roll(o[:, 128 * jj:128 * (jj + 1)], j, 1, stride=1, stride_axis=0)
                        accb = jnp.where((ln16 % 16) == (15 + j) % 16, v, accb)
                accb = accb * (D ** -0.5)
                nat = jnp.concatenate([jnp.take_along_axis(accb[8:16], rev_idx, axis=0),
                                       jnp.take_along_axis(accb[0:8], rev_idx, axis=0)], axis=0)
                blocks.append(nat)
            qa.append(jnp.concatenate(blocks, axis=1))
        qa = jnp.concatenate(qa, axis=0).astype(bf16)

        if first:
            copies[2].wait()
            for b in range(4):
                for k0 in range(0, S, 1024):
                    ckvT[128 * b:128 * (b + 1), k0:k0 + 1024] = _dot_t(
                        pm1, ckv[k0:k0 + 1024, 128 * b:128 * (b + 1)]).astype(bf16)
        KC = 1024
        mx = None
        for k0 in range(0, S, KC):
            sc = _dot(qa, ckvT[:, k0:k0 + KC])
            s_ref[:, k0:k0 + KC] = sc
            for j in range(KC // 128):
                blk = sc[:, 128 * j:128 * (j + 1)]
                mx = blk if mx is None else jnp.maximum(mx, blk)
        mx = jnp.max(mx, axis=1, keepdims=True)
        den = jnp.zeros((32, 128), f32)
        cx = jnp.zeros((32, C), f32)
        for k0 in range(0, S, KC):
            p = jnp.exp(s_ref[:, k0:k0 + KC] - mx)
            for j in range(KC // 128):
                den = den + p[:, 128 * j:128 * (j + 1)]
            cx = cx + _dot(p.astype(bf16), ckv[k0:k0 + KC, :])
        den = jnp.sum(den, axis=1, keepdims=True)
        cx = (cx / den).astype(bf16)
        xs = jnp.concatenate([cx[16 * hf:16 * hf + 16, 128 * b:128 * (b + 1)]
                              for hf in range(2) for b in range(4)], axis=0)
        sform = _dot(xs, p2)

        if first:
            copies[3].wait()
        ctx = []
        for hf in range(2):
            acc = jnp.zeros((16, 128), f32)
            for b in range(4):
                sb = sform[(hf * 4 + b) * 16:(hf * 4 + b + 1) * 16]
                for j0 in range(0, 16, T):
                    L = jnp.concatenate(
                        [jnp.where(diag_nat, pltpu.roll(sb, j, 1, stride=1, stride_axis=0), 0.0).astype(bf16)
                         for j in range(j0, j0 + T)], axis=1)
                    a0 = 16 * b + j0
                    W = wuv[8 * a0:8 * (a0 + T), 16 * hf:16 * hf + 16, :].reshape(128 * T, 128)
                    acc = acc + _dot(L, W)
            ctx.append(acc)

        if first:
            copies[4].wait()
            copies[5].wait()
            for src, dst in ((wg, wgT), (wu, wuT)):
                for g in range(5):
                    for f0, n in ((0, 896), (896, 832)):
                        dst[128 * g:128 * (g + 1), f0:f0 + n] = _dot_t(
                            eye, src[f0:f0 + n, 128 * g:128 * (g + 1)]).astype(bf16)
            copies[6].wait()
        acc = jnp.zeros((16, M), f32)
        HC = 4
        for h0 in range(0, H, HC):
            X = jnp.concatenate(
                [jnp.where(r16 == (h % 16), ctx[h // 16], 0.0).astype(bf16) for h in range(h0, h0 + HC)], axis=1)
            acc = acc + _dot(X, wo[128 * h0:128 * (h0 + HC), :])
        return jnp.sum(acc, axis=0, keepdims=True)

    def ffn(x, first):
        xn = _layernorm(x)
        r = jnp.sum(xn * wr, axis=1, keepdims=True)
        X = jnp.broadcast_to(xn, (16, M)).astype(bf16)
        g = _dot(X, wgT[...])
        u = _dot(X, wuT[...])
        h = (g * jax.nn.sigmoid(g) * u).astype(bf16)
        if first:
            copies[7].wait()
        y = _dot(h, wd[...])[0:1]
        return xn + y * jax.nn.sigmoid(r)

    x = x + attention(x, True)
    x = x + ffn(x, True)
    x = x + attention(x, False)
    x = x + ffn(x, False)
    out_ref[0] = x.astype(bf16)
  return kernel


@jax.jit
def pallas_interleave_layers__compressed_kv_cla__moe_arch_mod__decode_kernel(
        A_x, A_c_kv, A_w_q, A_w_uk, A_w_uv, A_w_o, B_x, B_w_r, B_w_gate, B_w_up, B_w_down):
    interpret, T = False, 8
    del B_x
    vm = pl.BlockSpec(memory_space=pltpu.VMEM)
    hbm = pl.BlockSpec(memory_space=pl.ANY)
    scratch = [
        pltpu.VMEM((M, H, D), bf16), pltpu.VMEM((C, H, D), bf16), pltpu.VMEM((S, C), bf16),
        pltpu.VMEM((C, H, D), bf16), pltpu.VMEM((F, M), bf16), pltpu.VMEM((F, M), bf16),
        pltpu.VMEM((H * D, M), bf16), pltpu.VMEM((F, M), bf16),
        pltpu.VMEM((2, D, 64 * 128), bf16), pltpu.VMEM((C, S), bf16),
        pltpu.VMEM((M, F), bf16), pltpu.VMEM((M, F), bf16),
        pltpu.VMEM((80, 128), u32), pltpu.VMEM((H, S), f32),
        pltpu.SemaphoreType.DMA((8,)),
    ]
    return pl.pallas_call(
        make_kernel(T),
        out_shape=jax.ShapeDtypeStruct((1, 1, M), bf16),
        in_specs=[vm, vm] + [hbm] * 8,
        out_specs=vm,
        scratch_shapes=scratch,
        compiler_params=pltpu.CompilerParams(vmem_limit_bytes=110 * 1024 * 1024),
        interpret=interpret,
        name="fused_decode",
    )(A_x, B_w_r, A_w_q, A_w_uk, A_c_kv.reshape(S, C), A_w_uv, B_w_gate.T, B_w_up.T,
      A_w_o.reshape(H * D, M), B_w_down)
```

```python
import functools
import jax
import jax.numpy as jnp
from jax import lax
from jax.experimental import pallas as pl
from jax.experimental.pallas import tpu as pltpu

M, H, D, C, S, F = 640, 32, 128, 512, 4096, 1728
f32, bf16, u32, i32 = jnp.float32, jnp.bfloat16, jnp.uint32, jnp.int32
EPS = 1e-5
WD_CHUNKS = ((0, 896), (896, 512), (1408, 320))
NC = 4
KC = S // NC


def _iota(shape, dim):
    return lax.broadcasted_iota(i32, shape, dim)


def _dot(a, b):
    return jnp.dot(a, b, preferred_element_type=f32)


def _dot_t(a, b):
    return lax.dot_general(a, b, (((1,), (1,)), ((), ())), preferred_element_type=f32)


def _c1(p):
    j = (p + 1) % 16
    ci = ((p - 15 - j) % 128) // 16
    return 8 * j + ci


def _c2(p):
    j = (-p) % 16
    ci = ((p + j) % 128) // 16
    return 8 * j + ci


def _dup(x):
    w = lax.bitcast_convert_type(x.astype(bf16).astype(f32), u32)
    return w | (w >> 16)


def _stats(x):
    m = jnp.mean(x, axis=-1, keepdims=True)
    xc = x - m
    v = jnp.mean(xc * xc, axis=-1, keepdims=True)
    return m, lax.rsqrt(v + EPS)


def make_kernel(T=8):
  def kernel(x_hbm, wr_hbm, wq_hbm, wuk_hbm, ckv_hbm, wuv_hbm, wg_hbm, wu_hbm, wo_hbm, wd_hbm,
             out_ref,
             xs, wrs, wq, wuk, ckv, wuv, wg, wu, wo, wd, wukT, ckvT, ckv2, wgT, wuT, qsum, sems):
    srcs = [x_hbm, wr_hbm, wq_hbm, wuk_hbm, ckv_hbm, wuv_hbm, wg_hbm, wu_hbm, wo_hbm]
    dsts = [xs, wrs, wq, wuk, ckv, wuv, wg, wu, wo]
    copies = [pltpu.make_async_copy(s, d, sems.at[i]) for i, (s, d) in enumerate(zip(srcs, dsts))]
    wd_copies = [pltpu.make_async_copy(wd_hbm.at[pl.ds(r0, n)], wd.at[pl.ds(r0, n)], sems.at[len(copies) + i])
                 for i, (r0, n) in enumerate(WD_CHUNKS)]
    for cp in copies + wd_copies:
        cp.start()
    cp_x, cp_wr, cp_wq, cp_wuk, cp_ckv, cp_wuv, cp_wg, cp_wu, cp_wo = copies

    sub = _iota((8, 128), 0)
    lane = _iota((8, 128), 1)
    l16 = lane % 16
    lo, hi, zero = jnp.uint32(0xFFFF), jnp.uint32(0xFFFF0000), jnp.uint32(0)
    ones_w = jnp.uint32(0x3F803F80)
    mask_rev = jnp.where(l16 == 15 - 2 * sub, lo, zero) | jnp.where(l16 == 14 - 2 * sub, hi, zero)
    r16 = _iota((16, 128), 0)
    ln16 = _iota((16, 128), 1)
    diag_nat = (ln16 % 16) == r16
    rev_idx = 7 - sub
    exp_idx = lane // 16

    cp_x.wait()
    cp_wr.wait()
    wr = jnp.broadcast_to(wrs[...].reshape(1, M).astype(f32), (8, M))
    x = jnp.broadcast_to(xs[0].astype(f32), (8, M))

    def consts128():
        rr = _iota((128, 128), 0)
        cc = _iota((128, 128), 1)
        return rr, cc

    def attention(x, first):
        xw = _dup(x)
        mean, rs = _stats(x)
        if first:
            cp_wq.wait()
        acc = [jnp.zeros((16, 128), f32), jnp.zeros((16, 128), f32)]
        if first:
            sacc = [jnp.zeros((16, 128), f32), jnp.zeros((16, 128), f32)]
            Lone = pltpu.bitcast(mask_rev & ones_w, bf16)
            Lone = jnp.concatenate([Lone] * T, axis=1)
        for c0 in range(0, 80, T):
            L = jnp.concatenate(
                [pltpu.bitcast(
                    jnp.take_along_axis(xw[:, 128 * (t // 16):128 * (t // 16 + 1)], exp_idx + 8 * (t % 16), axis=1)
                    & mask_rev, bf16) for t in range(c0, c0 + T)], axis=1)
            for hf in range(2):
                W = wq[8 * c0:8 * (c0 + T), 16 * hf:16 * hf + 16, :].reshape(128 * T, 128)
                if first:
                    o = _dot(jnp.concatenate([L, Lone], axis=0), W)
                    acc[hf] = acc[hf] + o[0:16]
                    sacc[hf] = sacc[hf] + o[16:32]
                else:
                    acc[hf] = acc[hf] + _dot(L, W)
        if first:
            for hf in range(2):
                qsum[hf] = sacc[hf]
        m16 = jnp.concatenate([mean, mean], axis=0)
        rs16 = jnp.concatenate([rs, rs], axis=0)
        q_rev = [((acc[hf] - m16 * qsum[hf]) * rs16).astype(bf16) for hf in range(2)]

        if first:
            cp_wuk.wait()
            rr, cc = consts128()
            eye = (rr == cc).astype(bf16)
            for hf in range(2):
                for a0 in range(0, 64, T):
                    W = wuk[8 * a0:8 * (a0 + T), 16 * hf:16 * hf + 16, :].reshape(128 * T, 128)
                    wukT[hf, :, 128 * a0:128 * (a0 + T)] = _dot_t(eye, W).astype(bf16)
        qa = []
        for b in range(4):
            halves = []
            for hf in range(2):
                accb = jnp.zeros((16, 128), f32)
                for j0 in range(0, 16, T):
                    a0 = 16 * b + j0
                    o = _dot(q_rev[hf], wukT[hf, :, 128 * a0:128 * (a0 + T)])
                    for jj in range(T):
                        j = j0 + jj
                        v = pltpu.roll(o[:, 128 * jj:128 * (jj + 1)], j, 1, stride=1, stride_axis=0)
                        accb = jnp.where((ln16 % 16) == (15 + j) % 16, v, accb)
                accb = accb * (D ** -0.5)
                halves += [jnp.take_along_axis(accb[8:16], rev_idx, axis=0),
                           jnp.take_along_axis(accb[0:8], rev_idx, axis=0)]
            qa.append(jnp.concatenate(halves, axis=0).astype(bf16))

        if first:
            cp_ckv.wait()
            rr, cc = consts128()
            pm1 = (cc == _c1(rr)).astype(bf16)
            p2 = (rr == _c2(cc)).astype(bf16)
            for k0 in range(0, S, 1024):
                for b in range(4):
                    blk = ckv[k0:k0 + 1024, 128 * b:128 * (b + 1)]
                    ckvT[128 * b:128 * (b + 1), k0:k0 + 1024] = _dot_t(pm1, blk).astype(bf16)
                    ckv2[k0:k0 + 1024, 128 * b:128 * (b + 1)] = _dot(blk, p2).astype(bf16)

        ms, ls, cxs = [], [], []

        def scores(i):
            k0 = i * KC
            sc = _dot(qa[0], ckvT[0:128, k0:k0 + KC])
            for b in range(1, 4):
                sc = sc + _dot(qa[b], ckvT[128 * b:128 * (b + 1), k0:k0 + KC])
            return sc

        def soft_ctx(i, sc):
            k0 = i * KC
            mx = sc[:, 0:128]
            for j in range(1, KC // 128):
                mx = jnp.maximum(mx, sc[:, 128 * j:128 * (j + 1)])
            mx = jnp.max(mx, axis=1, keepdims=True)
            p = jnp.exp(sc - mx)
            den = p[:, 0:128]
            for j in range(1, KC // 128):
                den = den + p[:, 128 * j:128 * (j + 1)]
            ms.append(mx)
            ls.append(den)
            cxs.append(_dot(p.astype(bf16), ckv2[k0:k0 + KC, :]))

        scs = [scores(0)]
        for i in range(NC):
            if i + 1 < NC:
                scs.append(scores(i + 1))
            soft_ctx(i, scs[i])
        mx = functools.reduce(jnp.maximum, ms)
        ws = [jnp.exp(m_ - mx) for m_ in ms]
        den = functools.reduce(jnp.add, [w_ * l_ for w_, l_ in zip(ws, ls)])
        inv = 1.0 / jnp.sum(den, axis=1, keepdims=True)
        cx = functools.reduce(jnp.add, [(w_ * inv) * c_ for w_, c_ in zip(ws, cxs)])
        cx = cx.astype(bf16).astype(f32)

        if first:
            cp_wuv.wait()
        ctx = []
        for hf in range(2):
            acc = jnp.zeros((16, 128), f32)
            for b in range(4):
                sb = cx[16 * hf:16 * hf + 16, 128 * b:128 * (b + 1)]
                for j0 in range(0, 16, T):
                    L = jnp.concatenate(
                        [jnp.where(diag_nat, pltpu.roll(sb, j, 1, stride=1, stride_axis=0), 0.0).astype(bf16)
                         for j in range(j0, j0 + T)], axis=1)
                    a0 = 16 * b + j0
                    W = wuv[8 * a0:8 * (a0 + T), 16 * hf:16 * hf + 16, :].reshape(128 * T, 128)
                    acc = acc + _dot(L, W)
            ctx.append(_dup(acc))

        if first:
            cp_wg.wait()
            cp_wu.wait()
            rr, cc = consts128()
            eye = (rr == cc).astype(bf16)
            for src, dst in ((wg, wgT), (wu, wuT)):
                for g in range(5):
                    for f0, n in ((0, 896), (896, 832)):
                        dst[128 * g:128 * (g + 1), f0:f0 + n] = _dot_t(
                            eye, src[f0:f0 + n, 128 * g:128 * (g + 1)]).astype(bf16)
            cp_wo.wait()
        acc = jnp.zeros((16, M), f32)
        HC = 4
        for h0 in range(0, H, HC):
            X = jnp.concatenate(
                [pltpu.bitcast(jnp.broadcast_to(ctx[h // 16][h % 16:h % 16 + 1], (8, 128)), bf16)
                 for h in range(h0, h0 + HC)], axis=1)
            acc = acc + _dot(X, wo[128 * h0:128 * (h0 + HC), :])
        return acc[0:8]

    def ffn(x, first):
        sub_m = _iota((8, M), 0)
        X = pltpu.bitcast(jnp.where(sub_m < 4, _dup(x), ones_w), bf16)
        mean, rs = _stats(x)
        xn = (x - mean) * rs
        r = jnp.sum(xn * wr, axis=1, keepdims=True)
        g = _dot(X, wgT[...])
        g = (g[0:8] - mean * g[8:16]) * rs
        u = _dot(X, wuT[...])
        u = (u[0:8] - mean * u[8:16]) * rs
        h = pltpu.bitcast(_dup(g * jax.nn.sigmoid(g) * u), bf16)
        y = None
        for i, (r0, n) in enumerate(WD_CHUNKS):
            if first:
                wd_copies[i].wait()
            o = _dot(h[:, r0:r0 + n], wd[r0:r0 + n, :])
            y = o if y is None else y + o
        return xn + y[0:8] * jax.nn.sigmoid(r)

    x = x + attention(x, True)
    x = x + ffn(x, True)
    x = x + attention(x, False)
    x = x + ffn(x, False)
    out_ref[0] = x[0:1].astype(bf16)
  return kernel


@jax.jit
def pallas_interleave_layers__compressed_kv_cla__moe_arch_mod__decode_kernel(
        A_x, A_c_kv, A_w_q, A_w_uk, A_w_uv, A_w_o, B_x, B_w_r, B_w_gate, B_w_up, B_w_down):
    interpret, T = False, 8
    del B_x
    vm = pl.BlockSpec(memory_space=pltpu.VMEM)
    hbm = pl.BlockSpec(memory_space=pl.ANY)
    scratch = [
        pltpu.VMEM((1, 1, M), bf16), pltpu.VMEM((M,), bf16),
        pltpu.VMEM((M, H, D), bf16), pltpu.VMEM((C, H, D), bf16), pltpu.VMEM((S, C), bf16),
        pltpu.VMEM((C, H, D), bf16), pltpu.VMEM((F, M), bf16), pltpu.VMEM((F, M), bf16),
        pltpu.VMEM((H * D, M), bf16), pltpu.VMEM((F, M), bf16),
        pltpu.VMEM((2, D, 64 * 128), bf16), pltpu.VMEM((C, S), bf16), pltpu.VMEM((S, C), bf16),
        pltpu.VMEM((M, F), bf16), pltpu.VMEM((M, F), bf16),
        pltpu.VMEM((2, 16, 128), f32),
        pltpu.SemaphoreType.DMA((9 + len(WD_CHUNKS),)),
    ]
    return pl.pallas_call(
        make_kernel(T),
        out_shape=jax.ShapeDtypeStruct((1, 1, M), bf16),
        in_specs=[hbm] * 10,
        out_specs=vm,
        scratch_shapes=scratch,
        compiler_params=pltpu.CompilerParams(vmem_limit_bytes=110 * 1024 * 1024),
        interpret=interpret,
        name="fused_decode",
    )(A_x, B_w_r, A_w_q, A_w_uk, A_c_kv.reshape(S, C), A_w_uv, B_w_gate.T, B_w_up.T,
      A_w_o.reshape(H * D, M), B_w_down)
```

```python
import functools
import jax
import jax.numpy as jnp
from jax import lax
from jax.experimental import pallas as pl
from jax.experimental.pallas import tpu as pltpu

M, H, D, C, S, F = 640, 32, 128, 512, 4096, 1728
f32, bf16, u32, i32 = jnp.float32, jnp.bfloat16, jnp.uint32, jnp.int32
EPS = 1e-5


class Cfg:
    T = 8
    MQ = 384
    HM = 18
    FV = 704
    WD_CHUNKS = ((0, 704), (704, 512), (1216, 384), (1600, 128))
    NC = 4


def _iota(shape, dim):
    return lax.broadcasted_iota(i32, shape, dim)


def _dot(a, b):
    return jnp.dot(a, b, preferred_element_type=f32)


def _dot_t(a, b):
    return lax.dot_general(a, b, (((1,), (1,)), ((), ())), preferred_element_type=f32)


def _ld(v):
    return pltpu.bitcast(v, bf16)


def _st(v):
    return pltpu.bitcast(v.astype(bf16), u32)


def _slab(ref, x0, n, hf):
    return _ld(ref[x0:x0 + n, 8 * hf:8 * hf + 8, :].reshape(8 * n, 128))


def _c1(p):
    j = (p + 1) % 16
    ci = ((p - 15 - j) % 128) // 16
    return 8 * j + ci


def _c2(p):
    j = (-p) % 16
    ci = ((p + j) % 128) // 16
    return 8 * j + ci


def _dup(x):
    w = lax.bitcast_convert_type(x.astype(bf16).astype(f32), u32)
    return w | (w >> 16)


def _stats(x):
    m = jnp.sum(x, axis=-1, keepdims=True) * (1.0 / M)
    ms = jnp.sum(x * x, axis=-1, keepdims=True) * (1.0 / M)
    return m, lax.rsqrt(jnp.maximum(ms - m * m, 0.0) + EPS)


def _subsum(v):
    v = v + pltpu.roll(v, 4, 0)
    v = v + pltpu.roll(v, 2, 0)
    return v + pltpu.roll(v, 1, 0)


def _spread(items, n):
    return [items[(len(items) * i) // n:(len(items) * (i + 1)) // n] for i in range(n)]


def make_kernel(cfg):
  T, MQ, HM, FV, WD_CHUNKS, NC = cfg.T, cfg.MQ, cfg.HM, cfg.FV, cfg.WD_CHUNKS, cfg.NC
  KC = S // NC
  FM = F - FV

  def kernel(x_hbm, wr_hbm, wq_hbm, wuk_hbm, ckv_hbm, wuv_hbm, wg_hbm, wu_hbm, wo_hbm, wd_hbm,
             out_ref,
             xs, wrs, wq, wuk, ckv, wuv, wg, wu, wo, wd,
             wukT, ckvT, ckv2, wgT, wuT, qsum, wqf, wof, wgf, wuf, wdf,
             st_x, st_y, st_h, sems):
    step = pl.program_id(0)
    srcs = [x_hbm, wr_hbm] + [r.bitcast(u32) for r in (wq_hbm, wuk_hbm, ckv_hbm, wuv_hbm, wg_hbm, wu_hbm, wo_hbm)]
    dsts = [xs, wrs, wq, wuk, ckv, wuv, wg, wu, wo]
    copies = [pltpu.make_async_copy(s, d, sems.at[i]) for i, (s, d) in enumerate(zip(srcs, dsts))]
    wd_w = wd_hbm.bitcast(u32)
    wd_copies = [pltpu.make_async_copy(wd_w.at[pl.ds(r0 // 2, n // 2)], wd.at[pl.ds(r0 // 2, n // 2)],
                                       sems.at[len(copies) + i])
                 for i, (r0, n) in enumerate(WD_CHUNKS)]
    cp_x, cp_wr, cp_wq, cp_wuk, cp_ckv, cp_wuv, cp_wg, cp_wu, cp_wo = copies

    sub = _iota((8, 128), 0)
    lane = _iota((8, 128), 1)
    l16 = lane % 16
    lo, hi, zero = jnp.uint32(0xFFFF), jnp.uint32(0xFFFF0000), jnp.uint32(0)
    ones_w = jnp.uint32(0x3F803F80)
    mask_rev = jnp.where(l16 == 15 - 2 * sub, lo, zero) | jnp.where(l16 == 14 - 2 * sub, hi, zero)
    r16 = _iota((16, 128), 0)
    ln16 = _iota((16, 128), 1)
    diag_nat = (ln16 % 16) == r16
    rev_idx = 7 - sub
    exp_idx = lane // 16
    col_idx = sub + 0 * lane

    def grid128():
        return _iota((128, 128), 0), _iota((128, 128), 1)

    def rev16(v):
        return jnp.concatenate([jnp.take_along_axis(v[8:16], rev_idx, axis=0),
                                jnp.take_along_axis(v[0:8], rev_idx, axis=0)], axis=0)

    def column(row_tile, first_lane):
        return jnp.take_along_axis(row_tile, col_idx + first_lane, axis=1)

    def attention(x, first):
        xw = _dup(x)
        mean, rs = _stats(x)
        if first:
            cp_wq.wait()
            for m0 in range(MQ, M, 32):
                wqf[m0 - MQ:m0 - MQ + 32] = _ld(wq[m0:m0 + 32]).astype(f32)
            sacc = [jnp.zeros((16, 128), f32), jnp.zeros((16, 128), f32)]
            Lone = jnp.concatenate([pltpu.bitcast(mask_rev & ones_w, bf16)] * T, axis=1)
        acc = [jnp.zeros((16, 128), f32), jnp.zeros((16, 128), f32)]
        vacc = [jnp.zeros((16, 128), f32), jnp.zeros((16, 128), f32)]
        nchunk = (M if first else MQ) // (8 * T)
        vparts = _spread([] if first else list(range(MQ // 8, M // 8)), nchunk)
        for ci in range(nchunk):
            c0 = ci * T
            L = jnp.concatenate(
                [pltpu.bitcast(
                    jnp.take_along_axis(xw[:, 128 * (t // 16):128 * (t // 16 + 1)], exp_idx + 8 * (t % 16), axis=1)
                    & mask_rev, bf16) for t in range(c0, c0 + T)], axis=1)
            for hf in range(2):
                W = _slab(wq, 8 * c0, 8 * T, hf)
                if first:
                    o = _dot(jnp.concatenate([L, Lone], axis=0), W)
                    acc[hf] = acc[hf] + o[0:16]
                    sacc[hf] = sacc[hf] + o[16:32]
                else:
                    acc[hf] = acc[hf] + _dot(L, W)
            for i in vparts[ci]:
                g = (8 * i) // 128
                col = column(x[:, 128 * g:128 * (g + 1)], (8 * i) % 128)
                for s_ in range(8):
                    sp = jnp.broadcast_to(col[s_:s_ + 1], (16, 128))
                    for hf in range(2):
                        vacc[hf] = vacc[hf] + sp * wqf[8 * i + s_ - MQ, 16 * hf:16 * hf + 16, :]
        if first:
            for hf in range(2):
                qsum[hf] = sacc[hf]
        else:
            acc = [acc[hf] + rev16(vacc[hf]) for hf in range(2)]
        m16 = jnp.concatenate([mean, mean], axis=0)
        rs16 = jnp.concatenate([rs, rs], axis=0)
        q_rev = [((acc[hf] - m16 * qsum[hf]) * rs16).astype(bf16) for hf in range(2)]

        if first:
            cp_wuk.wait()
            rr, cc = grid128()
            eye = (rr == cc).astype(bf16)
            for hf in range(2):
                for a0 in range(0, 64, T):
                    wukT[hf, :, 128 * a0:128 * (a0 + T)] = _st(_dot_t(eye, _slab(wuk, 8 * a0, 8 * T, hf)))
        qa = []
        for b in range(4):
            halves = []
            for hf in range(2):
                accb = jnp.zeros((16, 128), f32)
                for j0 in range(0, 16, T):
                    a0 = 16 * b + j0
                    o = _dot(q_rev[hf], _ld(wukT[hf, :, 128 * a0:128 * (a0 + T)]))
                    for jj in range(T):
                        j = j0 + jj
                        v = pltpu.roll(o[:, 128 * jj:128 * (jj + 1)], j, 1, stride=1, stride_axis=0)
                        accb = jnp.where((ln16 % 16) == (15 + j) % 16, v, accb)
                halves.append(rev16(accb * (D ** -0.5)))
            qa.append(jnp.concatenate(halves, axis=0).astype(bf16))

        if first:
            cp_ckv.wait()
            rr, cc = grid128()
            pm1 = (cc == _c1(rr)).astype(bf16)
            p2 = (rr == _c2(cc)).astype(bf16)
            for k0 in range(0, S, 1024):
                for b in range(4):
                    blk = _ld(ckv[k0 // 2:k0 // 2 + 512, 128 * b:128 * (b + 1)])
                    ckvT[64 * b:64 * (b + 1), k0:k0 + 1024] = _st(_dot_t(pm1, blk))
                    ckv2[k0 // 2:k0 // 2 + 512, 128 * b:128 * (b + 1)] = _st(_dot(blk, p2))
        ms, ls, cxs = [], [], []

        def scores(i):
            k0 = i * KC
            sc = _dot(qa[0], _ld(ckvT[0:64, k0:k0 + KC]))
            for b in range(1, 4):
                sc = sc + _dot(qa[b], _ld(ckvT[64 * b:64 * (b + 1), k0:k0 + KC]))
            return sc

        def soft_ctx(i, sc):
            k0 = i * KC
            mx = sc[:, 0:128]
            for j in range(1, KC // 128):
                mx = jnp.maximum(mx, sc[:, 128 * j:128 * (j + 1)])
            mx = jnp.max(mx, axis=1, keepdims=True)
            p = jnp.exp(sc - mx)
            den = p[:, 0:128]
            for j in range(1, KC // 128):
                den = den + p[:, 128 * j:128 * (j + 1)]
            ms.append(mx)
            ls.append(den)
            cxs.append(_dot(p.astype(bf16), _ld(ckv2[k0 // 2:(k0 + KC) // 2, :])))

        scs = [scores(0)]
        for i in range(NC):
            if i + 1 < NC:
                scs.append(scores(i + 1))
            soft_ctx(i, scs[i])
        mx = functools.reduce(jnp.maximum, ms)
        ws = [jnp.exp(m_ - mx) for m_ in ms]
        den = functools.reduce(jnp.add, [w_ * l_ for w_, l_ in zip(ws, ls)])
        inv = 1.0 / jnp.sum(den, axis=1, keepdims=True)
        cx = functools.reduce(jnp.add, [(w_ * inv) * c_ for w_, c_ in zip(ws, cxs)])

        if first:
            cp_wuv.wait()
        ctx = [None, None]
        for hf in (1, 0):
            acc = jnp.zeros((16, 128), f32)
            for b in range(4):
                sb = cx[16 * hf:16 * hf + 16, 128 * b:128 * (b + 1)]
                for j0 in range(0, 16, T):
                    L = jnp.concatenate(
                        [jnp.where(diag_nat, pltpu.roll(sb, j, 1, stride=1, stride_axis=0), 0.0).astype(bf16)
                         for j in range(j0, j0 + T)], axis=1)
                    acc = acc + _dot(L, _slab(wuv, 8 * (16 * b + j0), 8 * T, hf))
            ctx[hf] = acc

        if first:
            cp_wg.wait()
            cp_wu.wait()
            rr, cc = grid128()
            eye = (rr == cc).astype(bf16)
            for src, dst, dstf in ((wg, wgT, wgf), (wu, wuT, wuf)):
                for f0 in range(0, FV, 64):
                    dstf[f0:f0 + 64] = _ld(src[f0 // 2:f0 // 2 + 32]).astype(f32)
                for g in range(5):
                    for f0 in range(0, FM, 512):
                        dst[64 * g:64 * (g + 1), f0:f0 + 512] = _st(_dot_t(
                            eye, _ld(src[(FV + f0) // 2:(FV + f0 + 512) // 2, 128 * g:128 * (g + 1)])))
            cp_wo.wait()
            for r0 in range(128 * HM, H * D, 64):
                wof[r0 - 128 * HM:r0 - 128 * HM + 64] = _ld(wo[r0 // 2:r0 // 2 + 32]).astype(f32)
        ctxw = [_dup(c_) for c_ in ctx]
        acc = jnp.zeros((16, M), f32)
        vacc = jnp.zeros((8, M), f32)
        HC = 2
        mheads = list(range(H if first else HM))
        nchunk = len(mheads) // HC
        vparts = _spread([] if first else list(range(H - 1, HM - 1, -1)), nchunk)
        for ci in range(nchunk):
            hs = mheads[ci * HC:(ci + 1) * HC]
            X = jnp.concatenate(
                [pltpu.bitcast(jnp.broadcast_to(ctxw[h // 16][h % 16:h % 16 + 1], (8, 128)), bf16)
                 for h in hs], axis=1)
            acc = acc + _dot(X, _ld(wo[64 * hs[0]:64 * (hs[-1] + 1), :]))
            for h in vparts[ci]:
                row = jnp.broadcast_to(ctx[h // 16][h % 16:h % 16 + 1], (8, 128))
                for j in range(16):
                    r0 = 128 * (h - HM) + 8 * j
                    vacc = vacc + jnp.concatenate([column(row, 8 * j)] * 5, axis=1) * wof[r0:r0 + 8, :]
        out = acc[0:8]
        if not first:
            out = out + _subsum(vacc)
        return out

    def ffn_front(x):
        sub_m = _iota((8, M), 0)
        X = pltpu.bitcast(jnp.where(sub_m < 4, _dup(x), ones_w), bf16)
        mean, rs = _stats(x)
        xn = (x - mean) * rs
        wr = jnp.broadcast_to(wrs[...].reshape(1, M).astype(f32), (8, M))
        sig = jax.nn.sigmoid(jnp.sum(xn * wr, axis=1, keepdims=True))
        NB = FM // 256
        vparts = _spread(list(range(FV // 8)), NB)
        yv = jnp.zeros((8, M), f32)
        hs = []
        for bi in range(NB):
            g = _dot(X, _ld(wgT[:, 256 * bi:256 * (bi + 1)]))
            g = (g[0:8] - mean * g[8:16]) * rs
            u = _dot(X, _ld(wuT[:, 256 * bi:256 * (bi + 1)]))
            u = (u[0:8] - mean * u[8:16]) * rs
            hs.append(_dup(g * jax.nn.sigmoid(g) * u))
            for i in vparts[bi]:
                pg = wgf[8 * i:8 * i + 8, :] * xn
                pu = wuf[8 * i:8 * i + 8, :] * xn
                sg = pg[:, 0:128] + pg[:, 128:256] + pg[:, 256:384] + pg[:, 384:512] + pg[:, 512:640]
                su = pu[:, 0:128] + pu[:, 128:256] + pu[:, 256:384] + pu[:, 384:512] + pu[:, 512:640]
                gc = jnp.sum(sg, axis=1, keepdims=True)
                uc = jnp.sum(su, axis=1, keepdims=True)
                yv = yv + (gc * jax.nn.sigmoid(gc) * uc) * wdf[8 * i:8 * i + 8, :]
        return xn, sig, yv, jnp.concatenate(hs, axis=1)

    def down(hw, r0, n):
        return _dot(_ld(hw[:, r0 - FV:r0 - FV + n]), _ld(wd[r0 // 2:(r0 + n) // 2, :]))[0:8]

    @pl.when(step == 0)
    def _():
        for cp in copies + wd_copies:
            cp.start()
        cp_x.wait()
        cp_wr.wait()
        x = jnp.broadcast_to(xs[0].astype(f32), (8, M))
        x = x + attention(x, True)
        wd_copies[0].wait()
        for f0 in range(0, FV, 64):
            wdf[f0:f0 + 64] = _ld(wd[f0 // 2:f0 // 2 + 32]).astype(f32)
        xn, sig, yv, hw = ffn_front(x)
        y = _subsum(yv)
        for i, (r0, n) in enumerate(WD_CHUNKS[1:-1]):
            wd_copies[1 + i].wait()
            y = y + down(hw, r0, n)
        r0, n = WD_CHUNKS[-1]
        st_x[0] = x + xn + y * sig
        st_x[1] = jnp.broadcast_to(sig, (8, M))
        st_h[...] = hw[:, r0 - FV:r0 - FV + n]

    @pl.when(step == 1)
    def _():
        r0, n = WD_CHUNKS[-1]
        wd_copies[-1].wait()
        ylast = _dot(_ld(st_h[...]), _ld(wd[r0 // 2:(r0 + n) // 2, :]))[0:8]
        x = st_x[0] + ylast * st_x[1]
        x = x + attention(x, False)
        xn, sig, yv, hw = ffn_front(x)
        y = _subsum(yv) + down(hw, FV, FM)
        x = x + xn + y * sig
        out_ref[0] = x[0:1].astype(bf16)

  scratch = [
      pltpu.VMEM((1, 1, M), bf16), pltpu.VMEM((M,), bf16),
      pltpu.VMEM((M, H // 2, D), u32), pltpu.VMEM((C, H // 2, D), u32), pltpu.VMEM((S // 2, C), u32),
      pltpu.VMEM((C, H // 2, D), u32), pltpu.VMEM((F // 2, M), u32), pltpu.VMEM((F // 2, M), u32),
      pltpu.VMEM((H * D // 2, M), u32), pltpu.VMEM((F // 2, M), u32),
      pltpu.VMEM((2, D // 2, 64 * 128), u32), pltpu.VMEM((C // 2, S), u32), pltpu.VMEM((S // 2, C), u32),
      pltpu.VMEM((M // 2, FM), u32), pltpu.VMEM((M // 2, FM), u32),
      pltpu.VMEM((2, 16, 128), f32),
      pltpu.VMEM((M - MQ, H, D), f32), pltpu.VMEM(((H - HM) * D, M), f32),
      pltpu.VMEM((FV, M), f32), pltpu.VMEM((FV, M), f32), pltpu.VMEM((FV, M), f32),
      pltpu.VMEM((2, 8, M), f32), pltpu.VMEM((8, M), f32), pltpu.VMEM((8, WD_CHUNKS[-1][1]), u32),
      pltpu.SemaphoreType.DMA((9 + len(WD_CHUNKS),)),
  ]
  return kernel, scratch


@jax.jit
def pallas_interleave_layers__compressed_kv_cla__moe_arch_mod__decode_kernel(
        A_x, A_c_kv, A_w_q, A_w_uk, A_w_uv, A_w_o, B_x, B_w_r, B_w_gate, B_w_up, B_w_down):
    interpret, cfg = False, Cfg
    del B_x
    hbm = pl.BlockSpec(memory_space=pl.ANY)
    kernel, scratch = make_kernel(cfg)
    return pl.pallas_call(
        kernel,
        out_shape=jax.ShapeDtypeStruct((1, 1, M), bf16),
        grid=(2,),
        in_specs=[hbm] * 10,
        out_specs=pl.BlockSpec((1, 1, M), lambda i: (0, 0, 0)),
        scratch_shapes=scratch,
        compiler_params=pltpu.CompilerParams(vmem_limit_bytes=110 * 1024 * 1024,
                                             dimension_semantics=("arbitrary",)),
        interpret=interpret,
        name="fused_decode",
    )(A_x, B_w_r, A_w_q, A_w_uk, A_c_kv.reshape(S, C), A_w_uv, B_w_gate.T, B_w_up.T,
      A_w_o.reshape(H * D, M), B_w_down)
```

```python
import functools
import jax
import jax.numpy as jnp
from jax import lax
from jax.experimental import pallas as pl
from jax.experimental.pallas import tpu as pltpu

M, H, D, C, S, F = 640, 32, 128, 512, 4096, 1728
f32, bf16, u32, i32 = jnp.float32, jnp.bfloat16, jnp.uint32, jnp.int32
EPS = 1e-5


class Cfg:
    T = 8
    QV = ((240, 384), (448, 512), (576, 640))
    HM = 12
    HEARLY = 8
    GB = 4
    FV = 704
    WD = ((0, 1216, 0, 384), (1216, 512, 0, 384), (0, 1728, 384, 128), (0, 1728, 512, 128))
    NL = 2
    NC = 4


def _iota(shape, dim):
    return lax.broadcasted_iota(i32, shape, dim)


def _dot(a, b):
    return jnp.dot(a, b, preferred_element_type=f32)


def _dot_t(a, b):
    return lax.dot_general(a, b, (((1,), (1,)), ((), ())), preferred_element_type=f32)


def _ld(v):
    return pltpu.bitcast(v, bf16)


def _st(v):
    return pltpu.bitcast(v.astype(bf16), u32)


def _slab(ref, x0, n, hf):
    return _ld(ref[x0:x0 + n, 8 * hf:8 * hf + 8, :].reshape(8 * n, 128))


def _c1(p):
    j = (p + 1) % 16
    ci = ((p - 15 - j) % 128) // 16
    return 8 * j + ci


def _c2(p):
    j = (-p) % 16
    ci = ((p + j) % 128) // 16
    return 8 * j + ci


def _dup(x):
    w = lax.bitcast_convert_type(x.astype(bf16).astype(f32), u32)
    return w | (w >> 16)


def _dup_rows(x):
    return pltpu.bitcast(jnp.concatenate([x, x], axis=0).astype(bf16), u32)


def _stats(x):
    m = jnp.sum(x, axis=-1, keepdims=True) * (1.0 / M)
    ms = jnp.sum(x * x, axis=-1, keepdims=True) * (1.0 / M)
    return m, lax.rsqrt(jnp.maximum(ms - m * m, 0.0) + EPS)


def _subsum(v):
    v = v + pltpu.roll(v, 4, 0)
    v = v + pltpu.roll(v, 2, 0)
    return v + pltpu.roll(v, 1, 0)


def _silu(g):
    a = 0.5 * g
    return a + a * jnp.tanh(a)


def _sigmoid(r):
    return 0.5 + 0.5 * jnp.tanh(0.5 * r)


def _spread(items, n):
    return [items[(len(items) * i) // n:(len(items) * (i + 1)) // n] for i in range(n)]


def make_kernel(cfg):
  T, QV, HM, HEARLY, GB, FV, WD, NC = (cfg.T, cfg.QV, cfg.HM, cfg.HEARLY, cfg.GB, cfg.FV,
                                        cfg.WD, cfg.NC)
  HV = H - HM
  KC = S // NC
  FM = F - FV
  qv_rows = [m for lo_, hi_ in QV for m in range(lo_, hi_)]
  qv_pos = {m: i for i, m in enumerate(qv_rows)}

  def kernel(x_hbm, wr_hbm, wq_hbm, wuk_hbm, ckv_hbm, wuv_hbm, wg_hbm, wu_hbm, wo_hbm, wd_hbm,
             out_ref,
             xs, wrs, wq, wuk, ckv, wuv, wg, wu, wo, wd,
             wukT, ckvT, ckv2, wgT, wuT, qsum, wqf, woT, wgf, wuf, wdf,
             st_x, st_h, st_q, st_o, sems):
    step = pl.program_id(0)
    wg_w, wu_w = wg_hbm.bitcast(u32), wu_hbm.bitcast(u32)
    lo_f, hi_f = pl.ds(0, FV // 2), pl.ds(FV // 2, FM // 2)
    srcs = ([x_hbm, wr_hbm] + [r.bitcast(u32) for r in (wq_hbm, wuk_hbm, ckv_hbm, wuv_hbm, wo_hbm)]
            + [wg_w.at[hi_f], wu_w.at[hi_f], wg_w.at[lo_f], wu_w.at[lo_f]])
    dsts = [xs, wrs, wq, wuk, ckv, wuv, wo, wg.at[hi_f], wu.at[hi_f], wg.at[lo_f], wu.at[lo_f]]
    copies = [pltpu.make_async_copy(s, d, sems.at[i]) for i, (s, d) in enumerate(zip(srcs, dsts))]
    wd_w = wd_hbm.bitcast(u32)
    wd_copies = [pltpu.make_async_copy(wd_w.at[pl.ds(r0 // 2, n // 2), pl.ds(c0, nc)],
                                       wd.at[pl.ds(r0 // 2, n // 2), pl.ds(c0, nc)],
                                       sems.at[len(copies) + i])
                 for i, (r0, n, c0, nc) in enumerate(WD)]
    cp_x, cp_wr, cp_wq, cp_wuk, cp_ckv, cp_wuv, cp_wo, cp_wg1, cp_wu1, cp_wg0, cp_wu0 = copies

    sub = _iota((8, 128), 0)
    lane = _iota((8, 128), 1)
    l16 = lane % 16
    lo, hi, zero = jnp.uint32(0xFFFF), jnp.uint32(0xFFFF0000), jnp.uint32(0)
    ones_w = jnp.uint32(0x3F803F80)
    mask_rev = jnp.where(l16 == 15 - 2 * sub, lo, zero) | jnp.where(l16 == 14 - 2 * sub, hi, zero)
    mask_nat = jnp.where(l16 == 2 * sub, lo, zero) | jnp.where(l16 == 2 * sub + 1, hi, zero)
    ln16 = _iota((16, 128), 1)
    diag_nat = (ln16 % 16) == _iota((16, 128), 0)
    rev_idx = 7 - sub
    exp_idx = lane // 16
    col_idx = sub + 0 * lane
    zero_idx = 0 * lane

    def grid128():
        return _iota((128, 128), 0), _iota((128, 128), 1)

    def rev16(v):
        return jnp.concatenate([jnp.take_along_axis(v[8:16], rev_idx, axis=0),
                                jnp.take_along_axis(v[0:8], rev_idx, axis=0)], axis=0)

    def column(row_tile, first_lane):
        return jnp.take_along_axis(row_tile, col_idx + first_lane, axis=1)

    def q_partial(x, m_lo, m_hi, acc, with_sum):
        xw = _dup_rows(x)
        acc = list(acc)
        tiles = [t for t in range(m_lo // 8, m_hi // 8) if with_sum or 8 * t not in qv_pos]
        vgroups = [] if with_sum else [t for t in range(m_lo // 8, m_hi // 8) if 8 * t in qv_pos]
        chunks = [tiles[i:i + T] for i in range(0, len(tiles), T)]
        vparts = _spread(vgroups, len(chunks))
        if with_sum:
            sacc = [jnp.zeros((16, 128), f32), jnp.zeros((16, 128), f32)]
            one = pltpu.bitcast(mask_rev & ones_w, bf16)
        for ts, vs in zip(chunks, vparts):
            L = jnp.concatenate(
                [pltpu.bitcast(
                    jnp.take_along_axis(xw[:, 128 * (t // 16):128 * (t // 16 + 1)], exp_idx + 8 * (t % 16), axis=1)
                    & mask_rev, bf16) for t in ts], axis=1)
            for hf in range(2):
                W = jnp.concatenate([_slab(wq, 8 * t, 8, hf) for t in ts], axis=0)
                if with_sum:
                    o = _dot(jnp.concatenate([L, jnp.concatenate([one] * len(ts), axis=1)], axis=0), W)
                    acc[hf] = acc[hf] + o[0:16]
                    sacc[hf] = sacc[hf] + o[16:32]
                else:
                    acc[hf] = acc[hf] + _dot(L, W)
            for i in vs:
                g = (8 * i) // 128
                col = column(x[:, 128 * g:128 * (g + 1)], (8 * i) % 128)
                for s_ in range(0, 8, 2):
                    sp0 = jnp.broadcast_to(col[s_:s_ + 1], (16, 128))
                    sp1 = jnp.broadcast_to(col[s_ + 1:s_ + 2], (16, 128))
                    p0 = qv_pos[8 * i + s_]
                    for hf in range(2):
                        acc[2 + hf] = acc[2 + hf] + (sp0 * wqf[p0, 16 * hf:16 * hf + 16, :]
                                                     + sp1 * wqf[p0 + 1, 16 * hf:16 * hf + 16, :])
        if with_sum:
            for hf in range(2):
                qsum[hf] = sacc[hf]
        return acc

    def attention(x, qacc, first):
        mean, rs = _stats(x)
        m16 = jnp.concatenate([mean, mean], axis=0)
        rs16 = jnp.concatenate([rs, rs], axis=0)
        q_rev = [((qacc[hf] + rev16(qacc[2 + hf]) - m16 * qsum[hf]) * rs16).astype(bf16) for hf in range(2)]

        if first:
            cp_wuk.wait()
            rr, cc = grid128()
            eye = (rr == cc).astype(bf16)
            for hf in range(2):
                for a0 in range(0, 64, T):
                    wukT[hf, :, 128 * a0:128 * (a0 + T)] = _st(_dot_t(eye, _slab(wuk, 8 * a0, 8 * T, hf)))
        qa = []
        for b in range(4):
            halves = []
            for hf in range(2):
                accb = jnp.zeros((16, 128), f32)
                for j0 in range(0, 16, T):
                    a0 = 16 * b + j0
                    o = _dot(q_rev[hf], _ld(wukT[hf, :, 128 * a0:128 * (a0 + T)]))
                    for jj in range(T):
                        j = j0 + jj
                        v = pltpu.roll(o[:, 128 * jj:128 * (jj + 1)], j, 1, stride=1, stride_axis=0)
                        accb = jnp.where((ln16 % 16) == (15 + j) % 16, v, accb)
                halves.append(rev16(accb * (D ** -0.5)))
            qa.append(jnp.concatenate(halves, axis=0).astype(bf16))

        if first:
            cp_ckv.wait()
            rr, cc = grid128()
            pm1 = (cc == _c1(rr)).astype(bf16)
            p2 = (rr == _c2(cc)).astype(bf16)
            for k0 in range(0, S, 1024):
                for b in range(4):
                    blk = _ld(ckv[k0 // 2:k0 // 2 + 512, 128 * b:128 * (b + 1)])
                    ckvT[64 * b:64 * (b + 1), k0:k0 + 1024] = _st(_dot_t(pm1, blk))
                    ckv2[k0 // 2:k0 // 2 + 512, 128 * b:128 * (b + 1)] = _st(_dot(blk, p2))
        ms, ls, cxs, ps = [], [], [], []

        def scores(i):
            k0 = i * KC
            sc = _dot(qa[0], _ld(ckvT[0:64, k0:k0 + KC]))
            for b in range(1, 4):
                sc = sc + _dot(qa[b], _ld(ckvT[64 * b:64 * (b + 1), k0:k0 + KC]))
            return sc

        def soft(sc):
            mx = sc[:, 0:128]
            for j in range(1, KC // 128):
                mx = jnp.maximum(mx, sc[:, 128 * j:128 * (j + 1)])
            mx = jnp.max(mx, axis=1, keepdims=True)
            p = jnp.exp(sc - mx)
            den = p[:, 0:128]
            for j in range(1, KC // 128):
                den = den + p[:, 128 * j:128 * (j + 1)]
            ms.append(mx)
            ls.append(den)
            ps.append(p.astype(bf16))

        def ctx_all(i):
            o = _dot(ps[i], _ld(ckv2[i * KC // 2:(i + 1) * KC // 2, :]))
            cxs.append([o[:, 128 * b:128 * (b + 1)] for b in range(4)])

        def ctx_block(i, b):
            kq = KC // 4
            k0 = i * KC
            return functools.reduce(jnp.add, [
                _dot(ps[i][:, kq * u:kq * (u + 1)],
                     _ld(ckv2[(k0 + kq * u) // 2:(k0 + kq * (u + 1)) // 2, 128 * b:128 * (b + 1)]))
                for u in range(4)])

        NL = cfg.NL
        scs = [scores(0), scores(1)]
        soft(scs[0])
        for i in range(NC - NL):
            if i + 2 < NC:
                scs.append(scores(i + 2))
            ctx_all(i)
            soft(scs[i + 1])
        for i in range(NC - NL + 1, NC):
            soft(scs[i])
        tail = [[None] * 4 for _ in range(NL)]
        for b in range(4):
            for i in range(NL):
                tail[i][b] = ctx_block(NC - NL + i, b)
        cxs += tail
        mx = functools.reduce(jnp.maximum, ms)
        ws = [jnp.exp(m_ - mx) for m_ in ms]
        den = functools.reduce(jnp.add, [w_ * l_ for w_, l_ in zip(ws, ls)])
        inv = 1.0 / jnp.sum(den, axis=1, keepdims=True)
        cx = [functools.reduce(jnp.add, [w_ * c_[b] for w_, c_ in zip(ws, cxs)]) for b in range(4)]

        if first:
            cp_wuv.wait()
        ctx = [None, None]
        NG = M // 8
        vheads = [] if first else list(range(H - 1, HM - 1, -1))

        def vpu_block(g0, heads, init, final):
            if init:
                acc = [None] * GB
            else:
                acc = [st_o[g0 + k] for k in range(GB)]
            for h in heads:
                row = jnp.broadcast_to(ctx[h // 16][h % 16:h % 16 + 1], (8, 128))
                for k in range(GB):
                    t = woT[8 * (g0 + k):8 * (g0 + k + 1), 128 * (h - HM):128 * (h - HM + 1)] * row
                    acc[k] = t if acc[k] is None else acc[k] + t
            if not final:
                for k in range(GB):
                    st_o[g0 + k] = acc[k]
                return None
            return [jnp.sum(a_, axis=1, keepdims=True) for a_ in acc]

        blocks = list(range(0, NG, GB))
        for hf in (1, 0):
            acc = jnp.zeros((16, 128), f32)
            chunks = [(b, j0) for b in range(4) for j0 in range(0, 16, T)]
            vparts = _spread(blocks if (hf == 0 and not first) else [], len(chunks))
            for (b, j0), vs in zip(chunks, vparts):
                sb = cx[b][16 * hf:16 * hf + 16]
                L = jnp.concatenate(
                    [jnp.where(diag_nat, pltpu.roll(sb, j, 1, stride=1, stride_axis=0), 0.0)
                     for j in range(j0, j0 + T)], axis=1).astype(bf16)
                acc = acc + _dot(L, _slab(wuv, 8 * (16 * b + j0), 8 * T, hf))
                for g0 in vs:
                    vpu_block(g0, vheads[:HEARLY], True, False)
            ctx[hf] = acc * inv[16 * hf:16 * hf + 16]

        if first:
            cp_wo.wait()
            rr, cc = grid128()
            eye = (rr == cc).astype(bf16)
            for h in range(HM, H):
                woT[:, 128 * (h - HM):128 * (h - HM + 1)] = jnp.concatenate(
                    [_dot_t(eye, _ld(wo[64 * h:64 * (h + 1), 128 * g:128 * (g + 1)])) for g in range(5)], axis=0)
        acc = jnp.zeros((16, M), f32)
        HC = 2
        mheads = list(range(H if first else HM))
        nchunk = -(-len(mheads) // HC)
        vparts = _spread([] if first else blocks, nchunk)
        vrow = [jnp.zeros((8, 128), f32) for _ in range(5)]
        for ci in range(nchunk):
            hs = mheads[ci * HC:(ci + 1) * HC]
            X = jnp.concatenate(
                [jnp.broadcast_to(ctx[h // 16][h % 16:h % 16 + 1], (16, 128)) for h in hs], axis=1).astype(bf16)
            acc = acc + _dot(X, _ld(wo[64 * hs[0]:64 * (hs[-1] + 1), :]))
            for g0 in vparts[ci]:
                cols = vpu_block(g0, vheads[HEARLY:], False, True)
                for k, c_ in enumerate(cols):
                    gi = g0 + k
                    vrow[gi // 16] = jnp.where(lane == sub + 8 * (gi % 16), c_, vrow[gi // 16])
        out = acc[0:8]
        if not first:
            out = out + _subsum(jnp.concatenate(vrow, axis=1))
        return out

    def ffn_parts(x):
        X = jnp.concatenate([x, jnp.ones((8, M), f32)], axis=0).astype(bf16)
        mean, rs = _stats(x)
        xn = (x - mean) * rs
        wr = jnp.broadcast_to(wrs[...].reshape(1, M).astype(f32), (8, M))
        sig = _sigmoid(jnp.sum(xn * wr, axis=1, keepdims=True))
        return X, mean, rs, xn, sig

    def act(g, u, mean, rs):
        g = (g[0:8] - mean * g[8:16]) * rs
        u = (u[0:8] - mean * u[8:16]) * rs
        return _dup_rows(_silu(g) * u)

    def ffn_mxu_block(X, mean, rs, f0, n):
        return act(_dot(X, _ld(wgT[:, f0:f0 + n])), _dot(X, _ld(wuT[:, f0:f0 + n])), mean, rs)

    def wd_to_f32(c0, nc):
        for f0 in range(0, FV, 64):
            wdf[f0:f0 + 64, c0:c0 + nc] = _ld(wd[f0 // 2:f0 // 2 + 32, c0:c0 + nc]).astype(f32)

    @pl.when(step == 0)
    def _():
        for cp in copies + wd_copies:
            cp.start()
        cp_x.wait()
        cp_wr.wait()
        x = jnp.broadcast_to(xs[0].astype(f32), (8, M))
        cp_wq.wait()
        for lo_, hi_ in QV:
            for m0 in range(lo_, hi_, 16):
                wqf[qv_pos[m0]:qv_pos[m0] + 16] = _ld(wq[m0:m0 + 16]).astype(f32)
        z16 = jnp.zeros((16, 128), f32)
        qacc = q_partial(x, 0, M, [z16] * 4, True)
        x = x + attention(x, qacc, True)
        X, mean, rs, xn, sig = ffn_parts(x)
        rr, cc = grid128()
        eye = (rr == cc).astype(bf16)
        for cp, src, dst in ((cp_wg1, wg, wgT), (cp_wu1, wu, wuT)):
            cp.wait()
            for g in range(5):
                for f0 in range(0, FM, 512):
                    n = min(512, FM - f0)
                    dst[64 * g:64 * (g + 1), f0:f0 + n] = _st(_dot_t(
                        eye, _ld(src[(FV + f0) // 2:(FV + f0 + n) // 2, 128 * g:128 * (g + 1)])))
        hm = ffn_mxu_block(X, mean, rs, 0, FM)
        cp_wg0.wait()
        gv = _dot_t(X, _ld(wg[0:FV // 2, :]))
        for f0 in range(0, FV, 64):
            wgf[f0:f0 + 64] = _ld(wg[f0 // 2:f0 // 2 + 32]).astype(f32)
        cp_wu0.wait()
        hw = jnp.concatenate([act(gv, _dot_t(X, _ld(wu[0:FV // 2, :])), mean, rs), hm], axis=1)
        for f0 in range(0, FV, 64):
            wuf[f0:f0 + 64] = _ld(wu[f0 // 2:f0 // 2 + 32]).astype(f32)
        base = x + xn
        qacc = [z16] * 4
        ys = {}
        for cp, (r0, n, c0, nc) in zip(wd_copies[:-1], WD[:-1]):
            cp.wait()
            o = _dot(_ld(hw[:, r0:r0 + n]), _ld(wd[r0 // 2:(r0 + n) // 2, c0:c0 + nc]))[0:8]
            ys[c0] = o if c0 not in ys else ys[c0] + o
            if r0 + n == F:
                x2 = base[:, c0:c0 + nc] + ys[c0] * sig
                st_x[0, :, c0:c0 + nc] = x2
                xpad = jnp.concatenate([jnp.zeros((8, c0), f32), x2], axis=1) if c0 else x2
                qacc = q_partial(xpad, c0, c0 + nc, qacc, False)
                wd_to_f32(c0, nc)
        for i in range(4):
            st_q[i] = qacc[i]
        c0 = WD[-1][2]
        st_x[0, :, c0:M] = base[:, c0:M]
        st_x[1] = jnp.broadcast_to(sig, (8, M))
        st_h[...] = hw

    @pl.when(step == 1)
    def _():
        c0 = WD[-1][2]
        wd_copies[-1].wait()
        ylate = _dot(_ld(st_h[...]), _ld(wd[:, c0:M]))[0:8]
        x = jnp.concatenate([st_x[0, :, 0:c0], st_x[0, :, c0:M] + ylate * st_x[1, :, c0:M]], axis=1)
        qacc = q_partial(x, c0, M, [st_q[i] for i in range(4)], False)
        wd_to_f32(c0, M - c0)
        x = x + attention(x, qacc, False)
        X, mean, rs, xn, sig = ffn_parts(x)
        nb = FM // 128
        vparts = _spread(list(range(FV // 8)), nb)
        yv = jnp.zeros((8, M), f32)
        ym = None
        hs = []
        for bi in range(nb):
            hs.append(ffn_mxu_block(X, mean, rs, 128 * bi, 128))
            if bi >= 2:
                o = _dot(_ld(hs[bi - 2]), _ld(wd[(FV + 128 * (bi - 2)) // 2:(FV + 128 * (bi - 1)) // 2, :]))
                ym = o if ym is None else ym + o
            for i in vparts[bi]:
                pg = wgf[8 * i:8 * i + 8, :] * xn
                pu = wuf[8 * i:8 * i + 8, :] * xn
                sg = (pg[:, 0:128] + pg[:, 128:256]) + (pg[:, 256:384] + pg[:, 384:512]) + pg[:, 512:640]
                su = (pu[:, 0:128] + pu[:, 128:256]) + (pu[:, 256:384] + pu[:, 384:512]) + pu[:, 512:640]
                hc = _silu(jnp.sum(sg, axis=1, keepdims=True)) * jnp.sum(su, axis=1, keepdims=True)
                yv = yv + hc * wdf[8 * i:8 * i + 8, :]
        for bi in range(nb - 2, nb):
            ym = ym + _dot(_ld(hs[bi]), _ld(wd[(FV + 128 * bi) // 2:(FV + 128 * (bi + 1)) // 2, :]))
        y = _subsum(yv) + ym[0:8]
        x = x + xn + y * sig
        out_ref[0] = x[0:1].astype(bf16)

  scratch = [
      pltpu.VMEM((1, 1, M), bf16), pltpu.VMEM((M,), bf16),
      pltpu.VMEM((M, H // 2, D), u32), pltpu.VMEM((C, H // 2, D), u32), pltpu.VMEM((S // 2, C), u32),
      pltpu.VMEM((C, H // 2, D), u32), pltpu.VMEM((F // 2, M), u32), pltpu.VMEM((F // 2, M), u32),
      pltpu.VMEM((H * D // 2, M), u32), pltpu.VMEM((F // 2, M), u32),
      pltpu.VMEM((2, D // 2, 64 * 128), u32), pltpu.VMEM((C // 2, S), u32), pltpu.VMEM((S // 2, C), u32),
      pltpu.VMEM((M // 2, FM), u32), pltpu.VMEM((M // 2, FM), u32),
      pltpu.VMEM((2, 16, 128), f32),
      pltpu.VMEM((len(qv_rows), H, D), f32), pltpu.VMEM((M, HV * D), f32),
      pltpu.VMEM((FV, M), f32), pltpu.VMEM((FV, M), f32), pltpu.VMEM((FV, M), f32),
      pltpu.VMEM((2, 8, M), f32), pltpu.VMEM((8, F), u32), pltpu.VMEM((4, 16, 128), f32),
      pltpu.VMEM((M // 8, 8, 128), f32),
      pltpu.SemaphoreType.DMA((11 + len(WD),)),
  ]
  return kernel, scratch


@jax.jit
def pallas_interleave_layers__compressed_kv_cla__moe_arch_mod__decode_kernel(
        A_x, A_c_kv, A_w_q, A_w_uk, A_w_uv, A_w_o, B_x, B_w_r, B_w_gate, B_w_up, B_w_down):
    interpret, cfg = False, Cfg
    del B_x
    hbm = pl.BlockSpec(memory_space=pl.ANY)
    kernel, scratch = make_kernel(cfg)
    return pl.pallas_call(
        kernel,
        out_shape=jax.ShapeDtypeStruct((1, 1, M), bf16),
        grid=(2,),
        in_specs=[hbm] * 10,
        out_specs=pl.BlockSpec((1, 1, M), lambda i: (0, 0, 0)),
        scratch_shapes=scratch,
        compiler_params=pltpu.CompilerParams(vmem_limit_bytes=110 * 1024 * 1024,
                                             dimension_semantics=("arbitrary",)),
        interpret=interpret,
        name="fused_decode",
    )(A_x, B_w_r, A_w_q, A_w_uk, A_c_kv.reshape(S, C), A_w_uv, B_w_gate.T, B_w_up.T,
      A_w_o.reshape(H * D, M), B_w_down)
```

```python
import functools
import jax
import jax.numpy as jnp
from jax import lax
from jax.experimental import pallas as pl
from jax.experimental.pallas import tpu as pltpu

M, H, D, C, S, F = 640, 32, 128, 512, 4096, 1728
f32, bf16, u32, i32 = jnp.float32, jnp.bfloat16, jnp.uint32, jnp.int32
EPS = 1e-5


class Cfg:
    T = 8
    QV = ((240, 384), (448, 512), (576, 640))
    FV = 704
    WD = ((0, 1216, 0, 384), (1216, 512, 0, 384), (0, 1728, 384, 128), (0, 1728, 512, 128))
    NL = 2
    VG = 4
    NV = 40
    GATE_J = 8
    LAG = 6
    NC = 4


def _iota(shape, dim):
    return lax.broadcasted_iota(i32, shape, dim)


def _dot(a, b):
    return jnp.dot(a, b, preferred_element_type=f32)


def _dot_t(a, b):
    return lax.dot_general(a, b, (((1,), (1,)), ((), ())), preferred_element_type=f32)


def _ld(v):
    return pltpu.bitcast(v, bf16)


def _st(v):
    return pltpu.bitcast(v.astype(bf16), u32)


def _slab(ref, x0, n, hf):
    return _ld(ref[x0:x0 + n, 8 * hf:8 * hf + 8, :].reshape(8 * n, 128))


def _c1(p):
    return 16 * (p % 8) + (p // 8 + 15) % 16


def _c2(p):
    return 8 * (p % 16) + (p // 16 + 1) % 8


def _dup(x):
    w = lax.bitcast_convert_type(x.astype(bf16).astype(f32), u32)
    return w | (w >> 16)


def _dup_rows(x):
    return pltpu.bitcast(jnp.concatenate([x, x], axis=0).astype(bf16), u32)


def _stats(x):
    m = jnp.sum(x, axis=-1, keepdims=True) * (1.0 / M)
    ms = jnp.sum(x * x, axis=-1, keepdims=True) * (1.0 / M)
    return m, lax.rsqrt(jnp.maximum(ms - m * m, 0.0) + EPS)


def _subsum(v):
    v = v + pltpu.roll(v, 4, 0)
    v = v + pltpu.roll(v, 2, 0)
    return v + pltpu.roll(v, 1, 0)


def _silu(g):
    a = 0.5 * g
    return a + a * jnp.tanh(a)


def _sigmoid(r):
    return 0.5 + 0.5 * jnp.tanh(0.5 * r)


def _after(x, gate):
    return lax.bitcast_convert_type(lax.bitcast_convert_type(x, u32) | gate, f32)


def _spread(items, n):
    return [items[(len(items) * i) // n:(len(items) * (i + 1)) // n] for i in range(n)]


def make_kernel(cfg):
  T, QV, FV, WD, NC = cfg.T, cfg.QV, cfg.FV, cfg.WD, cfg.NC
  KC = S // NC
  FM = F - FV
  qv_rows = [m for lo_, hi_ in QV for m in range(lo_, hi_)]
  qv_pos = {m: i for i, m in enumerate(qv_rows)}

  def kernel(x_hbm, wr_hbm, wq_hbm, wuk_hbm, ckv_hbm, wuv_hbm, wg_hbm, wu_hbm, wo_hbm, wd_hbm,
             out_ref,
             xs, wrs, wq, wuk, ckv, wuv, wg, wu, wo, wd,
             wukT, wukTf, ckvT, ckv2, wgT, wuT, qsum, wqf, gat, wuvT, wof, wgf, wuf, wdf,
             st_x, st_h, st_q, sems):
    step = pl.program_id(0)
    wg_w, wu_w = wg_hbm.bitcast(u32), wu_hbm.bitcast(u32)
    lo_f, hi_f = pl.ds(0, FV // 2), pl.ds(FV // 2, FM // 2)
    srcs = ([x_hbm, wr_hbm] + [r.bitcast(u32) for r in (wq_hbm, wuk_hbm, ckv_hbm, wuv_hbm, wo_hbm)]
            + [wg_w.at[hi_f], wu_w.at[hi_f], wg_w.at[lo_f], wu_w.at[lo_f]])
    dsts = [xs, wrs, wq, wuk, ckv, wuv, wo, wg.at[hi_f], wu.at[hi_f], wg.at[lo_f], wu.at[lo_f]]
    copies = [pltpu.make_async_copy(s, d, sems.at[i]) for i, (s, d) in enumerate(zip(srcs, dsts))]
    wd_w = wd_hbm.bitcast(u32)
    wd_copies = [pltpu.make_async_copy(wd_w.at[pl.ds(r0 // 2, n // 2), pl.ds(c0, nc)],
                                       wd.at[pl.ds(r0 // 2, n // 2), pl.ds(c0, nc)],
                                       sems.at[len(copies) + i])
                 for i, (r0, n, c0, nc) in enumerate(WD)]
    cp_x, cp_wr, cp_wq, cp_wuk, cp_ckv, cp_wuv, cp_wo, cp_wg1, cp_wu1, cp_wg0, cp_wu0 = copies

    sub = _iota((8, 128), 0)
    lane = _iota((8, 128), 1)
    l16 = lane % 16
    lo, hi, zero = jnp.uint32(0xFFFF), jnp.uint32(0xFFFF0000), jnp.uint32(0)
    ones_w = jnp.uint32(0x3F803F80)
    mask_rev = jnp.where(l16 == 15 - 2 * sub, lo, zero) | jnp.where(l16 == 14 - 2 * sub, hi, zero)
    mask_nat = jnp.where(l16 == 2 * sub, lo, zero) | jnp.where(l16 == 2 * sub + 1, hi, zero)
    ln16 = _iota((16, 128), 1)
    diag_nat = (ln16 % 16) == _iota((16, 128), 0)
    rev_idx = 7 - sub
    exp_idx = lane // 16
    col_idx = sub + 0 * lane
    zero_idx = 0 * lane

    zero_w = jnp.full((8, 128), step - 1, i32).astype(u32)

    def fence(v):
        return lax.bitcast_convert_type(jnp.broadcast_to(v, (8, 128)), u32) & zero_w

    def grid128():
        return _iota((128, 128), 0), _iota((128, 128), 1)

    def rev16(v):
        return jnp.concatenate([jnp.take_along_axis(v[8:16], rev_idx, axis=0),
                                jnp.take_along_axis(v[0:8], rev_idx, axis=0)], axis=0)

    def column(row_tile, first_lane):
        return jnp.take_along_axis(row_tile, col_idx + first_lane, axis=1)

    def q_partial(x, m_lo, m_hi, acc, with_sum):
        xw = _dup_rows(x)
        acc = list(acc)
        tiles = [t for t in range(m_lo // 8, m_hi // 8) if with_sum or 8 * t not in qv_pos]
        vgroups = [] if with_sum else [t for t in range(m_lo // 8, m_hi // 8) if 8 * t in qv_pos]
        chunks = [tiles[i:i + T] for i in range(0, len(tiles), T)]
        vparts = _spread(vgroups, len(chunks))
        if with_sum:
            sacc = [jnp.zeros((16, 128), f32), jnp.zeros((16, 128), f32)]
            one = pltpu.bitcast(mask_rev & ones_w, bf16)
        for ts, vs in zip(chunks, vparts):
            L = jnp.concatenate(
                [pltpu.bitcast(
                    jnp.take_along_axis(xw[:, 128 * (t // 16):128 * (t // 16 + 1)], exp_idx + 8 * (t % 16), axis=1)
                    & mask_rev, bf16) for t in ts], axis=1)
            for hf in range(2):
                W = jnp.concatenate([_slab(wq, 8 * t, 8, hf) for t in ts], axis=0)
                if with_sum:
                    o = _dot(jnp.concatenate([L, jnp.concatenate([one] * len(ts), axis=1)], axis=0), W)
                    acc[hf] = acc[hf] + o[0:16]
                    sacc[hf] = sacc[hf] + o[16:32]
                else:
                    acc[hf] = acc[hf] + _dot(L, W)
            for i in vs:
                g = (8 * i) // 128
                col = column(x[:, 128 * g:128 * (g + 1)], (8 * i) % 128)
                for s_ in range(0, 8, 2):
                    sp0 = jnp.broadcast_to(col[s_:s_ + 1], (16, 128))
                    sp1 = jnp.broadcast_to(col[s_ + 1:s_ + 2], (16, 128))
                    p0 = qv_pos[8 * i + s_]
                    for hf in range(2):
                        acc[2 + hf] = acc[2 + hf] + (sp0 * wqf[p0, 16 * hf:16 * hf + 16, :]
                                                     + sp1 * wqf[p0 + 1, 16 * hf:16 * hf + 16, :])
        if with_sum:
            for hf in range(2):
                qsum[hf] = sacc[hf]
        return acc

    def attention(x, qacc, first):
        mean, rs = _stats(x)
        m16 = jnp.concatenate([mean, mean], axis=0)
        rs16 = jnp.concatenate([rs, rs], axis=0)
        q_rev = [(qacc[hf] + rev16(qacc[2 + hf]) - m16 * qsum[hf]) * rs16 for hf in range(2)]
        q_qt = [q_rev[qt // 2][8 * (1 - qt % 2):8 * (2 - qt % 2)] for qt in range(4)]

        vtiles = [(3 - i // 32, i % 32) for i in range(cfg.NV)]
        if first:
            cp_wuk.wait()
            rr, cc = grid128()
            eye = (rr == cc).astype(bf16)
            for qt in range(4):
                for a0 in range(0, 32, 4):
                    W = _ld(wuk[16 * a0:16 * (a0 + 4), 4 * qt:4 * qt + 4, :].reshape(256, 128))
                    o = _dot_t(eye, W)
                    wukT[qt, :, 128 * a0:128 * (a0 + 4)] = _st(o)
                    for a in range(a0, a0 + 4):
                        if (qt, a) in vtiles:
                            wukTf[vtiles.index((qt, a))] = o[:, 128 * (a - a0):128 * (a - a0 + 1)]
        acc = [[jnp.zeros((8, 128), f32) for _ in range(4)] for _ in range(4)]

        def place(qt, a, v):
            j = a % 8
            v = pltpu.roll(v, j + 1, 1, stride=1, stride_axis=0)
            acc[qt][a // 8] = jnp.where((lane % 8) == j, v, acc[qt][a // 8])

        for qt in range(4):
            lhs = jnp.concatenate([q_qt[qt], q_qt[qt]], axis=0).astype(bf16)
            mt = [a for a in range(32) if first or (qt, a) not in vtiles]
            for i0 in range(0, len(mt), T):
                run_ = mt[i0:i0 + T]
                assert run_ == list(range(run_[0], run_[0] + len(run_)))
                o = _dot(lhs, _ld(wukT[qt, :, 128 * run_[0]:128 * (run_[-1] + 1)]))[0:8]
                for k, a in enumerate(run_):
                    place(qt, a, o[:, 128 * k:128 * (k + 1)])
        if not first:
            for qt in sorted({t[0] for t in vtiles}, reverse=True):
                q_nat = jnp.take_along_axis(q_qt[qt], rev_idx, axis=0)
                qc = jnp.concatenate([q_nat] * 16, axis=0).T
                mine = [i for i, t in enumerate(vtiles) if t[0] == qt]
                for i0 in range(0, len(mine), cfg.VG):
                    grp = mine[i0:i0 + cfg.VG]
                    zs = [None] * len(grp)
                    for dv in range(16):
                        qv = qc[8 * dv:8 * dv + 8]
                        for k, i in enumerate(grp):
                            t = wukTf[i, 8 * dv:8 * dv + 8, :] * qv
                            zs[k] = t if zs[k] is None else zs[k] + t
                    for k, i in enumerate(grp):
                        place(qt, vtiles[i][1], _subsum(zs[k]))
        qa = [(jnp.concatenate([jnp.take_along_axis(acc[qt][b], rev_idx, axis=0) for qt in range(4)], axis=0)
               * (D ** -0.5)).astype(bf16) for b in range(4)]

        if first:
            cp_ckv.wait()
            rr, cc = grid128()
            pm1 = (cc == _c1(rr)).astype(bf16)
            p2 = (rr == _c2(cc)).astype(bf16)
            for k0 in range(0, S, 1024):
                for b in range(4):
                    blk = _ld(ckv[k0 // 2:k0 // 2 + 512, 128 * b:128 * (b + 1)])
                    ckvT[64 * b:64 * (b + 1), k0:k0 + 1024] = _st(_dot_t(pm1, blk))
                    ckv2[k0 // 2:k0 // 2 + 512, 128 * b:128 * (b + 1)] = _st(_dot(blk, p2))
        ms, ls, cxs, ps = [], [], [], []

        def scores(i):
            k0 = i * KC
            sc = _dot(qa[0], _ld(ckvT[0:64, k0:k0 + KC]))
            for b in range(1, 4):
                sc = sc + _dot(qa[b], _ld(ckvT[64 * b:64 * (b + 1), k0:k0 + KC]))
            return sc

        def soft(sc):
            mx = sc[:, 0:128]
            for j in range(1, KC // 128):
                mx = jnp.maximum(mx, sc[:, 128 * j:128 * (j + 1)])
            mx = jnp.max(mx, axis=1, keepdims=True)
            p = jnp.exp(sc - mx)
            den = p[:, 0:128]
            for j in range(1, KC // 128):
                den = den + p[:, 128 * j:128 * (j + 1)]
            ms.append(mx)
            ls.append(den)
            ps.append(p.astype(bf16))

        def ctx_all(i):
            o = _dot(ps[i], _ld(ckv2[i * KC // 2:(i + 1) * KC // 2, :]))
            cxs.append([o[:, 128 * b:128 * (b + 1)] for b in range(4)])

        def ctx_block(i, b):
            kq = KC // 4
            k0 = i * KC
            return functools.reduce(jnp.add, [
                _dot(ps[i][:, kq * u:kq * (u + 1)],
                     _ld(ckv2[(k0 + kq * u) // 2:(k0 + kq * (u + 1)) // 2, 128 * b:128 * (b + 1)]))
                for u in range(4)])

        NL = cfg.NL
        scs = [scores(0), scores(1)]
        soft(scs[0])
        for i in range(NC - NL):
            if i + 2 < NC:
                scs.append(scores(i + 2))
            ctx_all(i)
            soft(scs[i + 1])
        for i in range(NC - NL + 1, NC):
            soft(scs[i])
        tail = [[None] * 4 for _ in range(NL)]
        for b in range(4):
            for i in range(NL):
                tail[i][b] = ctx_block(NC - NL + i, b)
        cxs += tail
        mx = functools.reduce(jnp.maximum, ms)
        ws = [jnp.exp(m_ - mx) for m_ in ms]
        den = functools.reduce(jnp.add, [w_ * l_ for w_, l_ in zip(ws, ls)])
        inv = 1.0 / jnp.sum(den, axis=1, keepdims=True)
        cx = [functools.reduce(jnp.add, [w_ * c_[b] for w_, c_ in zip(ws, cxs)]) for b in range(4)]

        if first:
            cp_wuv.wait()
            for bq in range(64):
                b, q = bq // 16, bq % 16
                c0 = 128 * b + 64 * (q % 2) + (q // 2 + 1) % 8
                gat[:, 8 * bq:8 * bq + 8, :] = jnp.swapaxes(wuv[pl.ds(c0, 8, stride=8), 8:16, :], 0, 1)
            rr, cc = grid128()
            eye = (rr == cc).astype(bf16)
            for r in range(8):
                for b in range(4):
                    w = gat[r, 128 * b:128 * (b + 1), :]
                    for e, bits in enumerate((w << 16, w & hi)):
                        t = lax.bitcast_convert_type(bits, f32).astype(bf16)
                        wuvT[2 * r + e, :, 128 * b:128 * (b + 1)] = _dot_t(eye, t)

        def value_half(hf):
            acc = jnp.zeros((16, 128), f32)
            for b in range(4):
                sb = cx[b][16 * hf:16 * hf + 16]
                for j0 in range(0, 16, T):
                    L = jnp.concatenate(
                        [jnp.where(diag_nat, pltpu.roll(sb, 16 - j, 1, stride=1, stride_axis=0), 0.0)
                         for j in range(j0, j0 + T)], axis=1).astype(bf16)
                    acc = acc + _dot(L, _slab(wuv, 8 * (16 * b + j0), 8 * T, hf))
            return acc * inv[16 * hf:16 * hf + 16]

        ctx = [value_half(0)] + ([value_half(1)] if first else [])
        if first:
            cp_wo.wait()
            for r0 in range(0, 16 * D, 64):
                wof[r0:r0 + 64] = _ld(wo[(16 * D + r0) // 2:(16 * D + r0) // 2 + 32]).astype(f32)
        acc = jnp.zeros((16, M), f32)
        HC = 2
        for h0 in range(0, H if first else 16, HC):
            X = jnp.concatenate(
                [jnp.broadcast_to(ctx[h // 16][h % 16:h % 16 + 1], (16, 128)) for h in range(h0, h0 + HC)],
                axis=1).astype(bf16)
            acc = acc + _dot(X, _ld(wo[64 * h0:64 * (h0 + HC), :]))
        out = acc[0:8]
        if not first:
            cxn = [cx[b][16:32] * inv[16:32] for b in range(4)]
            vacc = jnp.zeros((8, M), f32)
            gates = []
            for h in range(16):
                rows = [jnp.broadcast_to(cxn[b][h:h + 1], (8, 128)) for b in range(4)]
                if h >= cfg.LAG:
                    rows = [_after(r_, gates[h - cfg.LAG]) for r_ in rows]
                for j in range(0, 16, 2):
                    cols = []
                    for jj in (j, j + 1):
                        w = wuvT[h, 8 * jj:8 * jj + 8, :]
                        s_ = ((w[:, 0:128] * rows[0] + w[:, 128:256] * rows[1])
                              + (w[:, 256:384] * rows[2] + w[:, 384:512] * rows[3]))
                        cols.append(jnp.sum(s_, axis=1, keepdims=True))
                    if j == cfg.GATE_J:
                        gates.append(fence(cols[0]))
                    r0 = 128 * h + 8 * j
                    vacc = vacc + (cols[0] * wof[r0:r0 + 8, :] + cols[1] * wof[r0 + 8:r0 + 16, :])
            out = out + _subsum(vacc)
        return out

    def ffn_parts(x):
        X = jnp.concatenate([x, jnp.ones((8, M), f32)], axis=0).astype(bf16)
        mean, rs = _stats(x)
        xn = (x - mean) * rs
        wr = jnp.broadcast_to(wrs[...].reshape(1, M).astype(f32), (8, M))
        sig = _sigmoid(jnp.sum(xn * wr, axis=1, keepdims=True))
        return X, mean, rs, xn, sig

    def act(g, u, mean, rs):
        g = (g[0:8] - mean * g[8:16]) * rs
        u = (u[0:8] - mean * u[8:16]) * rs
        return _dup_rows(_silu(g) * u)

    def ffn_mxu_block(X, mean, rs, f0, n):
        return act(_dot(X, _ld(wgT[:, f0:f0 + n])), _dot(X, _ld(wuT[:, f0:f0 + n])), mean, rs)

    def wd_to_f32(c0, nc):
        for f0 in range(0, FV, 64):
            wdf[f0:f0 + 64, c0:c0 + nc] = _ld(wd[f0 // 2:f0 // 2 + 32, c0:c0 + nc]).astype(f32)

    @pl.when(step == 0)
    def _():
        for cp in copies + wd_copies:
            cp.start()
        cp_x.wait()
        cp_wr.wait()
        x = jnp.broadcast_to(xs[0].astype(f32), (8, M))
        cp_wq.wait()
        for lo_, hi_ in QV:
            for m0 in range(lo_, hi_, 16):
                wqf[qv_pos[m0]:qv_pos[m0] + 16] = _ld(wq[m0:m0 + 16]).astype(f32)
        z16 = jnp.zeros((16, 128), f32)
        qacc = q_partial(x, 0, M, [z16] * 4, True)
        x = x + attention(x, qacc, True)
        X, mean, rs, xn, sig = ffn_parts(x)
        rr, cc = grid128()
        eye = (rr == cc).astype(bf16)
        for cp, src, dst in ((cp_wg1, wg, wgT), (cp_wu1, wu, wuT)):
            cp.wait()
            for g in range(5):
                for f0 in range(0, FM, 512):
                    n = min(512, FM - f0)
                    dst[64 * g:64 * (g + 1), f0:f0 + n] = _st(_dot_t(
                        eye, _ld(src[(FV + f0) // 2:(FV + f0 + n) // 2, 128 * g:128 * (g + 1)])))
        hm = ffn_mxu_block(X, mean, rs, 0, FM)
        cp_wg0.wait()
        gv = _dot_t(X, _ld(wg[0:FV // 2, :]))
        for f0 in range(0, FV, 64):
            wgf[f0:f0 + 64] = _ld(wg[f0 // 2:f0 // 2 + 32]).astype(f32)
        cp_wu0.wait()
        hw = jnp.concatenate([act(gv, _dot_t(X, _ld(wu[0:FV // 2, :])), mean, rs), hm], axis=1)
        for f0 in range(0, FV, 64):
            wuf[f0:f0 + 64] = _ld(wu[f0 // 2:f0 // 2 + 32]).astype(f32)
        base = x + xn
        qacc = [z16] * 4
        ys = {}
        for cp, (r0, n, c0, nc) in zip(wd_copies[:-1], WD[:-1]):
            cp.wait()
            o = _dot(_ld(hw[:, r0:r0 + n]), _ld(wd[r0 // 2:(r0 + n) // 2, c0:c0 + nc]))[0:8]
            ys[c0] = o if c0 not in ys else ys[c0] + o
            if r0 + n == F:
                x2 = base[:, c0:c0 + nc] + ys[c0] * sig
                st_x[0, :, c0:c0 + nc] = x2
                xpad = jnp.concatenate([jnp.zeros((8, c0), f32), x2], axis=1) if c0 else x2
                qacc = q_partial(xpad, c0, c0 + nc, qacc, False)
                wd_to_f32(c0, nc)
        for i in range(4):
            st_q[i] = qacc[i]
        c0 = WD[-1][2]
        st_x[0, :, c0:M] = base[:, c0:M]
        st_x[1] = jnp.broadcast_to(sig, (8, M))
        st_h[...] = hw

    @pl.when(step == 1)
    def _():
        c0 = WD[-1][2]
        wd_copies[-1].wait()
        ylate = _dot(_ld(st_h[...]), _ld(wd[:, c0:M]))[0:8]
        x = jnp.concatenate([st_x[0, :, 0:c0], st_x[0, :, c0:M] + ylate * st_x[1, :, c0:M]], axis=1)
        qacc = q_partial(x, c0, M, [st_q[i] for i in range(4)], False)
        wd_to_f32(c0, M - c0)
        x = x + attention(x, qacc, False)
        X, mean, rs, xn, sig = ffn_parts(x)
        nb = FM // 128
        vparts = _spread(list(range(FV // 8)), nb)
        yv = jnp.zeros((8, M), f32)
        ym = None
        hs = []
        for bi in range(nb):
            hs.append(ffn_mxu_block(X, mean, rs, 128 * bi, 128))
            if bi >= 2:
                o = _dot(_ld(hs[bi - 2]), _ld(wd[(FV + 128 * (bi - 2)) // 2:(FV + 128 * (bi - 1)) // 2, :]))
                ym = o if ym is None else ym + o
            for i in vparts[bi]:
                pg = wgf[8 * i:8 * i + 8, :] * xn
                pu = wuf[8 * i:8 * i + 8, :] * xn
                sg = (pg[:, 0:128] + pg[:, 128:256]) + (pg[:, 256:384] + pg[:, 384:512]) + pg[:, 512:640]
                su = (pu[:, 0:128] + pu[:, 128:256]) + (pu[:, 256:384] + pu[:, 384:512]) + pu[:, 512:640]
                hc = _silu(jnp.sum(sg, axis=1, keepdims=True)) * jnp.sum(su, axis=1, keepdims=True)
                yv = yv + hc * wdf[8 * i:8 * i + 8, :]
        for bi in range(nb - 2, nb):
            ym = ym + _dot(_ld(hs[bi]), _ld(wd[(FV + 128 * bi) // 2:(FV + 128 * (bi + 1)) // 2, :]))
        y = _subsum(yv) + ym[0:8]
        x = x + xn + y * sig
        out_ref[0] = x[0:1].astype(bf16)

  scratch = [
      pltpu.VMEM((1, 1, M), bf16), pltpu.VMEM((M,), bf16),
      pltpu.VMEM((M, H // 2, D), u32), pltpu.VMEM((C, H // 2, D), u32), pltpu.VMEM((S // 2, C), u32),
      pltpu.VMEM((C, H // 2, D), u32), pltpu.VMEM((F // 2, M), u32), pltpu.VMEM((F // 2, M), u32),
      pltpu.VMEM((H * D // 2, M), u32), pltpu.VMEM((F // 2, M), u32),
      pltpu.VMEM((4, D // 2, 32 * 128), u32), pltpu.VMEM((cfg.NV, D, 128), f32),
      pltpu.VMEM((C // 2, S), u32), pltpu.VMEM((S // 2, C), u32),
      pltpu.VMEM((M // 2, FM), u32), pltpu.VMEM((M // 2, FM), u32),
      pltpu.VMEM((2, 16, 128), f32),
      pltpu.VMEM((len(qv_rows), H, D), f32),
      pltpu.VMEM((8, C, D), u32), pltpu.VMEM((16, D, C), f32), pltpu.VMEM((16 * D, M), f32),
      pltpu.VMEM((FV, M), f32), pltpu.VMEM((FV, M), f32), pltpu.VMEM((FV, M), f32),
      pltpu.VMEM((2, 8, M), f32), pltpu.VMEM((8, F), u32), pltpu.VMEM((4, 16, 128), f32),
      pltpu.SemaphoreType.DMA((11 + len(WD),)),
  ]
  return kernel, scratch


@jax.jit
def pallas_interleave_layers__compressed_kv_cla__moe_arch_mod__decode_kernel(
        A_x, A_c_kv, A_w_q, A_w_uk, A_w_uv, A_w_o, B_x, B_w_r, B_w_gate, B_w_up, B_w_down):
    interpret, cfg = False, Cfg
    del B_x
    hbm = pl.BlockSpec(memory_space=pl.ANY)
    kernel, scratch = make_kernel(cfg)
    return pl.pallas_call(
        kernel,
        out_shape=jax.ShapeDtypeStruct((1, 1, M), bf16),
        grid=(2,),
        in_specs=[hbm] * 10,
        out_specs=pl.BlockSpec((1, 1, M), lambda i: (0, 0, 0)),
        scratch_shapes=scratch,
        compiler_params=pltpu.CompilerParams(vmem_limit_bytes=110 * 1024 * 1024,
                                             dimension_semantics=("arbitrary",)),
        interpret=interpret,
        name="fused_decode",
    )(A_x, B_w_r, A_w_q, A_w_uk, A_c_kv.reshape(S, C), A_w_uv, B_w_gate.T, B_w_up.T,
      A_w_o.reshape(H * D, M), B_w_down)
```

```python
import functools
import jax
import jax.numpy as jnp
from jax import lax
from jax.experimental import pallas as pl
from jax.experimental.pallas import tpu as pltpu

M, H, D, C, S, F = 640, 32, 128, 512, 4096, 1728
f32, bf16, u32, i32 = jnp.float32, jnp.bfloat16, jnp.uint32, jnp.int32
EPS = 1e-5


class Cfg:
    T = 8
    QV = ((240, 384), (448, 512), (576, 640))
    FV = 704
    WD = ((0, 1216, 0, 384), (1216, 512, 0, 384), (0, 1728, 384, 128), (0, 1728, 512, 128))
    NL = 2
    VG = 4
    NV = 40
    GATE_J = 8
    LAG = 6
    NC = 4


def _iota(shape, dim):
    return lax.broadcasted_iota(i32, shape, dim)


def _dot(a, b):
    return jnp.dot(a, b, preferred_element_type=f32)


def _dot_t(a, b):
    return lax.dot_general(a, b, (((1,), (1,)), ((), ())), preferred_element_type=f32)


def _ld(v):
    return pltpu.bitcast(v, bf16)


def _st(v):
    return pltpu.bitcast(v.astype(bf16), u32)


def _bslab(ref, x0, n, hf):
    return ref[x0:x0 + n, 16 * hf:16 * hf + 16, :].reshape(16 * n, 128)


def _words(v):
    return pltpu.bitcast(v, u32)


def _slab(ref, x0, n, hf):
    return _ld(ref[x0:x0 + n, 8 * hf:8 * hf + 8, :].reshape(8 * n, 128))


def _c1(p):
    return 16 * (p % 8) + (p // 8 + 15) % 16


def _c2(p):
    return 8 * (p % 16) + (p // 16 + 1) % 8


def _dup(x):
    w = lax.bitcast_convert_type(x.astype(bf16).astype(f32), u32)
    return w | (w >> 16)


def _dup_rows(x):
    return pltpu.bitcast(jnp.concatenate([x, x], axis=0).astype(bf16), u32)


def _stats(x):
    m = jnp.sum(x, axis=-1, keepdims=True) * (1.0 / M)
    ms = jnp.sum(x * x, axis=-1, keepdims=True) * (1.0 / M)
    return m, lax.rsqrt(jnp.maximum(ms - m * m, 0.0) + EPS)


def _subsum(v):
    v = v + pltpu.roll(v, 4, 0)
    v = v + pltpu.roll(v, 2, 0)
    return v + pltpu.roll(v, 1, 0)


def _silu(g):
    a = 0.5 * g
    return a + a * jnp.tanh(a)


def _sigmoid(r):
    return 0.5 + 0.5 * jnp.tanh(0.5 * r)


def _after(x, gate):
    return lax.bitcast_convert_type(lax.bitcast_convert_type(x, u32) | gate, f32)


def _spread(items, n):
    return [items[(len(items) * i) // n:(len(items) * (i + 1)) // n] for i in range(n)]


def make_kernel(cfg):
  T, QV, FV, WD, NC = cfg.T, cfg.QV, cfg.FV, cfg.WD, cfg.NC
  KC = S // NC
  FM = F - FV
  qv_rows = [m for lo_, hi_ in QV for m in range(lo_, hi_)]
  qv_pos = {m: i for i, m in enumerate(qv_rows)}

  def kernel(x_hbm, wr_hbm, wq_hbm, wuk_hbm, ckv_hbm, wuv_hbm, wg_hbm, wu_hbm, wo_hbm, wd_hbm,
             out_ref,
             xs, wrs, wqb, wuk, ckv, wuv, wg, wu, wo, wd, wq, wuv0, wo0, wdm,
             wukT, wukTf, ckvT, ckv2, wgT, wuT, qsum, wqf, gat, wuvT, wof, wgf, wuf, wdf,
             st_x, st_h, st_q, sems):
    step = pl.program_id(0)
    lo_f, hi_f = pl.ds(0, FV), pl.ds(FV, FM)
    srcs = [x_hbm, wr_hbm, wq_hbm, wuk_hbm, ckv_hbm, wuv_hbm, wo_hbm,
            wg_hbm.at[hi_f], wu_hbm.at[hi_f], wg_hbm.at[lo_f], wu_hbm.at[lo_f]]
    dsts = [xs, wrs, wqb, wuk, ckv, wuv, wo, wg.at[hi_f], wu.at[hi_f], wg.at[lo_f], wu.at[lo_f]]
    copies = [pltpu.make_async_copy(s, d, sems.at[i]) for i, (s, d) in enumerate(zip(srcs, dsts))]
    wd_copies = [pltpu.make_async_copy(wd_hbm.at[pl.ds(r0, n), pl.ds(c0, nc)],
                                       wd.at[pl.ds(r0, n), pl.ds(c0, nc)],
                                       sems.at[len(copies) + i])
                 for i, (r0, n, c0, nc) in enumerate(WD)]
    cp_x, cp_wr, cp_wq, cp_wuk, cp_ckv, cp_wuv, cp_wo, cp_wg1, cp_wu1, cp_wg0, cp_wu0 = copies

    sub = _iota((8, 128), 0)
    lane = _iota((8, 128), 1)
    l16 = lane % 16
    lo, hi, zero = jnp.uint32(0xFFFF), jnp.uint32(0xFFFF0000), jnp.uint32(0)
    ones_w = jnp.uint32(0x3F803F80)
    mask_rev = jnp.where(l16 == 15 - 2 * sub, lo, zero) | jnp.where(l16 == 14 - 2 * sub, hi, zero)
    mask_nat = jnp.where(l16 == 2 * sub, lo, zero) | jnp.where(l16 == 2 * sub + 1, hi, zero)
    ln16 = _iota((16, 128), 1)
    diag_nat = (ln16 % 16) == _iota((16, 128), 0)
    rev_idx = 7 - sub
    exp_idx = lane // 16
    col_idx = sub + 0 * lane
    zero_idx = 0 * lane

    zero_w = jnp.full((8, 128), step - 1, i32).astype(u32)

    def fence(v):
        return lax.bitcast_convert_type(jnp.broadcast_to(v, (8, 128)), u32) & zero_w

    def grid128():
        return _iota((128, 128), 0), _iota((128, 128), 1)

    def rev16(v):
        return jnp.concatenate([jnp.take_along_axis(v[8:16], rev_idx, axis=0),
                                jnp.take_along_axis(v[0:8], rev_idx, axis=0)], axis=0)

    def column(row_tile, first_lane):
        return jnp.take_along_axis(row_tile, col_idx + first_lane, axis=1)

    def q_partial(x, m_lo, m_hi, acc, with_sum):
        xw = _dup_rows(x)
        acc = list(acc)
        tiles = [t for t in range(m_lo // 8, m_hi // 8) if with_sum or 8 * t not in qv_pos]
        vgroups = [] if with_sum else [t for t in range(m_lo // 8, m_hi // 8) if 8 * t in qv_pos]
        chunks = [tiles[i:i + T] for i in range(0, len(tiles), T)]
        vparts = _spread(vgroups, len(chunks))
        if with_sum:
            sacc = [jnp.zeros((16, 128), f32), jnp.zeros((16, 128), f32)]
            one = pltpu.bitcast(mask_rev & ones_w, bf16)
        for ts, vs in zip(chunks, vparts):
            L = jnp.concatenate(
                [pltpu.bitcast(
                    jnp.take_along_axis(xw[:, 128 * (t // 16):128 * (t // 16 + 1)], exp_idx + 8 * (t % 16), axis=1)
                    & mask_rev, bf16) for t in ts], axis=1)
            for hf in range(2):
                W = jnp.concatenate([_slab(wq, 8 * t, 8, hf) for t in ts], axis=0)
                if with_sum:
                    o = _dot(jnp.concatenate([L, jnp.concatenate([one] * len(ts), axis=1)], axis=0), W)
                    acc[hf] = acc[hf] + o[0:16]
                    sacc[hf] = sacc[hf] + o[16:32]
                else:
                    acc[hf] = acc[hf] + _dot(L, W)
            for i in vs:
                g = (8 * i) // 128
                col = column(x[:, 128 * g:128 * (g + 1)], (8 * i) % 128)
                for s_ in range(0, 8, 2):
                    sp0 = jnp.broadcast_to(col[s_:s_ + 1], (16, 128))
                    sp1 = jnp.broadcast_to(col[s_ + 1:s_ + 2], (16, 128))
                    p0 = qv_pos[8 * i + s_]
                    for hf in range(2):
                        acc[2 + hf] = acc[2 + hf] + (sp0 * wqf[p0, 16 * hf:16 * hf + 16, :]
                                                     + sp1 * wqf[p0 + 1, 16 * hf:16 * hf + 16, :])
        if with_sum:
            for hf in range(2):
                qsum[hf] = sacc[hf]
        return acc

    def attention(x, qacc, first):
        mean, rs = _stats(x)
        m16 = jnp.concatenate([mean, mean], axis=0)
        rs16 = jnp.concatenate([rs, rs], axis=0)
        q_rev = [(qacc[hf] + rev16(qacc[2 + hf]) - m16 * qsum[hf]) * rs16 for hf in range(2)]
        q_qt = [q_rev[qt // 2][8 * (1 - qt % 2):8 * (2 - qt % 2)] for qt in range(4)]

        vtiles = [(3 - i // 32, i % 32) for i in range(cfg.NV)]
        if first:
            cp_wuk.wait()
            rr, cc = grid128()
            eye = (rr == cc).astype(bf16)
            for qt in range(4):
                for a0 in range(0, 32, 4):
                    W = wuk[16 * a0:16 * (a0 + 4), 8 * qt:8 * qt + 8, :].reshape(512, 128)
                    o = _dot_t(eye, W)
                    wukT[qt, :, 128 * a0:128 * (a0 + 4)] = _st(o)
                    for a in range(a0, a0 + 4):
                        if (qt, a) in vtiles:
                            wukTf[vtiles.index((qt, a))] = o[:, 128 * (a - a0):128 * (a - a0 + 1)]
        acc = [[jnp.zeros((8, 128), f32) for _ in range(4)] for _ in range(4)]

        def place(qt, a, v):
            j = a % 8
            v = pltpu.roll(v, j + 1, 1, stride=1, stride_axis=0)
            acc[qt][a // 8] = jnp.where((lane % 8) == j, v, acc[qt][a // 8])

        for qt in range(4):
            lhs = jnp.concatenate([q_qt[qt], q_qt[qt]], axis=0).astype(bf16)
            mt = [a for a in range(32) if first or (qt, a) not in vtiles]
            for i0 in range(0, len(mt), T):
                run_ = mt[i0:i0 + T]
                assert run_ == list(range(run_[0], run_[0] + len(run_)))
                o = _dot(lhs, _ld(wukT[qt, :, 128 * run_[0]:128 * (run_[-1] + 1)]))[0:8]
                for k, a in enumerate(run_):
                    place(qt, a, o[:, 128 * k:128 * (k + 1)])
        if not first:
            for qt in sorted({t[0] for t in vtiles}, reverse=True):
                q_nat = jnp.take_along_axis(q_qt[qt], rev_idx, axis=0)
                qc = jnp.concatenate([q_nat] * 16, axis=0).T
                mine = [i for i, t in enumerate(vtiles) if t[0] == qt]
                for i0 in range(0, len(mine), cfg.VG):
                    grp = mine[i0:i0 + cfg.VG]
                    zs = [None] * len(grp)
                    for dv in range(16):
                        qv = qc[8 * dv:8 * dv + 8]
                        for k, i in enumerate(grp):
                            t = wukTf[i, 8 * dv:8 * dv + 8, :] * qv
                            zs[k] = t if zs[k] is None else zs[k] + t
                    for k, i in enumerate(grp):
                        place(qt, vtiles[i][1], _subsum(zs[k]))
        qa = [(jnp.concatenate([jnp.take_along_axis(acc[qt][b], rev_idx, axis=0) for qt in range(4)], axis=0)
               * (D ** -0.5)).astype(bf16) for b in range(4)]

        if first:
            cp_ckv.wait()
            rr, cc = grid128()
            pm1 = (cc == _c1(rr)).astype(bf16)
            p2 = (rr == _c2(cc)).astype(bf16)
            for k0 in range(0, S, 1024):
                for b in range(4):
                    blk = ckv[k0:k0 + 1024, 128 * b:128 * (b + 1)]
                    ckvT[64 * b:64 * (b + 1), k0:k0 + 1024] = _st(_dot_t(pm1, blk))
                    ckv2[k0 // 2:k0 // 2 + 512, 128 * b:128 * (b + 1)] = _st(_dot(blk, p2))
        ms, ls, cxs, ps = [], [], [], []

        def scores(i):
            k0 = i * KC
            sc = _dot(qa[0], _ld(ckvT[0:64, k0:k0 + KC]))
            for b in range(1, 4):
                sc = sc + _dot(qa[b], _ld(ckvT[64 * b:64 * (b + 1), k0:k0 + KC]))
            return sc

        def soft(sc):
            mx = sc[:, 0:128]
            for j in range(1, KC // 128):
                mx = jnp.maximum(mx, sc[:, 128 * j:128 * (j + 1)])
            mx = jnp.max(mx, axis=1, keepdims=True)
            p = jnp.exp(sc - mx)
            den = p[:, 0:128]
            for j in range(1, KC // 128):
                den = den + p[:, 128 * j:128 * (j + 1)]
            ms.append(mx)
            ls.append(den)
            ps.append(p.astype(bf16))

        def ctx_all(i):
            o = _dot(ps[i], _ld(ckv2[i * KC // 2:(i + 1) * KC // 2, :]))
            cxs.append([o[:, 128 * b:128 * (b + 1)] for b in range(4)])

        def ctx_block(i, b):
            kq = KC // 4
            k0 = i * KC
            return functools.reduce(jnp.add, [
                _dot(ps[i][:, kq * u:kq * (u + 1)],
                     _ld(ckv2[(k0 + kq * u) // 2:(k0 + kq * (u + 1)) // 2, 128 * b:128 * (b + 1)]))
                for u in range(4)])

        NL = cfg.NL
        scs = [scores(0), scores(1)]
        soft(scs[0])
        for i in range(NC - NL):
            if i + 2 < NC:
                scs.append(scores(i + 2))
            ctx_all(i)
            soft(scs[i + 1])
        for i in range(NC - NL + 1, NC):
            soft(scs[i])
        tail = [[None] * 4 for _ in range(NL)]
        for b in range(4):
            for i in range(NL):
                tail[i][b] = ctx_block(NC - NL + i, b)
        cxs += tail
        mx = functools.reduce(jnp.maximum, ms)
        ws = [jnp.exp(m_ - mx) for m_ in ms]
        den = functools.reduce(jnp.add, [w_ * l_ for w_, l_ in zip(ws, ls)])
        inv = 1.0 / jnp.sum(den, axis=1, keepdims=True)
        cx = [functools.reduce(jnp.add, [w_ * c_[b] for w_, c_ in zip(ws, cxs)]) for b in range(4)]

        if first:
            cp_wuv.wait()
            for c0 in range(0, C, 16):
                wuv0[c0:c0 + 16] = _words(wuv[c0:c0 + 16, 0:16, :])
            for bq in range(64):
                b, q = bq // 16, bq % 16
                c0 = 128 * b + 64 * (q % 2) + (q // 2 + 1) % 8
                v = jnp.stack([_words(wuv[c0 + 8 * i, 16:32, :]) for i in range(8)], axis=0)
                gat[:, 8 * bq:8 * bq + 8, :] = jnp.swapaxes(v, 0, 1)
            rr, cc = grid128()
            eye = (rr == cc).astype(bf16)
            for r in range(8):
                for b in range(4):
                    w = gat[r, 128 * b:128 * (b + 1), :]
                    for e, bits in enumerate((w << 16, w & hi)):
                        t = lax.bitcast_convert_type(bits, f32).astype(bf16)
                        wuvT[2 * r + e, :, 128 * b:128 * (b + 1)] = _dot_t(eye, t)

        def value_half(hf):
            acc = jnp.zeros((16, 128), f32)
            for b in range(4):
                sb = cx[b][16 * hf:16 * hf + 16]
                for j0 in range(0, 16, T):
                    L = jnp.concatenate(
                        [jnp.where(diag_nat, pltpu.roll(sb, 16 - j, 1, stride=1, stride_axis=0), 0.0)
                         for j in range(j0, j0 + T)], axis=1).astype(bf16)
                    x0 = 8 * (16 * b + j0)
                    W = _bslab(wuv, x0, 8 * T, hf) if first else _ld(wuv0[x0:x0 + 8 * T].reshape(64 * T, 128))
                    acc = acc + _dot(L, W)
            return acc * inv[16 * hf:16 * hf + 16]

        ctx = [value_half(0)] + ([value_half(1)] if first else [])
        if first:
            cp_wo.wait()
            for r0 in range(0, 16 * D, 64):
                wof[r0:r0 + 64] = wo[16 * D + r0:16 * D + r0 + 64].astype(f32)
                wo0[r0 // 2:r0 // 2 + 32] = _words(wo[r0:r0 + 64])
        acc = jnp.zeros((16, M), f32)
        HC = 2
        for h0 in range(0, H if first else 16, HC):
            X = jnp.concatenate(
                [jnp.broadcast_to(ctx[h // 16][h % 16:h % 16 + 1], (16, 128)) for h in range(h0, h0 + HC)],
                axis=1).astype(bf16)
            W = wo[128 * h0:128 * (h0 + HC), :] if first else _ld(wo0[64 * h0:64 * (h0 + HC), :])
            acc = acc + _dot(X, W)
        out = acc[0:8]
        if not first:
            cxn = [cx[b][16:32] * inv[16:32] for b in range(4)]
            vacc = jnp.zeros((8, M), f32)
            gates = []
            for h in range(16):
                rows = [jnp.broadcast_to(cxn[b][h:h + 1], (8, 128)) for b in range(4)]
                if h >= cfg.LAG:
                    rows = [_after(r_, gates[h - cfg.LAG]) for r_ in rows]
                for j in range(0, 16, 2):
                    cols = []
                    for jj in (j, j + 1):
                        w = wuvT[h, 8 * jj:8 * jj + 8, :]
                        s_ = ((w[:, 0:128] * rows[0] + w[:, 128:256] * rows[1])
                              + (w[:, 256:384] * rows[2] + w[:, 384:512] * rows[3]))
                        cols.append(jnp.sum(s_, axis=1, keepdims=True))
                    if j == cfg.GATE_J:
                        gates.append(fence(cols[0]))
                    r0 = 128 * h + 8 * j
                    vacc = vacc + (cols[0] * wof[r0:r0 + 8, :] + cols[1] * wof[r0 + 8:r0 + 16, :])
            out = out + _subsum(vacc)
        return out

    def ffn_parts(x):
        X = jnp.concatenate([x, jnp.ones((8, M), f32)], axis=0).astype(bf16)
        mean, rs = _stats(x)
        xn = (x - mean) * rs
        wr = jnp.broadcast_to(wrs[...].reshape(1, M).astype(f32), (8, M))
        sig = _sigmoid(jnp.sum(xn * wr, axis=1, keepdims=True))
        return X, mean, rs, xn, sig

    def act(g, u, mean, rs):
        g = (g[0:8] - mean * g[8:16]) * rs
        u = (u[0:8] - mean * u[8:16]) * rs
        return _dup_rows(_silu(g) * u)

    def ffn_mxu_block(X, mean, rs, f0, n):
        return act(_dot(X, _ld(wgT[:, f0:f0 + n])), _dot(X, _ld(wuT[:, f0:f0 + n])), mean, rs)

    def wd_to_f32(c0, nc):
        for f0 in range(0, FV, 64):
            wdf[f0:f0 + 64, c0:c0 + nc] = wd[f0:f0 + 64, c0:c0 + nc].astype(f32)

    def wd_pack(r0, r1, c0, nc):
        for f0 in range(max(r0, FV), r1, 64):
            wdm[(f0 - FV) // 2:(f0 - FV) // 2 + 32, c0:c0 + nc] = _words(wd[f0:f0 + 64, c0:c0 + nc])

    @pl.when(step == 0)
    def _():
        for cp in copies + wd_copies:
            cp.start()
        cp_x.wait()
        cp_wr.wait()
        x = jnp.broadcast_to(xs[0].astype(f32), (8, M))
        cp_wq.wait()
        for m0 in range(0, M, 16):
            wq[m0:m0 + 16] = _words(wqb[m0:m0 + 16])
        for lo_, hi_ in QV:
            for m0 in range(lo_, hi_, 16):
                wqf[qv_pos[m0]:qv_pos[m0] + 16] = wqb[m0:m0 + 16].astype(f32)
        z16 = jnp.zeros((16, 128), f32)
        qacc = q_partial(x, 0, M, [z16] * 4, True)
        x = x + attention(x, qacc, True)
        X, mean, rs, xn, sig = ffn_parts(x)
        rr, cc = grid128()
        eye = (rr == cc).astype(bf16)
        for cp, src, dst in ((cp_wg1, wg, wgT), (cp_wu1, wu, wuT)):
            cp.wait()
            for g in range(5):
                for f0 in range(0, FM, 512):
                    n = min(512, FM - f0)
                    dst[64 * g:64 * (g + 1), f0:f0 + n] = _st(_dot_t(
                        eye, src[FV + f0:FV + f0 + n, 128 * g:128 * (g + 1)]))
        hm = ffn_mxu_block(X, mean, rs, 0, FM)
        cp_wg0.wait()
        gv = _dot_t(X, wg[0:FV, :])
        for f0 in range(0, FV, 64):
            wgf[f0:f0 + 64] = wg[f0:f0 + 64].astype(f32)
        cp_wu0.wait()
        hw = jnp.concatenate([act(gv, _dot_t(X, wu[0:FV, :]), mean, rs), hm], axis=1)
        for f0 in range(0, FV, 64):
            wuf[f0:f0 + 64] = wu[f0:f0 + 64].astype(f32)
        base = x + xn
        qacc = [z16] * 4
        ys = {}
        for cp, (r0, n, c0, nc) in zip(wd_copies[:-1], WD[:-1]):
            cp.wait()
            o = _dot(_ld(hw[:, r0:r0 + n]), wd[r0:r0 + n, c0:c0 + nc])[0:8]
            ys[c0] = o if c0 not in ys else ys[c0] + o
            if r0 + n == F:
                x2 = base[:, c0:c0 + nc] + ys[c0] * sig
                st_x[0, :, c0:c0 + nc] = x2
                xpad = jnp.concatenate([jnp.zeros((8, c0), f32), x2], axis=1) if c0 else x2
                qacc = q_partial(xpad, c0, c0 + nc, qacc, False)
            if r0 == 0 and n < F:
                wd_to_f32(c0, nc)
                wd_pack(r0, r0 + n, c0, nc)
        for i in range(4):
            st_q[i] = qacc[i]
        c0 = WD[-1][2]
        st_x[0, :, c0:M] = base[:, c0:M]
        st_x[1] = jnp.broadcast_to(sig, (8, M))
        st_h[...] = hw

    @pl.when(step == 1)
    def _():
        c0 = WD[-1][2]
        wd_copies[-1].wait()
        ylate = _dot(_ld(st_h[...]), wd[:, c0:M])[0:8]
        x = jnp.concatenate([st_x[0, :, 0:c0], st_x[0, :, c0:M] + ylate * st_x[1, :, c0:M]], axis=1)
        qacc = q_partial(x, c0, M, [st_q[i] for i in range(4)], False)
        for r0, n, cc0, nc in WD[1:]:
            if r0 == 0:
                wd_to_f32(cc0, nc)
            wd_pack(r0, r0 + n, cc0, nc)
        x = x + attention(x, qacc, False)
        X, mean, rs, xn, sig = ffn_parts(x)
        nb = FM // 128
        vparts = _spread(list(range(FV // 8)), nb)
        yv = jnp.zeros((8, M), f32)
        ym = None
        hs = []
        for bi in range(nb):
            hs.append(ffn_mxu_block(X, mean, rs, 128 * bi, 128))
            if bi >= 2:
                o = _dot(_ld(hs[bi - 2]), _ld(wdm[64 * (bi - 2):64 * (bi - 1), :]))
                ym = o if ym is None else ym + o
            for i in vparts[bi]:
                pg = wgf[8 * i:8 * i + 8, :] * xn
                pu = wuf[8 * i:8 * i + 8, :] * xn
                sg = (pg[:, 0:128] + pg[:, 128:256]) + (pg[:, 256:384] + pg[:, 384:512]) + pg[:, 512:640]
                su = (pu[:, 0:128] + pu[:, 128:256]) + (pu[:, 256:384] + pu[:, 384:512]) + pu[:, 512:640]
                hc = _silu(jnp.sum(sg, axis=1, keepdims=True)) * jnp.sum(su, axis=1, keepdims=True)
                yv = yv + hc * wdf[8 * i:8 * i + 8, :]
        for bi in range(nb - 2, nb):
            ym = ym + _dot(_ld(hs[bi]), _ld(wdm[64 * bi:64 * (bi + 1), :]))
        y = _subsum(yv) + ym[0:8]
        x = x + xn + y * sig
        out_ref[0] = x[0:1].astype(bf16)

  scratch = [
      pltpu.VMEM((1, 1, M), bf16), pltpu.VMEM((M,), bf16),
      pltpu.VMEM((M, H, D), bf16), pltpu.VMEM((C, H, D), bf16), pltpu.VMEM((S, C), bf16),
      pltpu.VMEM((C, H, D), bf16), pltpu.VMEM((F, M), bf16), pltpu.VMEM((F, M), bf16),
      pltpu.VMEM((H * D, M), bf16), pltpu.VMEM((F, M), bf16),
      pltpu.VMEM((M, H // 2, D), u32), pltpu.VMEM((C, 8, D), u32), pltpu.VMEM((8 * D, M), u32),
      pltpu.VMEM((FM // 2, M), u32),
      pltpu.VMEM((4, D // 2, 32 * 128), u32), pltpu.VMEM((cfg.NV, D, 128), f32),
      pltpu.VMEM((C // 2, S), u32), pltpu.VMEM((S // 2, C), u32),
      pltpu.VMEM((M // 2, FM), u32), pltpu.VMEM((M // 2, FM), u32),
      pltpu.VMEM((2, 16, 128), f32),
      pltpu.VMEM((len(qv_rows), H, D), f32),
      pltpu.VMEM((8, C, D), u32), pltpu.VMEM((16, D, C), f32), pltpu.VMEM((16 * D, M), f32),
      pltpu.VMEM((FV, M), f32), pltpu.VMEM((FV, M), f32), pltpu.VMEM((FV, M), f32),
      pltpu.VMEM((2, 8, M), f32), pltpu.VMEM((8, F), u32), pltpu.VMEM((4, 16, 128), f32),
      pltpu.SemaphoreType.DMA((11 + len(WD),)),
  ]
  return kernel, scratch


@jax.jit
def pallas_interleave_layers__compressed_kv_cla__moe_arch_mod__decode_kernel(
        A_x, A_c_kv, A_w_q, A_w_uk, A_w_uv, A_w_o, B_x, B_w_r, B_w_gate, B_w_up, B_w_down):
    interpret, cfg = False, Cfg
    del B_x
    hbm = pl.BlockSpec(memory_space=pl.ANY)
    kernel, scratch = make_kernel(cfg)
    return pl.pallas_call(
        kernel,
        out_shape=jax.ShapeDtypeStruct((1, 1, M), bf16),
        grid=(2,),
        in_specs=[hbm] * 10,
        out_specs=pl.BlockSpec((1, 1, M), lambda i: (0, 0, 0)),
        scratch_shapes=scratch,
        compiler_params=pltpu.CompilerParams(vmem_limit_bytes=120 * 1024 * 1024,
                                             dimension_semantics=("arbitrary",)),
        interpret=interpret,
        name="fused_decode",
    )(A_x, B_w_r, A_w_q, A_w_uk, A_c_kv.reshape(S, C), A_w_uv, B_w_gate.T, B_w_up.T,
      A_w_o.reshape(H * D, M), B_w_down)
```

```python
import functools
import jax
import jax.numpy as jnp
from jax import lax
from jax.experimental import pallas as pl
from jax.experimental.pallas import tpu as pltpu

M, H, D, C, S, F = 640, 32, 128, 512, 4096, 1728
f32, bf16, u32, i32 = jnp.float32, jnp.bfloat16, jnp.uint32, jnp.int32
EPS = 1e-5


class Cfg:
    T = 8
    QV = ((240, 384), (448, 512), (576, 640))
    FV = 704
    WD = ((0, 1216, 0, 384), (1216, 512, 0, 384), (0, 1728, 384, 128), (0, 1728, 512, 128))
    NL = 2
    KM = 0
    PERHEAD = True
    GATE_J = 14
    LAG = 3
    VG = 4
    NV = 40
    NC = 4


def _iota(shape, dim):
    return lax.broadcasted_iota(i32, shape, dim)


def _dot(a, b):
    return jnp.dot(a, b, preferred_element_type=f32)


def _dot_t(a, b):
    return lax.dot_general(a, b, (((1,), (1,)), ((), ())), preferred_element_type=f32)


def _ld(v):
    return pltpu.bitcast(v, bf16)


def _st(v):
    return pltpu.bitcast(v.astype(bf16), u32)


def _bslab(ref, x0, n, hf):
    return ref[x0:x0 + n, 16 * hf:16 * hf + 16, :].reshape(16 * n, 128)


def _words(v):
    return pltpu.bitcast(v, u32)


def _slab(ref, x0, n, hf):
    return _ld(ref[x0:x0 + n, 8 * hf:8 * hf + 8, :].reshape(8 * n, 128))


def _c1(p):
    return 16 * (p % 8) + (p // 8 + 15) % 16


def _c2(p):
    return 8 * (p % 16) + (p // 16 + 1) % 8


def _dup(x):
    w = lax.bitcast_convert_type(x.astype(bf16).astype(f32), u32)
    return w | (w >> 16)


def _dup_rows(x):
    return pltpu.bitcast(jnp.concatenate([x, x], axis=0).astype(bf16), u32)


def _stats(x):
    m = jnp.sum(x, axis=-1, keepdims=True) * (1.0 / M)
    ms = jnp.sum(x * x, axis=-1, keepdims=True) * (1.0 / M)
    return m, lax.rsqrt(jnp.maximum(ms - m * m, 0.0) + EPS)


def _subsum(v):
    v = v + pltpu.roll(v, 4, 0)
    v = v + pltpu.roll(v, 2, 0)
    return v + pltpu.roll(v, 1, 0)


def _silu(g):
    a = 0.5 * g
    return a + a * jnp.tanh(a)


def _sigmoid(r):
    return 0.5 + 0.5 * jnp.tanh(0.5 * r)


def _after(x, gate):
    return lax.bitcast_convert_type(lax.bitcast_convert_type(x, u32) | gate, f32)


def _spread(items, n):
    return [items[(len(items) * i) // n:(len(items) * (i + 1)) // n] for i in range(n)]


def make_kernel(cfg):
  T, QV, FV, WD, NC = cfg.T, cfg.QV, cfg.FV, cfg.WD, cfg.NC
  KC = S // NC
  FM = F - FV
  qv_rows = [m for lo_, hi_ in QV for m in range(lo_, hi_)]
  qv_pos = {m: i for i, m in enumerate(qv_rows)}

  def kernel(x_hbm, wr_hbm, wq_hbm, wuk_hbm, ckv_hbm, wuv_hbm, wg_hbm, wu_hbm, wo_hbm, wd_hbm,
             out_ref,
             xs, wrs, wqb, wuk, ckv, wuv, wg, wu, wo, wd, wq, wuv0, wo0, wdm,
             wukT, wukTf, ckvT, ckv2, wgT, wuT, qsum, wqf, gat, wuvT, wuvG, wof, wgf, wuf, wdf,
             st_x, st_h, st_q, sems):
    step = pl.program_id(0)
    lo_f, hi_f = pl.ds(0, FV), pl.ds(FV, FM)
    srcs = [wq_hbm, x_hbm, wr_hbm, wuk_hbm, ckv_hbm, wuv_hbm, wo_hbm,
            wg_hbm.at[hi_f], wu_hbm.at[hi_f], wg_hbm.at[lo_f], wu_hbm.at[lo_f]]
    dsts = [wqb, xs, wrs, wuk, ckv, wuv, wo, wg.at[hi_f], wu.at[hi_f], wg.at[lo_f], wu.at[lo_f]]
    copies = [pltpu.make_async_copy(s, d, sems.at[i]) for i, (s, d) in enumerate(zip(srcs, dsts))]
    wd_copies = [pltpu.make_async_copy(wd_hbm.at[pl.ds(r0, n), pl.ds(c0, nc)],
                                       wd.at[pl.ds(r0, n), pl.ds(c0, nc)],
                                       sems.at[len(copies) + i])
                 for i, (r0, n, c0, nc) in enumerate(WD)]
    cp_wq, cp_x, cp_wr, cp_wuk, cp_ckv, cp_wuv, cp_wo, cp_wg1, cp_wu1, cp_wg0, cp_wu0 = copies

    sub = _iota((8, 128), 0)
    lane = _iota((8, 128), 1)
    l16 = lane % 16
    lo, hi, zero = jnp.uint32(0xFFFF), jnp.uint32(0xFFFF0000), jnp.uint32(0)
    ones_w = jnp.uint32(0x3F803F80)
    mask_rev = jnp.where(l16 == 15 - 2 * sub, lo, zero) | jnp.where(l16 == 14 - 2 * sub, hi, zero)
    mask_nat = jnp.where(l16 == 2 * sub, lo, zero) | jnp.where(l16 == 2 * sub + 1, hi, zero)
    ln16 = _iota((16, 128), 1)
    diag_nat = (ln16 % 16) == _iota((16, 128), 0)
    rev_idx = 7 - sub
    exp_idx = lane // 16
    col_idx = sub + 0 * lane
    zero_idx = 0 * lane

    zero_w = jnp.full((8, 128), step - 1, i32).astype(u32)

    def fence(v):
        return lax.bitcast_convert_type(jnp.broadcast_to(v, (8, 128)), u32) & zero_w

    def grid128():
        return _iota((128, 128), 0), _iota((128, 128), 1)

    def rev16(v):
        return jnp.concatenate([jnp.take_along_axis(v[8:16], rev_idx, axis=0),
                                jnp.take_along_axis(v[0:8], rev_idx, axis=0)], axis=0)

    def column(row_tile, first_lane):
        return jnp.take_along_axis(row_tile, col_idx + first_lane, axis=1)

    def q_partial(x, m_lo, m_hi, acc, with_sum):
        xw = _dup_rows(x)
        acc = list(acc)
        tiles = [t for t in range(m_lo // 8, m_hi // 8) if with_sum or 8 * t not in qv_pos]
        vgroups = [] if with_sum else [t for t in range(m_lo // 8, m_hi // 8) if 8 * t in qv_pos]
        chunks = [tiles[i:i + T] for i in range(0, len(tiles), T)]
        vparts = _spread(vgroups, len(chunks))
        if with_sum:
            sacc = [jnp.zeros((16, 128), f32), jnp.zeros((16, 128), f32)]
            one = pltpu.bitcast(mask_rev & ones_w, bf16)
        for ts, vs in zip(chunks, vparts):
            L = jnp.concatenate(
                [pltpu.bitcast(
                    jnp.take_along_axis(xw[:, 128 * (t // 16):128 * (t // 16 + 1)], exp_idx + 8 * (t % 16), axis=1)
                    & mask_rev, bf16) for t in ts], axis=1)
            for hf in range(2):
                W = jnp.concatenate([_slab(wq, 8 * t, 8, hf) for t in ts], axis=0)
                if with_sum:
                    o = _dot(jnp.concatenate([L, jnp.concatenate([one] * len(ts), axis=1)], axis=0), W)
                    acc[hf] = acc[hf] + o[0:16]
                    sacc[hf] = sacc[hf] + o[16:32]
                else:
                    acc[hf] = acc[hf] + _dot(L, W)
            for i in vs:
                g = (8 * i) // 128
                col = column(x[:, 128 * g:128 * (g + 1)], (8 * i) % 128)
                for s_ in range(0, 8, 2):
                    sp0 = jnp.broadcast_to(col[s_:s_ + 1], (16, 128))
                    sp1 = jnp.broadcast_to(col[s_ + 1:s_ + 2], (16, 128))
                    p0 = qv_pos[8 * i + s_]
                    for hf in range(2):
                        acc[2 + hf] = acc[2 + hf] + (sp0 * wqf[p0, 16 * hf:16 * hf + 16, :]
                                                     + sp1 * wqf[p0 + 1, 16 * hf:16 * hf + 16, :])
        if with_sum:
            for hf in range(2):
                qsum[hf] = sacc[hf]
        return acc

    def attention(x, qacc, first):
        mean, rs = _stats(x)
        m16 = jnp.concatenate([mean, mean], axis=0)
        rs16 = jnp.concatenate([rs, rs], axis=0)
        q_rev = [(qacc[hf] + rev16(qacc[2 + hf]) - m16 * qsum[hf]) * rs16 for hf in range(2)]
        q_qt = [q_rev[qt // 2][8 * (1 - qt % 2):8 * (2 - qt % 2)] for qt in range(4)]

        vtiles = [(3 - i // 32, i % 32) for i in range(cfg.NV)]
        if first:
            cp_wuk.wait()
            rr, cc = grid128()
            eye = (rr == cc).astype(bf16)
            for qt in range(4):
                for a0 in range(0, 32, 4):
                    W = wuk[16 * a0:16 * (a0 + 4), 8 * qt:8 * qt + 8, :].reshape(512, 128)
                    o = _dot_t(eye, W)
                    wukT[qt, :, 128 * a0:128 * (a0 + 4)] = _st(o)
                    for a in range(a0, a0 + 4):
                        if (qt, a) in vtiles:
                            wukTf[vtiles.index((qt, a))] = o[:, 128 * (a - a0):128 * (a - a0 + 1)]
        acc = [[jnp.zeros((8, 128), f32) for _ in range(4)] for _ in range(4)]

        def place(qt, a, v):
            j = a % 8
            v = pltpu.roll(v, j + 1, 1, stride=1, stride_axis=0)
            acc[qt][a // 8] = jnp.where((lane % 8) == j, v, acc[qt][a // 8])

        for qt in range(4):
            lhs = jnp.concatenate([q_qt[qt], q_qt[qt]], axis=0).astype(bf16)
            mt = [a for a in range(32) if first or (qt, a) not in vtiles]
            for i0 in range(0, len(mt), T):
                run_ = mt[i0:i0 + T]
                assert run_ == list(range(run_[0], run_[0] + len(run_)))
                o = _dot(lhs, _ld(wukT[qt, :, 128 * run_[0]:128 * (run_[-1] + 1)]))[0:8]
                for k, a in enumerate(run_):
                    place(qt, a, o[:, 128 * k:128 * (k + 1)])
        if not first:
            for qt in sorted({t[0] for t in vtiles}, reverse=True):
                q_nat = jnp.take_along_axis(q_qt[qt], rev_idx, axis=0)
                qc = jnp.concatenate([q_nat] * 16, axis=0).T
                mine = [i for i, t in enumerate(vtiles) if t[0] == qt]
                for i0 in range(0, len(mine), cfg.VG):
                    grp = mine[i0:i0 + cfg.VG]
                    zs = [None] * len(grp)
                    for dv in range(16):
                        qv = qc[8 * dv:8 * dv + 8]
                        for k, i in enumerate(grp):
                            t = wukTf[i, 8 * dv:8 * dv + 8, :] * qv
                            zs[k] = t if zs[k] is None else zs[k] + t
                    for k, i in enumerate(grp):
                        place(qt, vtiles[i][1], _subsum(zs[k]))
        qa = [(jnp.concatenate([jnp.take_along_axis(acc[qt][b], rev_idx, axis=0) for qt in range(4)], axis=0)
               * (D ** -0.5)).astype(bf16) for b in range(4)]

        if first:
            cp_ckv.wait()
            rr, cc = grid128()
            pm1 = (cc == _c1(rr)).astype(bf16)
            p2 = (rr == _c2(cc)).astype(bf16)
            for k0 in range(0, S, 1024):
                for b in range(4):
                    blk = ckv[k0:k0 + 1024, 128 * b:128 * (b + 1)]
                    ckvT[64 * b:64 * (b + 1), k0:k0 + 1024] = _st(_dot_t(pm1, blk))
                    ckv2[k0 // 2:k0 // 2 + 512, 128 * b:128 * (b + 1)] = _st(_dot(blk, p2))
        ms, ls, cxs, ps = [], [], [], []

        def scores(i):
            k0 = i * KC
            sc = _dot(qa[0], _ld(ckvT[0:64, k0:k0 + KC]))
            for b in range(1, 4):
                sc = sc + _dot(qa[b], _ld(ckvT[64 * b:64 * (b + 1), k0:k0 + KC]))
            return sc

        def soft(sc):
            mx = sc[:, 0:128]
            for j in range(1, KC // 128):
                mx = jnp.maximum(mx, sc[:, 128 * j:128 * (j + 1)])
            mx = jnp.max(mx, axis=1, keepdims=True)
            p = jnp.exp(sc - mx)
            den = p[:, 0:128]
            for j in range(1, KC // 128):
                den = den + p[:, 128 * j:128 * (j + 1)]
            ms.append(mx)
            ls.append(den)
            ps.append(p.astype(bf16))

        def ctx_all(i):
            o = _dot(ps[i], _ld(ckv2[i * KC // 2:(i + 1) * KC // 2, :]))
            cxs.append([o[:, 128 * b:128 * (b + 1)] for b in range(4)])

        def ctx_block(i, b):
            kq = KC // 4
            k0 = i * KC
            return functools.reduce(jnp.add, [
                _dot(ps[i][:, kq * u:kq * (u + 1)],
                     _ld(ckv2[(k0 + kq * u) // 2:(k0 + kq * (u + 1)) // 2, 128 * b:128 * (b + 1)]))
                for u in range(4)])

        NL = cfg.NL
        scs = [scores(0), scores(1)]
        soft(scs[0])
        for i in range(NC - NL):
            if i + 2 < NC:
                scs.append(scores(i + 2))
            ctx_all(i)
            soft(scs[i + 1])
        for i in range(NC - NL + 1, NC):
            soft(scs[i])
        tail = [[None] * 4 for _ in range(NL)]
        for b in range(4):
            for i in range(NL):
                tail[i][b] = ctx_block(NC - NL + i, b)
        cxs += tail
        mx = functools.reduce(jnp.maximum, ms)
        ws = [jnp.exp(m_ - mx) for m_ in ms]
        den = functools.reduce(jnp.add, [w_ * l_ for w_, l_ in zip(ws, ls)])
        inv = 1.0 / jnp.sum(den, axis=1, keepdims=True)
        cx = [functools.reduce(jnp.add, [w_ * c_[b] for w_, c_ in zip(ws, cxs)]) for b in range(4)]

        if first:
            cp_wuv.wait()
            for c0 in range(0, C, 16):
                wuv0[c0:c0 + 16] = _words(wuv[c0:c0 + 16, 0:16, :])
            for bq in range(64):
                b, q = bq // 16, bq % 16
                c0 = 128 * b + 64 * (q % 2) + (q // 2 + 1) % 8
                v = jnp.stack([_words(wuv[c0 + 8 * i, 16:32, :]) for i in range(8)], axis=0)
                gat[:, 8 * bq:8 * bq + 8, :] = jnp.swapaxes(v, 0, 1)
            rr, cc = grid128()
            eye = (rr == cc).astype(bf16)
            for r in range(8):
                for b in range(4):
                    w = gat[r, 128 * b:128 * (b + 1), :]
                    for e, bits in enumerate((w << 16, w & hi)):
                        t = lax.bitcast_convert_type(bits, f32).astype(bf16)
                        if 2 * r + e < cfg.KM:
                            wuvG[2 * r + e, 64 * b:64 * (b + 1), :] = _words(t)
                        else:
                            wuvT[2 * r + e, :, 128 * b:128 * (b + 1)] = _dot_t(eye, t)

        def value_half(hf):
            acc = jnp.zeros((16, 128), f32)
            for b in range(4):
                sb = cx[b][16 * hf:16 * hf + 16]
                for j0 in range(0, 16, T):
                    L = jnp.concatenate(
                        [jnp.where(diag_nat, pltpu.roll(sb, 16 - j, 1, stride=1, stride_axis=0), 0.0)
                         for j in range(j0, j0 + T)], axis=1).astype(bf16)
                    x0 = 8 * (16 * b + j0)
                    W = _bslab(wuv, x0, 8 * T, hf) if first else _ld(wuv0[x0:x0 + 8 * T].reshape(64 * T, 128))
                    acc = acc + _dot(L, W)
            return acc * inv[16 * hf:16 * hf + 16]

        extra = []
        if not first:
            for k in range(cfg.KM):
                X = jnp.concatenate([jnp.broadcast_to(cx[b][16 + k:17 + k], (16, 128)) for b in range(4)],
                                    axis=1).astype(bf16)
                extra.append(_dot(X, _ld(wuvG[k])) * jnp.broadcast_to(inv[16 + k:17 + k], (16, 1)))
        ctx = [value_half(0)] + ([value_half(1)] if first else [])
        if first:
            cp_wo.wait()
            for r0 in range(cfg.KM * D, 16 * D, 64):
                wof[r0:r0 + 64] = wo[16 * D + r0:16 * D + r0 + 64].astype(f32)
            for r0 in range(0, (16 + cfg.KM) * D, 64):
                wo0[r0 // 2:r0 // 2 + 32] = _words(wo[r0:r0 + 64])
        acc = jnp.zeros((16, M), f32)
        for k, e_ in enumerate(extra):
            acc = acc + _dot(e_.astype(bf16), _ld(wo0[64 * (16 + k):64 * (17 + k), :]))
        HC = 2
        for h0 in range(0, H if first else 16, HC):
            X = jnp.concatenate(
                [jnp.broadcast_to(ctx[h // 16][h % 16:h % 16 + 1], (16, 128)) for h in range(h0, h0 + HC)],
                axis=1).astype(bf16)
            W = wo[128 * h0:128 * (h0 + HC), :] if first else _ld(wo0[64 * h0:64 * (h0 + HC), :])
            acc = acc + _dot(X, W)
        out = acc[0:8]
        if not first:
            vacc = None
            gates = []
            vheads = list(range(cfg.KM, 16))
            for n_, h in enumerate(vheads):
                rows = [jnp.broadcast_to(cx[b][16 + h:17 + h], (8, 128)) for b in range(4)]
                if not cfg.PERHEAD:
                    rows = [r_ * jnp.broadcast_to(inv[16 + h:17 + h], (8, 1)) for r_ in rows]
                if n_ >= cfg.LAG:
                    rows = [_after(r_, gates[n_ - cfg.LAG]) for r_ in rows]
                hacc = None if cfg.PERHEAD else vacc
                for j in range(0, 16, 2):
                    cols = []
                    for jj in (j, j + 1):
                        w = wuvT[h, 8 * jj:8 * jj + 8, :]
                        s_ = ((w[:, 0:128] * rows[0] + w[:, 128:256] * rows[1])
                              + (w[:, 256:384] * rows[2] + w[:, 384:512] * rows[3]))
                        cols.append(jnp.sum(s_, axis=1, keepdims=True))
                    if j == cfg.GATE_J:
                        gates.append(fence(cols[0]))
                    r0 = 128 * h + 8 * j
                    t = cols[0] * wof[r0:r0 + 8, :] + cols[1] * wof[r0 + 8:r0 + 16, :]
                    hacc = t if hacc is None else hacc + t
                if cfg.PERHEAD:
                    t = hacc * jnp.broadcast_to(inv[16 + h:17 + h], (8, 1))
                    vacc = t if vacc is None else vacc + t
                else:
                    vacc = hacc
            out = out + _subsum(vacc)
        return out

    def ffn_parts(x):
        X = jnp.concatenate([x, jnp.ones((8, M), f32)], axis=0).astype(bf16)
        mean, rs = _stats(x)
        xn = (x - mean) * rs
        wr = jnp.broadcast_to(wrs[...].reshape(1, M).astype(f32), (8, M))
        sig = _sigmoid(jnp.sum(xn * wr, axis=1, keepdims=True))
        return X, mean, rs, xn, sig

    def act(g, u, mean, rs):
        g = (g[0:8] - mean * g[8:16]) * rs
        u = (u[0:8] - mean * u[8:16]) * rs
        return _dup_rows(_silu(g) * u)

    def ffn_mxu_block(X, mean, rs, f0, n):
        return act(_dot(X, _ld(wgT[:, f0:f0 + n])), _dot(X, _ld(wuT[:, f0:f0 + n])), mean, rs)

    def wd_to_f32(c0, nc):
        for f0 in range(0, FV, 64):
            wdf[f0:f0 + 64, c0:c0 + nc] = wd[f0:f0 + 64, c0:c0 + nc].astype(f32)

    def wd_pack(r0, r1, c0, nc):
        for f0 in range(max(r0, FV), r1, 64):
            wdm[(f0 - FV) // 2:(f0 - FV) // 2 + 32, c0:c0 + nc] = _words(wd[f0:f0 + 64, c0:c0 + nc])

    @pl.when(step == 0)
    def _():
        for cp in copies + wd_copies:
            cp.start()
        if getattr(cfg, "FAST", False):
            for cp in copies + wd_copies[:-1]:
                cp.wait()
            st_x[0] = jnp.zeros((8, M), f32)
            return
        cp_x.wait()
        cp_wr.wait()
        x = jnp.broadcast_to(xs[0].astype(f32), (8, M))
        cp_wq.wait()
        for m0 in range(0, M, 16):
            wq[m0:m0 + 16] = _words(wqb[m0:m0 + 16])
        for lo_, hi_ in QV:
            for m0 in range(lo_, hi_, 16):
                wqf[qv_pos[m0]:qv_pos[m0] + 16] = wqb[m0:m0 + 16].astype(f32)
        z16 = jnp.zeros((16, 128), f32)
        qacc = q_partial(x, 0, M, [z16] * 4, True)
        x = x + attention(x, qacc, True)
        X, mean, rs, xn, sig = ffn_parts(x)
        rr, cc = grid128()
        eye = (rr == cc).astype(bf16)
        for cp, src, dst in ((cp_wg1, wg, wgT), (cp_wu1, wu, wuT)):
            cp.wait()
            for g in range(5):
                for f0 in range(0, FM, 512):
                    n = min(512, FM - f0)
                    dst[64 * g:64 * (g + 1), f0:f0 + n] = _st(_dot_t(
                        eye, src[FV + f0:FV + f0 + n, 128 * g:128 * (g + 1)]))
        hm = ffn_mxu_block(X, mean, rs, 0, FM)
        cp_wg0.wait()
        gv = _dot_t(X, wg[0:FV, :])
        for f0 in range(0, FV, 64):
            wgf[f0:f0 + 64] = wg[f0:f0 + 64].astype(f32) * 0.5
        cp_wu0.wait()
        hw = jnp.concatenate([act(gv, _dot_t(X, wu[0:FV, :]), mean, rs), hm], axis=1)
        for f0 in range(0, FV, 64):
            wuf[f0:f0 + 64] = wu[f0:f0 + 64].astype(f32)
        base = x + xn
        qacc = [z16] * 4
        ys = {}
        for cp, (r0, n, c0, nc) in zip(wd_copies[:-1], WD[:-1]):
            cp.wait()
            o = _dot(_ld(hw[:, r0:r0 + n]), wd[r0:r0 + n, c0:c0 + nc])[0:8]
            ys[c0] = o if c0 not in ys else ys[c0] + o
            if r0 + n == F:
                x2 = base[:, c0:c0 + nc] + ys[c0] * sig
                st_x[0, :, c0:c0 + nc] = x2
                xpad = jnp.concatenate([jnp.zeros((8, c0), f32), x2], axis=1) if c0 else x2
                if not (getattr(cfg, "SKIPQ", 0) and c0 >= cfg.SKIPQ - 1):
                    qacc = q_partial(xpad, c0, c0 + nc, qacc, False)
            if r0 == 0 and n < F:
                wd_to_f32(c0, nc)
                wd_pack(r0, r0 + n, c0, nc)
        for i in range(4):
            st_q[i] = qacc[i]
        c0 = WD[-1][2]
        st_x[0, :, c0:M] = base[:, c0:M]
        st_x[1] = jnp.broadcast_to(sig, (8, M))
        st_h[...] = hw

    @pl.when(step == 1)
    def _():
        c0 = WD[-1][2]
        wd_copies[-1].wait()
        if getattr(cfg, "NOL2", False):
            out_ref[0] = st_x[0, 0:1, :].astype(bf16)
            return
        ylate = _dot(_ld(st_h[...]), wd[:, c0:M])[0:8]
        x = jnp.concatenate([st_x[0, :, 0:c0], st_x[0, :, c0:M] + ylate * st_x[1, :, c0:M]], axis=1)
        qacc = q_partial(x, c0, M, [st_q[i] for i in range(4)], False)
        for r0, n, cc0, nc in WD[1:]:
            if r0 == 0:
                wd_to_f32(cc0, nc)
            wd_pack(r0, r0 + n, cc0, nc)
        x = x + attention(x, qacc, False)
        X, mean, rs, xn, sig = ffn_parts(x)
        nb = FM // 128
        hs = [ffn_mxu_block(X, mean, rs, 128 * bi, 128) for bi in range(nb)]
        ym = None
        for bi in range(nb):
            o = _dot(_ld(hs[bi]), _ld(wdm[64 * bi:64 * (bi + 1), :]))[0:8]
            ym = o if ym is None else ym + o
        yv = jnp.zeros((8, M), f32)
        for i in range(FV // 8):
            pg = wgf[8 * i:8 * i + 8, :] * xn
            pu = wuf[8 * i:8 * i + 8, :] * xn
            sg = (pg[:, 0:128] + pg[:, 128:256]) + (pg[:, 256:384] + pg[:, 384:512]) + pg[:, 512:640]
            su = (pu[:, 0:128] + pu[:, 128:256]) + (pu[:, 256:384] + pu[:, 384:512]) + pu[:, 512:640]
            a_ = jnp.sum(sg, axis=1, keepdims=True)
            hc = (a_ + a_ * jnp.tanh(a_)) * jnp.sum(su, axis=1, keepdims=True)
            yv = yv + hc * wdf[8 * i:8 * i + 8, :]
        y = _subsum(yv) + ym
        x = x + xn + y * sig
        out_ref[0] = x[0:1].astype(bf16)

  scratch = [
      pltpu.VMEM((1, 1, M), bf16), pltpu.VMEM((M,), bf16),
      pltpu.VMEM((M, H, D), bf16), pltpu.VMEM((C, H, D), bf16), pltpu.VMEM((S, C), bf16),
      pltpu.VMEM((C, H, D), bf16), pltpu.VMEM((F, M), bf16), pltpu.VMEM((F, M), bf16),
      pltpu.VMEM((H * D, M), bf16), pltpu.VMEM((F, M), bf16),
      pltpu.VMEM((M, H // 2, D), u32), pltpu.VMEM((C, 8, D), u32), pltpu.VMEM(((16 + cfg.KM) * D // 2, M), u32),
      pltpu.VMEM((FM // 2, M), u32),
      pltpu.VMEM((4, D // 2, 32 * 128), u32), pltpu.VMEM((cfg.NV, D, 128), f32),
      pltpu.VMEM((C // 2, S), u32), pltpu.VMEM((S // 2, C), u32),
      pltpu.VMEM((M // 2, FM), u32), pltpu.VMEM((M // 2, FM), u32),
      pltpu.VMEM((2, 16, 128), f32),
      pltpu.VMEM((len(qv_rows), H, D), f32),
      pltpu.VMEM((8, C, D), u32), pltpu.VMEM((16, D, C), f32), pltpu.VMEM((max(cfg.KM, 1), C // 2, D), u32),
      pltpu.VMEM((16 * D, M), f32),
      pltpu.VMEM((FV, M), f32), pltpu.VMEM((FV, M), f32), pltpu.VMEM((FV, M), f32),
      pltpu.VMEM((2, 8, M), f32), pltpu.VMEM((8, F), u32), pltpu.VMEM((4, 16, 128), f32),
      pltpu.SemaphoreType.DMA((11 + len(WD),)),
  ]
  return kernel, scratch


@jax.jit
def pallas_interleave_layers__compressed_kv_cla__moe_arch_mod__decode_kernel(
        A_x, A_c_kv, A_w_q, A_w_uk, A_w_uv, A_w_o, B_x, B_w_r, B_w_gate, B_w_up, B_w_down):
    interpret, cfg = False, Cfg
    del B_x
    hbm = pl.BlockSpec(memory_space=pl.ANY)
    kernel, scratch = make_kernel(cfg)
    return pl.pallas_call(
        kernel,
        out_shape=jax.ShapeDtypeStruct((1, 1, M), bf16),
        grid=(2,),
        in_specs=[hbm] * 10,
        out_specs=pl.BlockSpec((1, 1, M), lambda i: (0, 0, 0)),
        scratch_shapes=scratch,
        compiler_params=pltpu.CompilerParams(vmem_limit_bytes=120 * 1024 * 1024,
                                             dimension_semantics=("arbitrary",)),
        interpret=interpret,
        name="fused_decode",
    )(A_x, B_w_r, A_w_q, A_w_uk, A_c_kv.reshape(S, C), A_w_uv, B_w_gate.T, B_w_up.T,
      A_w_o.reshape(H * D, M), B_w_down)
```

```python
import functools

import jax
import jax.numpy as jnp
from jax import lax
from jax.experimental import pallas as pl
from jax.experimental.pallas import tpu as pltpu

M, H, D, C, S, F = 640, 32, 128, 512, 4096, 1728
f32, bf16, u32, i32 = jnp.float32, jnp.bfloat16, jnp.uint32, jnp.int32
EPS = 1e-5

T = 4
QV = ((160, 384), (416, 512), (576, 640))
NV = 41
FV = 704
FM = F - FV
FB = 256
NC = 4
NL = 2
KC = S // NC
LAG, GATE_J = 3, 14
WD = ((0, 1216, 0, 384), (1216, 512, 0, 384), (0, 1728, 384, 128), (0, 1728, 512, 128))

QV_ROWS = [m for lo, hi in QV for m in range(lo, hi)]
QV_POS = {m: i for i, m in enumerate(QV_ROWS)}
VTILES = [(3 - i // 32, i % 32) for i in range(NV)]


def _iota(shape, dim):
    return lax.broadcasted_iota(i32, shape, dim)


def _dot(a, b):
    return jnp.dot(a, b, preferred_element_type=f32)


def _dot_t(a, b):
    return lax.dot_general(a, b, (((1,), (1,)), ((), ())), preferred_element_type=f32)


def _rows(v):
    return pltpu.bitcast(v, bf16)


def _words(v):
    return pltpu.bitcast(v, u32)


def _c1(p):
    return 16 * (p % 8) + (p // 8 + 15) % 16


def _c2(p):
    return 8 * (p % 16) + (p // 16 + 1) % 8


def _dup_rows(x):
    return _words(jnp.concatenate([x, x], axis=0).astype(bf16))


def _stats(x):
    m = jnp.sum(x, axis=-1, keepdims=True) * (1.0 / M)
    ms = jnp.sum(x * x, axis=-1, keepdims=True) * (1.0 / M)
    return m, lax.rsqrt(jnp.maximum(ms - m * m, 0.0) + EPS)


def _subsum(v):
    v = v + pltpu.roll(v, 4, 0)
    v = v + pltpu.roll(v, 2, 0)
    return v + pltpu.roll(v, 1, 0)


def _half_silu(a):
    return a + a * jnp.tanh(a)


def _kernel(x_hbm, wr_hbm, wq_hbm, wuk_hbm, ckv_hbm, wuv_hbm, wg_hbm, wu_hbm, wo_hbm, wd_hbm,
            out_ref,
            xs, wrs, wqb, wuk, ckv, wuv, wg, wu, wo, wd,
            wq, wuv0, wo0, wdm, wukT, ckvT, ckv2, wgT, wuT,
            wqf, wukTf, wuvT, wof, wgf, wuf, wdf,
            gat, qsum, st_x, st_h, st_q, sems):
    step = pl.program_id(0)
    lo_f, hi_f = pl.ds(0, FV), pl.ds(FV, FM)
    srcs = [wq_hbm, x_hbm, wr_hbm, wuk_hbm, ckv_hbm, wuv_hbm, wo_hbm,
            wg_hbm.at[hi_f], wu_hbm.at[hi_f], wg_hbm.at[lo_f], wu_hbm.at[lo_f]]
    dsts = [wqb, xs, wrs, wuk, ckv, wuv, wo, wg.at[hi_f], wu.at[hi_f], wg.at[lo_f], wu.at[lo_f]]
    copies = [pltpu.make_async_copy(s, d, sems.at[i]) for i, (s, d) in enumerate(zip(srcs, dsts))]
    wd_copies = [pltpu.make_async_copy(wd_hbm.at[pl.ds(r0, n), pl.ds(c0, nc)],
                                       wd.at[pl.ds(r0, n), pl.ds(c0, nc)], sems.at[len(copies) + i])
                 for i, (r0, n, c0, nc) in enumerate(WD)]
    cp_wq, cp_x, cp_wr, cp_wuk, cp_ckv, cp_wuv, cp_wo, cp_wg1, cp_wu1, cp_wg0, cp_wu0 = copies

    sub = _iota((8, 128), 0)
    lane = _iota((8, 128), 1)
    l16 = lane % 16
    lo, hi, zero = jnp.uint32(0xFFFF), jnp.uint32(0xFFFF0000), jnp.uint32(0)
    mask_rev = jnp.where(l16 == 15 - 2 * sub, lo, zero) | jnp.where(l16 == 14 - 2 * sub, hi, zero)
    diag_nat = (_iota((16, 128), 1) % 16) == _iota((16, 128), 0)
    rev_idx = 7 - sub
    exp_idx = lane // 16
    col_idx = sub + 0 * lane
    zero_w = jnp.full((8, 128), step - 1, i32).astype(u32)

    def grid128():
        return _iota((128, 128), 0), _iota((128, 128), 1)

    def eye128():
        rr, cc = grid128()
        return (rr == cc).astype(bf16)

    def rev8(v):
        return jnp.take_along_axis(v, rev_idx, axis=0)

    def q_partial(x, m_lo, m_hi, acc, first):
        xw = _dup_rows(x)
        acc = list(acc)
        tiles = [t for t in range(m_lo // 8, m_hi // 8) if first or 8 * t not in QV_POS]
        vgroups = [] if first else [t for t in range(m_lo // 8, m_hi // 8) if 8 * t in QV_POS]
        chunks = [tiles[i:i + T] for i in range(0, len(tiles), T)]
        if first:
            sacc = [jnp.zeros((16, 128), f32), jnp.zeros((16, 128), f32)]
            one = _rows(mask_rev & jnp.uint32(0x3F803F80))
        for ci, ts in enumerate(chunks):
            lhs = jnp.concatenate(
                [_rows(jnp.take_along_axis(xw[:, 128 * (t // 16):128 * (t // 16 + 1)], exp_idx + 8 * (t % 16), axis=1)
                       & mask_rev) for t in ts], axis=1)
            for hf in range(2):
                w = jnp.concatenate([_rows(wq[8 * t:8 * t + 8, 8 * hf:8 * hf + 8, :].reshape(64, 128)) for t in ts],
                                    axis=0)
                if first:
                    o = _dot(jnp.concatenate([lhs, jnp.concatenate([one] * len(ts), axis=1)], axis=0), w)
                    acc[hf] = acc[hf] + o[0:16]
                    sacc[hf] = sacc[hf] + o[16:32]
                else:
                    acc[hf] = acc[hf] + _dot(lhs, w)
            for i in vgroups[len(vgroups) * ci // len(chunks):len(vgroups) * (ci + 1) // len(chunks)]:
                g = (8 * i) // 128
                col = jnp.take_along_axis(x[:, 128 * g:128 * (g + 1)], col_idx + (8 * i) % 128, axis=1)
                for s_ in range(0, 8, 2):
                    sp0 = jnp.broadcast_to(col[s_:s_ + 1], (16, 128))
                    sp1 = jnp.broadcast_to(col[s_ + 1:s_ + 2], (16, 128))
                    p0 = QV_POS[8 * i + s_]
                    for hf in range(2):
                        acc[2 + hf] = acc[2 + hf] + (sp0 * wqf[p0, 16 * hf:16 * hf + 16, :]
                                                     + sp1 * wqf[p0 + 1, 16 * hf:16 * hf + 16, :])
        if first:
            for hf in range(2):
                qsum[hf] = sacc[hf]
        return acc

    def absorb(q_rev, first):
        q_qt = [q_rev[qt // 2][8 * (1 - qt % 2):8 * (2 - qt % 2)] for qt in range(4)]
        if first:
            cp_wuk.wait()
            eye = eye128()
            for qt in range(4):
                for a0 in range(0, 32, 4):
                    o = _dot_t(eye, wuk[16 * a0:16 * (a0 + 4), 8 * qt:8 * qt + 8, :].reshape(512, 128))
                    wukT[qt, :, 128 * a0:128 * (a0 + 4)] = _words(o.astype(bf16))
                    for a in range(a0, a0 + 4):
                        if (qt, a) in VTILES:
                            wukTf[VTILES.index((qt, a))] = o[:, 128 * (a - a0):128 * (a - a0 + 1)]
        acc = [[jnp.zeros((8, 128), f32) for _ in range(4)] for _ in range(4)]

        def place(qt, a, v):
            j = a % 8
            v = pltpu.roll(v, j + 1, 1, stride=1, stride_axis=0)
            acc[qt][a // 8] = jnp.where((lane % 8) == j, v, acc[qt][a // 8])

        for qt in range(4):
            lhs = jnp.concatenate([q_qt[qt], q_qt[qt]], axis=0).astype(bf16)
            mine = [a for a in range(32) if first or (qt, a) not in VTILES]
            for i0 in range(0, len(mine), T):
                run = mine[i0:i0 + T]
                o = _dot(lhs, _rows(wukT[qt, :, 128 * run[0]:128 * (run[-1] + 1)]))[0:8]
                for k, a in enumerate(run):
                    place(qt, a, o[:, 128 * k:128 * (k + 1)])
        if not first:
            for qt in sorted({t[0] for t in VTILES}, reverse=True):
                qc = jnp.concatenate([rev8(q_qt[qt])] * 16, axis=0).T
                for i, (tq, a) in enumerate(VTILES):
                    if tq == qt:
                        z = None
                        for dv in range(16):
                            t = wukTf[i, 8 * dv:8 * dv + 8, :] * qc[8 * dv:8 * dv + 8]
                            z = t if z is None else z + t
                        place(qt, a, _subsum(z))
        return [(jnp.concatenate([rev8(acc[qt][b]) for qt in range(4)], axis=0) * (D ** -0.5)).astype(bf16)
                for b in range(4)]

    def attend(qa, first):
        if first:
            cp_ckv.wait()
            rr, cc = grid128()
            pm1 = (cc == _c1(rr)).astype(bf16)
            pm2 = (rr == _c2(cc)).astype(bf16)
            for k0 in range(0, S, 1024):
                for b in range(4):
                    blk = ckv[k0:k0 + 1024, 128 * b:128 * (b + 1)]
                    ckvT[64 * b:64 * (b + 1), k0:k0 + 1024] = _words(_dot_t(pm1, blk).astype(bf16))
                    ckv2[k0 // 2:k0 // 2 + 512, 128 * b:128 * (b + 1)] = _words(_dot(blk, pm2).astype(bf16))
        ms, ls, cxs, ps = [], [], [], []

        def scores(i):
            k0 = i * KC
            sc = _dot(qa[0], _rows(ckvT[0:64, k0:k0 + KC]))
            for b in range(1, 4):
                sc = sc + _dot(qa[b], _rows(ckvT[64 * b:64 * (b + 1), k0:k0 + KC]))
            return sc

        def soft(sc):
            mx = sc[:, 0:128]
            for j in range(1, KC // 128):
                mx = jnp.maximum(mx, sc[:, 128 * j:128 * (j + 1)])
            mx = jnp.max(mx, axis=1, keepdims=True)
            p = jnp.exp(sc - mx)
            den = p[:, 0:128]
            for j in range(1, KC // 128):
                den = den + p[:, 128 * j:128 * (j + 1)]
            ms.append(mx)
            ls.append(den)
            ps.append(p.astype(bf16))

        def ctx_all(i):
            o = _dot(ps[i], _rows(ckv2[i * KC // 2:(i + 1) * KC // 2, :]))
            cxs.append([o[:, 128 * b:128 * (b + 1)] for b in range(4)])

        def ctx_block(i, b):
            kq = KC // 4
            k0 = i * KC
            return functools.reduce(jnp.add, [
                _dot(ps[i][:, kq * u:kq * (u + 1)],
                     _rows(ckv2[(k0 + kq * u) // 2:(k0 + kq * (u + 1)) // 2, 128 * b:128 * (b + 1)]))
                for u in range(4)])

        scs = [scores(0), scores(1)]
        soft(scs[0])
        for i in range(NC - NL):
            if i + 2 < NC:
                scs.append(scores(i + 2))
            ctx_all(i)
            soft(scs[i + 1])
        for i in range(NC - NL + 1, NC):
            soft(scs[i])
        tail = [[None] * 4 for _ in range(NL)]
        for b in range(4):
            for i in range(NL):
                tail[i][b] = ctx_block(NC - NL + i, b)
        cxs += tail
        mx = functools.reduce(jnp.maximum, ms)
        ws = [jnp.exp(m_ - mx) for m_ in ms]
        den = functools.reduce(jnp.add, [w_ * l_ for w_, l_ in zip(ws, ls)])
        inv = 1.0 / jnp.sum(den, axis=1, keepdims=True)
        cx = [functools.reduce(jnp.add, [w_ * c_[b] for w_, c_ in zip(ws, cxs)]) for b in range(4)]
        return cx, inv

    def value_mxu(cx, inv, hf, first):
        acc = jnp.zeros((16, 128), f32)
        for b in range(4):
            sb = cx[b][16 * hf:16 * hf + 16]
            for j0 in range(0, 16, T):
                lhs = jnp.concatenate(
                    [jnp.where(diag_nat, pltpu.roll(sb, 16 - j, 1, stride=1, stride_axis=0), 0.0)
                     for j in range(j0, j0 + T)], axis=1).astype(bf16)
                x0 = 8 * (16 * b + j0)
                if first:
                    w = wuv[x0:x0 + 8 * T, 16 * hf:16 * hf + 16, :].reshape(128 * T, 128)
                else:
                    w = _rows(wuv0[x0:x0 + 8 * T].reshape(64 * T, 128))
                acc = acc + _dot(lhs, w)
        return acc * inv[16 * hf:16 * hf + 16]

    def out_mxu(ctx, first):
        acc = jnp.zeros((16, M), f32)
        hc = 4
        for h0 in range(0, 16 * len(ctx), hc):
            lhs = jnp.concatenate(
                [jnp.broadcast_to(ctx[h // 16][h % 16:h % 16 + 1], (16, 128)) for h in range(h0, h0 + hc)],
                axis=1).astype(bf16)
            w = wo[128 * h0:128 * (h0 + hc), :] if first else _rows(wo0[64 * h0:64 * (h0 + hc), :])
            acc = acc + _dot(lhs, w)
        return acc[0:8]

    def value_out_vpu(cx, inv):
        vacc = None
        gates = []
        for h in range(16):
            rows = [jnp.broadcast_to(cx[b][16 + h:17 + h], (8, 128)) for b in range(4)]
            if h >= LAG:
                rows = [lax.bitcast_convert_type(lax.bitcast_convert_type(r_, u32) | gates[h - LAG], f32)
                        for r_ in rows]
            hacc = None
            for j in range(0, 16, 2):
                cols = []
                for jj in (j, j + 1):
                    w = wuvT[h, 8 * jj:8 * jj + 8, :]
                    s_ = ((w[:, 0:128] * rows[0] + w[:, 128:256] * rows[1])
                          + (w[:, 256:384] * rows[2] + w[:, 384:512] * rows[3]))
                    cols.append(jnp.sum(s_, axis=1, keepdims=True))
                if j == GATE_J:
                    gates.append(lax.bitcast_convert_type(jnp.broadcast_to(cols[0], (8, 128)), u32) & zero_w)
                r0 = 128 * h + 8 * j
                t = cols[0] * wof[r0:r0 + 8, :] + cols[1] * wof[r0 + 8:r0 + 16, :]
                hacc = t if hacc is None else hacc + t
            t = hacc * jnp.broadcast_to(inv[16 + h:17 + h], (8, 1))
            vacc = t if vacc is None else vacc + t
        return _subsum(vacc)

    def normalise_q(qacc, x):
        mean, rs = _stats(x)
        m16 = jnp.concatenate([mean, mean], axis=0)
        rs16 = jnp.concatenate([rs, rs], axis=0)
        return [(qacc[hf] + jnp.concatenate([rev8(qacc[2 + hf][8:16]), rev8(qacc[2 + hf][0:8])], axis=0)
                 - m16 * qsum[hf]) * rs16 for hf in range(2)]

    def ffn_parts(x):
        lhs = jnp.concatenate([x, jnp.ones((8, M), f32)], axis=0).astype(bf16)
        mean, rs = _stats(x)
        xn = (x - mean) * rs
        wr = jnp.broadcast_to(wrs[...].reshape(1, M).astype(f32), (8, M))
        sig = 0.5 + 0.5 * jnp.tanh(0.5 * jnp.sum(xn * wr, axis=1, keepdims=True))
        return lhs, mean, rs, xn, sig

    def act(g, u, mean, rs):
        g = (g[0:8] - mean * g[8:16]) * rs
        u = (u[0:8] - mean * u[8:16]) * rs
        return _dup_rows(_half_silu(0.5 * g) * u)

    def ffn_mxu_block(lhs, mean, rs, f0, n):
        return act(_dot(lhs, _rows(wgT[:, f0:f0 + n])), _dot(lhs, _rows(wuT[:, f0:f0 + n])), mean, rs)

    def wd_relayout(r0, n, c0, nc):
        if r0 == 0:
            for f0 in range(0, FV, 64):
                wdf[f0:f0 + 64, c0:c0 + nc] = wd[f0:f0 + 64, c0:c0 + nc].astype(f32)
        for f0 in range(max(r0, FV), r0 + n, 64):
            wdm[(f0 - FV) // 2:(f0 - FV) // 2 + 32, c0:c0 + nc] = _words(wd[f0:f0 + 64, c0:c0 + nc])

    @pl.when(step == 0)
    def _():
        for cp in copies + wd_copies:
            cp.start()
        cp_x.wait()
        cp_wr.wait()
        x = jnp.broadcast_to(xs[0].astype(f32), (8, M))
        z16 = jnp.zeros((16, 128), f32)
        cp_wq.wait()
        for m0 in range(0, M, 16):
            wq[m0:m0 + 16] = _words(wqb[m0:m0 + 16])
        for m_lo, m_hi in QV:
            for m0 in range(m_lo, m_hi, 16):
                wqf[QV_POS[m0]:QV_POS[m0] + 16] = wqb[m0:m0 + 16].astype(f32)
        qacc = q_partial(x, 0, M, [z16] * 4, True)
        cx, inv = attend(absorb(normalise_q(qacc, x), True), True)
        cp_wuv.wait()
        for c0 in range(0, C, 16):
            wuv0[c0:c0 + 16] = _words(wuv[c0:c0 + 16, 0:16, :])
        for bq in range(64):
            b, q = bq // 16, bq % 16
            c0 = 128 * b + 64 * (q % 2) + (q // 2 + 1) % 8
            v = jnp.stack([_words(wuv[c0 + 8 * i, 16:32, :]) for i in range(8)], axis=0)
            gat[:, 8 * bq:8 * bq + 8, :] = jnp.swapaxes(v, 0, 1)
        eye = eye128()
        for r in range(8):
            for b in range(4):
                w = gat[r, 128 * b:128 * (b + 1), :]
                for e, bits in enumerate((w << 16, w & hi)):
                    t = lax.bitcast_convert_type(bits, f32).astype(bf16)
                    wuvT[2 * r + e, :, 128 * b:128 * (b + 1)] = _dot_t(eye, t)
        ctx = [value_mxu(cx, inv, 0, True), value_mxu(cx, inv, 1, True)]
        cp_wo.wait()
        for r0 in range(0, 16 * D, 64):
            wof[r0:r0 + 64] = wo[16 * D + r0:16 * D + r0 + 64].astype(f32)
            wo0[r0 // 2:r0 // 2 + 32] = _words(wo[r0:r0 + 64])
        x = x + out_mxu(ctx, True)
        lhs, mean, rs, xn, sig = ffn_parts(x)
        eye = eye128()
        for cp, src, dst in ((cp_wg1, wg, wgT), (cp_wu1, wu, wuT)):
            cp.wait()
            for g in range(5):
                for f0 in range(0, FM, 512):
                    dst[64 * g:64 * (g + 1), f0:f0 + 512] = _words(_dot_t(
                        eye, src[FV + f0:FV + f0 + 512, 128 * g:128 * (g + 1)]).astype(bf16))
        hm = ffn_mxu_block(lhs, mean, rs, 0, FM)
        cp_wg0.wait()
        gv = _dot_t(lhs, wg[0:FV, :])
        for f0 in range(0, FV, 64):
            wgf[f0:f0 + 64] = wg[f0:f0 + 64].astype(f32) * 0.5
        cp_wu0.wait()
        hw = jnp.concatenate([act(gv, _dot_t(lhs, wu[0:FV, :]), mean, rs), hm], axis=1)
        for f0 in range(0, FV, 64):
            wuf[f0:f0 + 64] = wu[f0:f0 + 64].astype(f32)
        base = x + xn
        qacc = [z16] * 4
        ys = {}
        for cp, (r0, n, c0, nc) in zip(wd_copies[:-1], WD[:-1]):
            cp.wait()
            o = _dot(_rows(hw[:, r0:r0 + n]), wd[r0:r0 + n, c0:c0 + nc])[0:8]
            ys[c0] = o if c0 not in ys else ys[c0] + o
            if r0 + n == F:
                x2 = base[:, c0:c0 + nc] + ys[c0] * sig
                st_x[0, :, c0:c0 + nc] = x2
                xpad = jnp.concatenate([jnp.zeros((8, c0), f32), x2], axis=1) if c0 else x2
                qacc = q_partial(xpad, c0, c0 + nc, qacc, False)
            wd_relayout(r0, n, c0, nc)
        for i in range(4):
            st_q[i] = qacc[i]
        c0 = WD[-1][2]
        st_x[0, :, c0:M] = base[:, c0:M]
        st_x[1] = jnp.broadcast_to(sig, (8, M))
        st_h[...] = hw

    @pl.when(step == 1)
    def _():
        c0 = WD[-1][2]
        wd_copies[-1].wait()
        ylate = _dot(_rows(st_h[...]), wd[:, c0:M])[0:8]
        x = jnp.concatenate([st_x[0, :, 0:c0], st_x[0, :, c0:M] + ylate * st_x[1, :, c0:M]], axis=1)
        qacc = q_partial(x, c0, M, [st_q[i] for i in range(4)], False)
        wd_relayout(*WD[-1])
        cx, inv = attend(absorb(normalise_q(qacc, x), False), False)
        x = x + (out_mxu([value_mxu(cx, inv, 0, False)], False) + value_out_vpu(cx, inv))
        lhs, mean, rs, xn, sig = ffn_parts(x)
        hs = [ffn_mxu_block(lhs, mean, rs, f0, FB) for f0 in range(0, FM, FB)]
        ym = functools.reduce(jnp.add, [_dot(_rows(h_), _rows(wdm[FB // 2 * i:FB // 2 * (i + 1), :]))[0:8]
                                        for i, h_ in enumerate(hs)])
        yv = jnp.zeros((8, M), f32)
        for i in range(FV // 8):
            pg = wgf[8 * i:8 * i + 8, :] * xn
            pu = wuf[8 * i:8 * i + 8, :] * xn
            sg = (pg[:, 0:128] + pg[:, 128:256]) + (pg[:, 256:384] + pg[:, 384:512]) + pg[:, 512:640]
            su = (pu[:, 0:128] + pu[:, 128:256]) + (pu[:, 256:384] + pu[:, 384:512]) + pu[:, 512:640]
            hc = _half_silu(jnp.sum(sg, axis=1, keepdims=True)) * jnp.sum(su, axis=1, keepdims=True)
            yv = yv + hc * wdf[8 * i:8 * i + 8, :]
        x = x + xn + (_subsum(yv) + ym) * sig
        out_ref[0] = x[0:1].astype(bf16)


_SCRATCH = [
    pltpu.VMEM((1, 1, M), bf16), pltpu.VMEM((M,), bf16),
    pltpu.VMEM((M, H, D), bf16), pltpu.VMEM((C, H, D), bf16), pltpu.VMEM((S, C), bf16),
    pltpu.VMEM((C, H, D), bf16), pltpu.VMEM((F, M), bf16), pltpu.VMEM((F, M), bf16),
    pltpu.VMEM((H * D, M), bf16), pltpu.VMEM((F, M), bf16),
    pltpu.VMEM((M, H // 2, D), u32), pltpu.VMEM((C, 8, D), u32), pltpu.VMEM((8 * D, M), u32),
    pltpu.VMEM((FM // 2, M), u32), pltpu.VMEM((4, D // 2, 32 * 128), u32),
    pltpu.VMEM((C // 2, S), u32), pltpu.VMEM((S // 2, C), u32),
    pltpu.VMEM((M // 2, FM), u32), pltpu.VMEM((M // 2, FM), u32),
    pltpu.VMEM((len(QV_ROWS), H, D), f32), pltpu.VMEM((NV, D, 128), f32), pltpu.VMEM((16, D, C), f32),
    pltpu.VMEM((16 * D, M), f32), pltpu.VMEM((FV, M), f32), pltpu.VMEM((FV, M), f32), pltpu.VMEM((FV, M), f32),
    pltpu.VMEM((8, C, D), u32), pltpu.VMEM((2, 16, 128), f32),
    pltpu.VMEM((2, 8, M), f32), pltpu.VMEM((8, F), u32), pltpu.VMEM((4, 16, 128), f32),
    pltpu.SemaphoreType.DMA((11 + len(WD),)),
]


@jax.jit
def pallas_interleave_layers__compressed_kv_cla__moe_arch_mod__decode_kernel(
        A_x, A_c_kv, A_w_q, A_w_uk, A_w_uv, A_w_o, B_x, B_w_r, B_w_gate, B_w_up, B_w_down):
    del B_x
    return pl.pallas_call(
        _kernel,
        out_shape=jax.ShapeDtypeStruct((1, 1, M), bf16),
        grid=(2,),
        in_specs=[pl.BlockSpec(memory_space=pl.ANY)] * 10,
        out_specs=pl.BlockSpec((1, 1, M), lambda i: (0, 0, 0)),
        scratch_shapes=_SCRATCH,
        compiler_params=pltpu.CompilerParams(vmem_limit_bytes=120 * 1024 * 1024,
                                             dimension_semantics=("arbitrary",)),
        name="fused_decode",
    )(A_x, B_w_r, A_w_q, A_w_uk, A_c_kv.reshape(S, C), A_w_uv, B_w_gate.T, B_w_up.T,
      A_w_o.reshape(H * D, M), B_w_down)
```

```python
import functools

import jax
import jax.numpy as jnp
from jax import lax
from jax.experimental import pallas as pl
from jax.experimental.pallas import tpu as pltpu

M, H, D, C, S, F = 640, 32, 128, 512, 4096, 1728
f32, bf16, u32, i32 = jnp.float32, jnp.bfloat16, jnp.uint32, jnp.int32
EPS = 1e-5

T = 4
QV = ((160, 384), (416, 512), (576, 640))
NV = 40
FV = 704
FM = F - FV
FB = 128
NC = 4
NL = 2
KC = S // NC
HEAD_LAG = 3
FFN_EVERY, FFN_LAG = 10, 20
WD = ((0, 1216, 0, 384), (1216, 512, 0, 384), (0, 1728, 384, 128), (0, 1728, 512, 128))

QV_ROWS = [m for lo, hi in QV for m in range(lo, hi)]
QV_POS = {m: i for i, m in enumerate(QV_ROWS)}
VTILES = [(3 - i // 32, i % 32) for i in range(NV)]


def _iota(shape, dim):
    return lax.broadcasted_iota(i32, shape, dim)


def _dot(a, b):
    return jnp.dot(a, b, preferred_element_type=f32)


def _dot_t(a, b):
    return lax.dot_general(a, b, (((1,), (1,)), ((), ())), preferred_element_type=f32)


def _rows(v):
    return pltpu.bitcast(v, bf16)


def _words(v):
    return pltpu.bitcast(v, u32)


def _c1(p):
    return 16 * (p % 8) + (p // 8 + 15) % 16


def _c2(p):
    return 8 * (p % 16) + (p // 16 + 1) % 8


def _dup_rows(x):
    return _words(jnp.concatenate([x, x], axis=0).astype(bf16))


def _stats(x):
    m = jnp.sum(x, axis=-1, keepdims=True) * (1.0 / M)
    ms = jnp.sum(x * x, axis=-1, keepdims=True) * (1.0 / M)
    return m, lax.rsqrt(jnp.maximum(ms - m * m, 0.0) + EPS)


def _subsum(v):
    v = v + pltpu.roll(v, 4, 0)
    v = v + pltpu.roll(v, 2, 0)
    return v + pltpu.roll(v, 1, 0)


def _half_silu(a):
    return a + a * jnp.tanh(a)


def _kernel(x_hbm, wr_hbm, wq_hbm, wuk_hbm, ckv_hbm, wuv_hbm, wg_hbm, wu_hbm, wo_hbm, wd_hbm,
            out_ref,
            xs, wrs, wqb, wuk, ckv, wuv, wg, wu, wo, wd,
            wq, wuv0, wo0, wdm, wukT, ckvT, ckv2, wgT, wuT,
            wqf, wukTf, wuvT, wof, wgf, wuf, wdf,
            gat, qsum, st_x, st_h, st_q, sems):
    step = pl.program_id(0)
    lo_f, hi_f = pl.ds(0, FV), pl.ds(FV, FM)
    srcs = [wq_hbm, x_hbm, wr_hbm, wuk_hbm, ckv_hbm, wuv_hbm, wo_hbm,
            wg_hbm.at[hi_f], wu_hbm.at[hi_f], wg_hbm.at[lo_f], wu_hbm.at[lo_f]]
    dsts = [wqb, xs, wrs, wuk, ckv, wuv, wo, wg.at[hi_f], wu.at[hi_f], wg.at[lo_f], wu.at[lo_f]]
    copies = [pltpu.make_async_copy(s, d, sems.at[i]) for i, (s, d) in enumerate(zip(srcs, dsts))]
    wd_copies = [pltpu.make_async_copy(wd_hbm.at[pl.ds(r0, n), pl.ds(c0, nc)],
                                       wd.at[pl.ds(r0, n), pl.ds(c0, nc)], sems.at[len(copies) + i])
                 for i, (r0, n, c0, nc) in enumerate(WD)]
    cp_wq, cp_x, cp_wr, cp_wuk, cp_ckv, cp_wuv, cp_wo, cp_wg1, cp_wu1, cp_wg0, cp_wu0 = copies

    sub = _iota((8, 128), 0)
    lane = _iota((8, 128), 1)
    l16 = lane % 16
    lo, hi, zero = jnp.uint32(0xFFFF), jnp.uint32(0xFFFF0000), jnp.uint32(0)
    mask_rev = jnp.where(l16 == 15 - 2 * sub, lo, zero) | jnp.where(l16 == 14 - 2 * sub, hi, zero)
    diag_nat = (_iota((16, 128), 1) % 16) == _iota((16, 128), 0)
    rev_idx = 7 - sub
    exp_idx = lane // 16
    col_idx = sub + 0 * lane
    zero_w = jnp.full((8, 128), step - 1, i32).astype(u32)

    def grid128():
        return _iota((128, 128), 0), _iota((128, 128), 1)

    def eye128():
        rr, cc = grid128()
        return (rr == cc).astype(bf16)

    def rev8(v):
        return jnp.take_along_axis(v, rev_idx, axis=0)

    def q_partial(x, m_lo, m_hi, acc, first):
        xw = _dup_rows(x)
        acc = list(acc)
        tiles = [t for t in range(m_lo // 8, m_hi // 8) if first or 8 * t not in QV_POS]
        vgroups = [] if first else [t for t in range(m_lo // 8, m_hi // 8) if 8 * t in QV_POS]
        chunks = [tiles[i:i + T] for i in range(0, len(tiles), T)]
        if first:
            sacc = [jnp.zeros((16, 128), f32), jnp.zeros((16, 128), f32)]
            one = _rows(mask_rev & jnp.uint32(0x3F803F80))
        for ci, ts in enumerate(chunks):
            lhs = jnp.concatenate(
                [_rows(jnp.take_along_axis(xw[:, 128 * (t // 16):128 * (t // 16 + 1)], exp_idx + 8 * (t % 16), axis=1)
                       & mask_rev) for t in ts], axis=1)
            for hf in range(2):
                w = jnp.concatenate([_rows(wq[8 * t:8 * t + 8, 8 * hf:8 * hf + 8, :].reshape(64, 128)) for t in ts],
                                    axis=0)
                if first:
                    o = _dot(jnp.concatenate([lhs, jnp.concatenate([one] * len(ts), axis=1)], axis=0), w)
                    acc[hf] = acc[hf] + o[0:16]
                    sacc[hf] = sacc[hf] + o[16:32]
                else:
                    acc[hf] = acc[hf] + _dot(lhs, w)
            for i in vgroups[len(vgroups) * ci // len(chunks):len(vgroups) * (ci + 1) // len(chunks)]:
                g = (8 * i) // 128
                col = jnp.take_along_axis(x[:, 128 * g:128 * (g + 1)], col_idx + (8 * i) % 128, axis=1)
                for s_ in range(0, 8, 2):
                    sp0 = jnp.broadcast_to(col[s_:s_ + 1], (16, 128))
                    sp1 = jnp.broadcast_to(col[s_ + 1:s_ + 2], (16, 128))
                    p0 = QV_POS[8 * i + s_]
                    for hf in range(2):
                        acc[2 + hf] = acc[2 + hf] + (sp0 * wqf[p0, 16 * hf:16 * hf + 16, :]
                                                     + sp1 * wqf[p0 + 1, 16 * hf:16 * hf + 16, :])
        if first:
            for hf in range(2):
                qsum[hf] = sacc[hf]
        return acc

    def absorb(q_rev, first):
        q_qt = [q_rev[qt // 2][8 * (1 - qt % 2):8 * (2 - qt % 2)] for qt in range(4)]
        if first:
            cp_wuk.wait()
            eye = eye128()
            for qt in range(4):
                for a0 in range(0, 32, 4):
                    o = _dot_t(eye, wuk[16 * a0:16 * (a0 + 4), 8 * qt:8 * qt + 8, :].reshape(512, 128))
                    wukT[qt, :, 128 * a0:128 * (a0 + 4)] = _words(o.astype(bf16))
                    for a in range(a0, a0 + 4):
                        if (qt, a) in VTILES:
                            wukTf[VTILES.index((qt, a))] = o[:, 128 * (a - a0):128 * (a - a0 + 1)]
        acc = [[jnp.zeros((8, 128), f32) for _ in range(4)] for _ in range(4)]

        def place(qt, a, v):
            j = a % 8
            v = pltpu.roll(v, j + 1, 1, stride=1, stride_axis=0)
            acc[qt][a // 8] = jnp.where((lane % 8) == j, v, acc[qt][a // 8])

        for qt in range(4):
            lhs = jnp.concatenate([q_qt[qt], q_qt[qt]], axis=0).astype(bf16)
            mine = [a for a in range(32) if first or (qt, a) not in VTILES]
            for i0 in range(0, len(mine), T):
                run = mine[i0:i0 + T]
                o = _dot(lhs, _rows(wukT[qt, :, 128 * run[0]:128 * (run[-1] + 1)]))[0:8]
                for k, a in enumerate(run):
                    place(qt, a, o[:, 128 * k:128 * (k + 1)])
        if not first:
            for qt in sorted({t[0] for t in VTILES}, reverse=True):
                qc = jnp.concatenate([rev8(q_qt[qt])] * 16, axis=0).T
                for i, (tq, a) in enumerate(VTILES):
                    if tq == qt:
                        z = None
                        for dv in range(16):
                            t = wukTf[i, 8 * dv:8 * dv + 8, :] * qc[8 * dv:8 * dv + 8]
                            z = t if z is None else z + t
                        place(qt, a, _subsum(z))
        return [(jnp.concatenate([rev8(acc[qt][b]) for qt in range(4)], axis=0) * (D ** -0.5)).astype(bf16)
                for b in range(4)]

    def attend(qa, first):
        if first:
            cp_ckv.wait()
            rr, cc = grid128()
            pm1 = (cc == _c1(rr)).astype(bf16)
            pm2 = (rr == _c2(cc)).astype(bf16)
            for k0 in range(0, S, 1024):
                for b in range(4):
                    blk = ckv[k0:k0 + 1024, 128 * b:128 * (b + 1)]
                    ckvT[64 * b:64 * (b + 1), k0:k0 + 1024] = _words(_dot_t(pm1, blk).astype(bf16))
                    ckv2[k0 // 2:k0 // 2 + 512, 128 * b:128 * (b + 1)] = _words(_dot(blk, pm2).astype(bf16))
        ms, ls, cxs, ps = [], [], [], []

        def scores(i):
            k0 = i * KC
            sc = _dot(qa[0], _rows(ckvT[0:64, k0:k0 + KC]))
            for b in range(1, 4):
                sc = sc + _dot(qa[b], _rows(ckvT[64 * b:64 * (b + 1), k0:k0 + KC]))
            return sc

        def soft(sc):
            mx = sc[:, 0:128]
            for j in range(1, KC // 128):
                mx = jnp.maximum(mx, sc[:, 128 * j:128 * (j + 1)])
            mx = jnp.max(mx, axis=1, keepdims=True)
            p = jnp.exp(sc - mx)
            den = p[:, 0:128]
            for j in range(1, KC // 128):
                den = den + p[:, 128 * j:128 * (j + 1)]
            ms.append(mx)
            ls.append(den)
            ps.append(p.astype(bf16))

        def ctx_all(i):
            o = _dot(ps[i], _rows(ckv2[i * KC // 2:(i + 1) * KC // 2, :]))
            cxs.append([o[:, 128 * b:128 * (b + 1)] for b in range(4)])

        def ctx_block(i, b):
            kq = KC // 4
            k0 = i * KC
            return functools.reduce(jnp.add, [
                _dot(ps[i][:, kq * u:kq * (u + 1)],
                     _rows(ckv2[(k0 + kq * u) // 2:(k0 + kq * (u + 1)) // 2, 128 * b:128 * (b + 1)]))
                for u in range(4)])

        scs = [scores(0), scores(1)]
        soft(scs[0])
        for i in range(NC - NL):
            if i + 2 < NC:
                scs.append(scores(i + 2))
            ctx_all(i)
            soft(scs[i + 1])
        for i in range(NC - NL + 1, NC):
            soft(scs[i])
        tail = [[None] * 4 for _ in range(NL)]
        for b in range(4):
            for i in range(NL):
                tail[i][b] = ctx_block(NC - NL + i, b)
        cxs += tail
        mx = functools.reduce(jnp.maximum, ms)
        ws = [jnp.exp(m_ - mx) for m_ in ms]
        den = functools.reduce(jnp.add, [w_ * l_ for w_, l_ in zip(ws, ls)])
        inv = 1.0 / jnp.sum(den, axis=1, keepdims=True)
        cx = [functools.reduce(jnp.add, [w_ * c_[b] for w_, c_ in zip(ws, cxs)]) for b in range(4)]
        return cx, inv

    def value_mxu(cx, inv, hf, first):
        acc = jnp.zeros((16, 128), f32)
        for b in range(4):
            sb = cx[b][16 * hf:16 * hf + 16]
            for j0 in range(0, 16, T):
                lhs = jnp.concatenate(
                    [jnp.where(diag_nat, pltpu.roll(sb, 16 - j, 1, stride=1, stride_axis=0), 0.0)
                     for j in range(j0, j0 + T)], axis=1).astype(bf16)
                x0 = 8 * (16 * b + j0)
                if first:
                    w = wuv[x0:x0 + 8 * T, 16 * hf:16 * hf + 16, :].reshape(128 * T, 128)
                else:
                    w = _rows(wuv0[x0:x0 + 8 * T].reshape(64 * T, 128))
                acc = acc + _dot(lhs, w)
        return acc * inv[16 * hf:16 * hf + 16]

    def out_mxu(ctx, first):
        acc = jnp.zeros((16, M), f32)
        hc = 4
        for h0 in range(0, 16 * len(ctx), hc):
            lhs = jnp.concatenate(
                [jnp.broadcast_to(ctx[h // 16][h % 16:h % 16 + 1], (16, 128)) for h in range(h0, h0 + hc)],
                axis=1).astype(bf16)
            w = wo[128 * h0:128 * (h0 + hc), :] if first else _rows(wo0[64 * h0:64 * (h0 + hc), :])
            acc = acc + _dot(lhs, w)
        return acc[0:8]

    def after(x, gate):
        return lax.bitcast_convert_type(lax.bitcast_convert_type(x, u32) | gate, f32)

    def fence(v):
        return lax.bitcast_convert_type(jnp.broadcast_to(v, (8, 128)), u32) & zero_w

    def value_out_vpu(cx, inv):
        vacc = None
        gates = []
        for n, h in enumerate(range(15, -1, -1)):
            rows = [jnp.broadcast_to(cx[b][16 + h:17 + h], (8, 128)) for b in range(4)]
            if n >= HEAD_LAG:
                rows = [after(r_, gates[n - HEAD_LAG]) for r_ in rows]
            hacc = None
            for j in range(0, 16, 2):
                cols = []
                for jj in (j, j + 1):
                    w = wuvT[h, 8 * jj:8 * jj + 8, :]
                    s_ = functools.reduce(jnp.add, [w[:, 128 * b:128 * (b + 1)] * rows[b] for b in range(4)])
                    cols.append(jnp.sum(s_, axis=1, keepdims=True))
                r0 = 128 * h + 8 * j
                t = cols[0] * wof[r0:r0 + 8, :] + cols[1] * wof[r0 + 8:r0 + 16, :]
                hacc = t if hacc is None else hacc + t
            gates.append(fence(cols[0]))
            t = hacc * jnp.broadcast_to(inv[16 + h:17 + h], (8, 1))
            vacc = t if vacc is None else vacc + t
        return _subsum(vacc)

    def normalise_q(qacc, x):
        mean, rs = _stats(x)
        m16 = jnp.concatenate([mean, mean], axis=0)
        rs16 = jnp.concatenate([rs, rs], axis=0)
        return [(qacc[hf] + jnp.concatenate([rev8(qacc[2 + hf][8:16]), rev8(qacc[2 + hf][0:8])], axis=0)
                 - m16 * qsum[hf]) * rs16 for hf in range(2)]

    def ffn_parts(x):
        lhs = jnp.concatenate([x, jnp.ones((8, M), f32)], axis=0).astype(bf16)
        mean, rs = _stats(x)
        xn = (x - mean) * rs
        wr = jnp.broadcast_to(wrs[...].reshape(1, M).astype(f32), (8, M))
        sig = 0.5 + 0.5 * jnp.tanh(0.5 * jnp.sum(xn * wr, axis=1, keepdims=True))
        return lhs, mean, rs, xn, sig

    def act(g, u, mean, rs):
        g = (g[0:8] - mean * g[8:16]) * rs
        u = (u[0:8] - mean * u[8:16]) * rs
        return _dup_rows(_half_silu(0.5 * g) * u)

    def ffn_mxu_block(lhs, mean, rs, f0, n):
        return act(_dot(lhs, _rows(wgT[:, f0:f0 + n])), _dot(lhs, _rows(wuT[:, f0:f0 + n])), mean, rs)

    def wd_relayout(r0, n, c0, nc):
        if r0 == 0:
            for f0 in range(0, FV, 64):
                wdf[f0:f0 + 64, c0:c0 + nc] = wd[f0:f0 + 64, c0:c0 + nc].astype(f32)
        for f0 in range(max(r0, FV), r0 + n, 64):
            wdm[(f0 - FV) // 2:(f0 - FV) // 2 + 32, c0:c0 + nc] = _words(wd[f0:f0 + 64, c0:c0 + nc])

    @pl.when(step == 0)
    def _():
        for cp in copies + wd_copies:
            cp.start()
        cp_x.wait()
        cp_wr.wait()
        x = jnp.broadcast_to(xs[0].astype(f32), (8, M))
        z16 = jnp.zeros((16, 128), f32)
        cp_wq.wait()
        for m0 in range(0, M, 16):
            wq[m0:m0 + 16] = _words(wqb[m0:m0 + 16])
        for m_lo, m_hi in QV:
            for m0 in range(m_lo, m_hi, 16):
                wqf[QV_POS[m0]:QV_POS[m0] + 16] = wqb[m0:m0 + 16].astype(f32)
        qacc = q_partial(x, 0, M, [z16] * 4, True)
        cx, inv = attend(absorb(normalise_q(qacc, x), True), True)
        cp_wuv.wait()
        for c0 in range(0, C, 16):
            wuv0[c0:c0 + 16] = _words(wuv[c0:c0 + 16, 0:16, :])
        for bq in range(64):
            b, q = bq // 16, bq % 16
            c0 = 128 * b + 64 * (q % 2) + (q // 2 + 1) % 8
            v = jnp.stack([_words(wuv[c0 + 8 * i, 16:32, :]) for i in range(8)], axis=0)
            gat[:, 8 * bq:8 * bq + 8, :] = jnp.swapaxes(v, 0, 1)
        eye = eye128()
        for r in range(8):
            for b in range(4):
                w = gat[r, 128 * b:128 * (b + 1), :]
                for e, bits in enumerate((w << 16, w & hi)):
                    t = lax.bitcast_convert_type(bits, f32).astype(bf16)
                    wuvT[2 * r + e, :, 128 * b:128 * (b + 1)] = _dot_t(eye, t)
        ctx = [value_mxu(cx, inv, 0, True), value_mxu(cx, inv, 1, True)]
        cp_wo.wait()
        for r0 in range(0, 16 * D, 64):
            wof[r0:r0 + 64] = wo[16 * D + r0:16 * D + r0 + 64].astype(f32)
            wo0[r0 // 2:r0 // 2 + 32] = _words(wo[r0:r0 + 64])
        x = x + out_mxu(ctx, True)
        lhs, mean, rs, xn, sig = ffn_parts(x)
        eye = eye128()
        for cp, src, dst in ((cp_wg1, wg, wgT), (cp_wu1, wu, wuT)):
            cp.wait()
            for g in range(5):
                for f0 in range(0, FM, 512):
                    dst[64 * g:64 * (g + 1), f0:f0 + 512] = _words(_dot_t(
                        eye, src[FV + f0:FV + f0 + 512, 128 * g:128 * (g + 1)]).astype(bf16))
        hm = ffn_mxu_block(lhs, mean, rs, 0, FM)
        cp_wg0.wait()
        gv = _dot_t(lhs, wg[0:FV, :])
        for f0 in range(0, FV, 64):
            wgf[f0:f0 + 64] = wg[f0:f0 + 64].astype(f32) * 0.5
        cp_wu0.wait()
        hw = jnp.concatenate([act(gv, _dot_t(lhs, wu[0:FV, :]), mean, rs), hm], axis=1)
        for f0 in range(0, FV, 64):
            wuf[f0:f0 + 64] = wu[f0:f0 + 64].astype(f32)
        base = x + xn
        qacc = [z16] * 4
        ys = {}
        for cp, (r0, n, c0, nc) in zip(wd_copies[:-1], WD[:-1]):
            cp.wait()
            o = _dot(_rows(hw[:, r0:r0 + n]), wd[r0:r0 + n, c0:c0 + nc])[0:8]
            ys[c0] = o if c0 not in ys else ys[c0] + o
            if r0 + n == F:
                x2 = base[:, c0:c0 + nc] + ys[c0] * sig
                st_x[0, :, c0:c0 + nc] = x2
                xpad = jnp.concatenate([jnp.zeros((8, c0), f32), x2], axis=1) if c0 else x2
                qacc = q_partial(xpad, c0, c0 + nc, qacc, False)
            wd_relayout(r0, n, c0, nc)
        for i in range(4):
            st_q[i] = qacc[i]
        c0 = WD[-1][2]
        st_x[0, :, c0:M] = base[:, c0:M]
        st_x[1] = jnp.broadcast_to(sig, (8, M))
        st_h[...] = hw

    @pl.when(step == 1)
    def _():
        c0 = WD[-1][2]
        wd_copies[-1].wait()
        ylate = _dot(_rows(st_h[...]), wd[:, c0:M])[0:8]
        x = jnp.concatenate([st_x[0, :, 0:c0], st_x[0, :, c0:M] + ylate * st_x[1, :, c0:M]], axis=1)
        qacc = q_partial(x, c0, M, [st_q[i] for i in range(4)], False)
        wd_relayout(*WD[-1])
        cx, inv = attend(absorb(normalise_q(qacc, x), False), False)
        x = x + (out_mxu([value_mxu(cx, inv, 0, False)], False) + value_out_vpu(cx, inv))
        lhs, mean, rs, xn, sig = ffn_parts(x)
        hs = [ffn_mxu_block(lhs, mean, rs, f0, FB) for f0 in range(0, FM, FB)]
        ym = functools.reduce(jnp.add, [_dot(_rows(h_), _rows(wdm[FB // 2 * i:FB // 2 * (i + 1), :]))[0:8]
                                        for i, h_ in enumerate(hs)])
        yv = jnp.zeros((8, M), f32)
        xg = xn
        gates = []
        for i in range(FV // 8):
            if i % FFN_EVERY == 0 and i >= FFN_LAG:
                xg = jnp.concatenate([after(xn[:, 128 * k:128 * (k + 1)], gates[i - FFN_LAG]) for k in range(5)], axis=1)
            pg = wgf[8 * i:8 * i + 8, :] * xg
            pu = wuf[8 * i:8 * i + 8, :] * xg
            sg = (pg[:, 0:128] + pg[:, 128:256]) + (pg[:, 256:384] + pg[:, 384:512]) + pg[:, 512:640]
            su = (pu[:, 0:128] + pu[:, 128:256]) + (pu[:, 256:384] + pu[:, 384:512]) + pu[:, 512:640]
            hc = _half_silu(jnp.sum(sg, axis=1, keepdims=True)) * jnp.sum(su, axis=1, keepdims=True)
            gates.append(fence(hc))
            yv = yv + hc * wdf[8 * i:8 * i + 8, :]
        x = x + xn + (_subsum(yv) + ym) * sig
        out_ref[0] = x[0:1].astype(bf16)


_SCRATCH = [
    pltpu.VMEM((1, 1, M), bf16), pltpu.VMEM((M,), bf16),
    pltpu.VMEM((M, H, D), bf16), pltpu.VMEM((C, H, D), bf16), pltpu.VMEM((S, C), bf16),
    pltpu.VMEM((C, H, D), bf16), pltpu.VMEM((F, M), bf16), pltpu.VMEM((F, M), bf16),
    pltpu.VMEM((H * D, M), bf16), pltpu.VMEM((F, M), bf16),
    pltpu.VMEM((M, H // 2, D), u32), pltpu.VMEM((C, 8, D), u32), pltpu.VMEM((8 * D, M), u32),
    pltpu.VMEM((FM // 2, M), u32), pltpu.VMEM((4, D // 2, 32 * 128), u32),
    pltpu.VMEM((C // 2, S), u32), pltpu.VMEM((S // 2, C), u32),
    pltpu.VMEM((M // 2, FM), u32), pltpu.VMEM((M // 2, FM), u32),
    pltpu.VMEM((len(QV_ROWS), H, D), f32), pltpu.VMEM((NV, D, 128), f32), pltpu.VMEM((16, D, C), f32),
    pltpu.VMEM((16 * D, M), f32), pltpu.VMEM((FV, M), f32), pltpu.VMEM((FV, M), f32), pltpu.VMEM((FV, M), f32),
    pltpu.VMEM((8, C, D), u32), pltpu.VMEM((2, 16, 128), f32),
    pltpu.VMEM((2, 8, M), f32), pltpu.VMEM((8, F), u32), pltpu.VMEM((4, 16, 128), f32),
    pltpu.SemaphoreType.DMA((11 + len(WD),)),
]


@jax.jit
def pallas_interleave_layers__compressed_kv_cla__moe_arch_mod__decode_kernel(
        A_x, A_c_kv, A_w_q, A_w_uk, A_w_uv, A_w_o, B_x, B_w_r, B_w_gate, B_w_up, B_w_down):
    del B_x
    return pl.pallas_call(
        _kernel,
        out_shape=jax.ShapeDtypeStruct((1, 1, M), bf16),
        grid=(2,),
        in_specs=[pl.BlockSpec(memory_space=pl.ANY)] * 10,
        out_specs=pl.BlockSpec((1, 1, M), lambda i: (0, 0, 0)),
        scratch_shapes=_SCRATCH,
        compiler_params=pltpu.CompilerParams(vmem_limit_bytes=120 * 1024 * 1024,
                                             dimension_semantics=("arbitrary",)),
        name="fused_decode",
    )(A_x, B_w_r, A_w_q, A_w_uk, A_c_kv.reshape(S, C), A_w_uv, B_w_gate.T, B_w_up.T,
      A_w_o.reshape(H * D, M), B_w_down)
```

```python
import functools

import jax
import jax.numpy as jnp
from jax import lax
from jax.experimental import pallas as pl
from jax.experimental.pallas import tpu as pltpu

M, H, D, C, S, F = 640, 32, 128, 512, 4096, 1728
f32, bf16, u32, i32 = jnp.float32, jnp.bfloat16, jnp.uint32, jnp.int32
EPS = 1e-5

T = 4
QV = ((160, 384), (416, 512), (576, 640))
NV = 40
FV = 704
FM = F - FV
FB = 128
NC = 4
NL = 2
KC = S // NC
HEAD_LAG = 3
FFN_EVERY, FFN_LAG = 10, 20
WD = ((0, 1216, 0, 384), (1216, 512, 0, 384), (0, 1728, 384, 128), (0, 1728, 512, 128))

QV_ROWS = [m for lo, hi in QV for m in range(lo, hi)]
QV_POS = {m: i for i, m in enumerate(QV_ROWS)}
VTILES = [(3 - i // 32, i % 32) for i in range(NV)]


def _iota(shape, dim):
    return lax.broadcasted_iota(i32, shape, dim)


def _dot(a, b):
    return jnp.dot(a, b, preferred_element_type=f32)


def _dot_t(a, b):
    return lax.dot_general(a, b, (((1,), (1,)), ((), ())), preferred_element_type=f32)


def _rows(v):
    return pltpu.bitcast(v, bf16)


def _words(v):
    return pltpu.bitcast(v, u32)


def _c1(p):
    return 16 * (p % 8) + (p // 8 + 15) % 16


def _c2(p):
    return 8 * (p % 16) + (p // 16 + 1) % 8


def _dup_rows(x):
    return _words(jnp.concatenate([x, x], axis=0).astype(bf16))


def _stats(x, centred):
    m = jnp.sum(x, axis=-1, keepdims=True) * (1.0 / M)
    if centred:
        xc = x - m
        var = jnp.sum(xc * xc, axis=-1, keepdims=True) * (1.0 / M)
    else:
        var = jnp.maximum(jnp.sum(x * x, axis=-1, keepdims=True) * (1.0 / M) - m * m, 0.0)
    return m, lax.rsqrt(var + EPS)


def _subsum(v):
    v = v + pltpu.roll(v, 4, 0)
    v = v + pltpu.roll(v, 2, 0)
    return v + pltpu.roll(v, 1, 0)


def _half_silu(a):
    return a + a * jnp.tanh(a)


def _kernel(x_hbm, wr_hbm, wq_hbm, wuk_hbm, ckv_hbm, wuv_hbm, wg_hbm, wu_hbm, wo_hbm, wd_hbm,
            out_ref,
            xs, wrs, wqb, wuk, ckv, wuv, wg, wu, wo, wd,
            wq, wuv0, wo0, wdm, wukT, ckvT, ckv2, wgT, wuT,
            wqf, wukTf, wuvT, wof, wgf, wuf, wdf,
            gat, qsum, st_x, st_h, st_q, sems):
    step = pl.program_id(0)
    lo_f, hi_f = pl.ds(0, FV), pl.ds(FV, FM)
    srcs = [wq_hbm, x_hbm, wr_hbm, wuk_hbm, ckv_hbm, wuv_hbm, wo_hbm,
            wg_hbm.at[hi_f], wu_hbm.at[hi_f], wg_hbm.at[lo_f], wu_hbm.at[lo_f]]
    dsts = [wqb, xs, wrs, wuk, ckv, wuv, wo, wg.at[hi_f], wu.at[hi_f], wg.at[lo_f], wu.at[lo_f]]
    copies = [pltpu.make_async_copy(s, d, sems.at[i]) for i, (s, d) in enumerate(zip(srcs, dsts))]
    wd_copies = [pltpu.make_async_copy(wd_hbm.at[pl.ds(r0, n), pl.ds(c0, nc)],
                                       wd.at[pl.ds(r0, n), pl.ds(c0, nc)], sems.at[len(copies) + i])
                 for i, (r0, n, c0, nc) in enumerate(WD)]
    cp_wq, cp_x, cp_wr, cp_wuk, cp_ckv, cp_wuv, cp_wo, cp_wg1, cp_wu1, cp_wg0, cp_wu0 = copies

    sub = _iota((8, 128), 0)
    lane = _iota((8, 128), 1)
    l16 = lane % 16
    lo, hi, zero = jnp.uint32(0xFFFF), jnp.uint32(0xFFFF0000), jnp.uint32(0)
    mask_rev = jnp.where(l16 == 15 - 2 * sub, lo, zero) | jnp.where(l16 == 14 - 2 * sub, hi, zero)
    diag_nat = (_iota((16, 128), 1) % 16) == _iota((16, 128), 0)
    rev_idx = 7 - sub
    exp_idx = lane // 16
    col_idx = sub + 0 * lane
    zero_w = jnp.full((8, 128), step - 1, i32).astype(u32)

    def grid128():
        return _iota((128, 128), 0), _iota((128, 128), 1)

    def eye128():
        rr, cc = grid128()
        return (rr == cc).astype(bf16)

    def rev8(v):
        return jnp.take_along_axis(v, rev_idx, axis=0)

    def q_partial(x, m_lo, m_hi, acc, first):
        xw = _dup_rows(x)
        acc = list(acc)
        tiles = [t for t in range(m_lo // 8, m_hi // 8) if first or 8 * t not in QV_POS]
        vgroups = [] if first else [t for t in range(m_lo // 8, m_hi // 8) if 8 * t in QV_POS]
        chunks = [tiles[i:i + T] for i in range(0, len(tiles), T)]
        if first:
            sacc = [jnp.zeros((16, 128), f32), jnp.zeros((16, 128), f32)]
            one = _rows(mask_rev & jnp.uint32(0x3F803F80))
        for ci, ts in enumerate(chunks):
            lhs = jnp.concatenate(
                [_rows(jnp.take_along_axis(xw[:, 128 * (t // 16):128 * (t // 16 + 1)], exp_idx + 8 * (t % 16), axis=1)
                       & mask_rev) for t in ts], axis=1)
            for hf in range(2):
                w = jnp.concatenate([_rows(wq[8 * t:8 * t + 8, 8 * hf:8 * hf + 8, :].reshape(64, 128)) for t in ts],
                                    axis=0)
                if first:
                    o = _dot(jnp.concatenate([lhs, jnp.concatenate([one] * len(ts), axis=1)], axis=0), w)
                    acc[hf] = acc[hf] + o[0:16]
                    sacc[hf] = sacc[hf] + o[16:32]
                else:
                    acc[hf] = acc[hf] + _dot(lhs, w)
            for i in vgroups[len(vgroups) * ci // len(chunks):len(vgroups) * (ci + 1) // len(chunks)]:
                g = (8 * i) // 128
                col = jnp.take_along_axis(x[:, 128 * g:128 * (g + 1)], col_idx + (8 * i) % 128, axis=1)
                for s_ in range(0, 8, 2):
                    sp0 = jnp.broadcast_to(col[s_:s_ + 1], (16, 128))
                    sp1 = jnp.broadcast_to(col[s_ + 1:s_ + 2], (16, 128))
                    p0 = QV_POS[8 * i + s_]
                    for hf in range(2):
                        acc[2 + hf] = acc[2 + hf] + (sp0 * wqf[p0, 16 * hf:16 * hf + 16, :]
                                                     + sp1 * wqf[p0 + 1, 16 * hf:16 * hf + 16, :])
        if first:
            for hf in range(2):
                qsum[hf] = sacc[hf]
        return acc

    def absorb(q_rev, first):
        q_qt = [q_rev[qt // 2][8 * (1 - qt % 2):8 * (2 - qt % 2)] for qt in range(4)]
        if first:
            cp_wuk.wait()
            eye = eye128()
            for qt in range(4):
                for a0 in range(0, 32, 4):
                    o = _dot_t(eye, wuk[16 * a0:16 * (a0 + 4), 8 * qt:8 * qt + 8, :].reshape(512, 128))
                    wukT[qt, :, 128 * a0:128 * (a0 + 4)] = _words(o.astype(bf16))
                    for a in range(a0, a0 + 4):
                        if (qt, a) in VTILES:
                            wukTf[VTILES.index((qt, a))] = o[:, 128 * (a - a0):128 * (a - a0 + 1)]
        acc = [[jnp.zeros((8, 128), f32) for _ in range(4)] for _ in range(4)]

        def place(qt, a, v):
            j = a % 8
            v = pltpu.roll(v, j + 1, 1, stride=1, stride_axis=0)
            acc[qt][a // 8] = jnp.where((lane % 8) == j, v, acc[qt][a // 8])

        for qt in range(4):
            lhs = jnp.concatenate([q_qt[qt], q_qt[qt]], axis=0).astype(bf16)
            mine = [a for a in range(32) if first or (qt, a) not in VTILES]
            for i0 in range(0, len(mine), T):
                run = mine[i0:i0 + T]
                o = _dot(lhs, _rows(wukT[qt, :, 128 * run[0]:128 * (run[-1] + 1)]))[0:8]
                for k, a in enumerate(run):
                    place(qt, a, o[:, 128 * k:128 * (k + 1)])
        if not first:
            for qt in sorted({t[0] for t in VTILES}, reverse=True):
                qc = jnp.concatenate([rev8(q_qt[qt])] * 16, axis=0).T
                for i, (tq, a) in enumerate(VTILES):
                    if tq == qt:
                        z = None
                        for dv in range(16):
                            t = wukTf[i, 8 * dv:8 * dv + 8, :] * qc[8 * dv:8 * dv + 8]
                            z = t if z is None else z + t
                        place(qt, a, _subsum(z))
        return [(jnp.concatenate([rev8(acc[qt][b]) for qt in range(4)], axis=0) * (D ** -0.5)).astype(bf16)
                for b in range(4)]

    def attend(qa, first):
        if first:
            cp_ckv.wait()
            rr, cc = grid128()
            pm1 = (cc == _c1(rr)).astype(bf16)
            pm2 = (rr == _c2(cc)).astype(bf16)
            for k0 in range(0, S, 1024):
                for b in range(4):
                    blk = ckv[k0:k0 + 1024, 128 * b:128 * (b + 1)]
                    ckvT[64 * b:64 * (b + 1), k0:k0 + 1024] = _words(_dot_t(pm1, blk).astype(bf16))
                    ckv2[k0 // 2:k0 // 2 + 512, 128 * b:128 * (b + 1)] = _words(_dot(blk, pm2).astype(bf16))
        ms, ls, cxs, ps = [], [], [], []

        def scores(i):
            k0 = i * KC
            sc = _dot(qa[0], _rows(ckvT[0:64, k0:k0 + KC]))
            for b in range(1, 4):
                sc = sc + _dot(qa[b], _rows(ckvT[64 * b:64 * (b + 1), k0:k0 + KC]))
            return sc

        def soft(sc):
            mx = sc[:, 0:128]
            for j in range(1, KC // 128):
                mx = jnp.maximum(mx, sc[:, 128 * j:128 * (j + 1)])
            mx = jnp.max(mx, axis=1, keepdims=True)
            p = jnp.exp(sc - mx)
            den = p[:, 0:128]
            for j in range(1, KC // 128):
                den = den + p[:, 128 * j:128 * (j + 1)]
            ms.append(mx)
            ls.append(den)
            ps.append(p.astype(bf16))

        def ctx_all(i):
            o = _dot(ps[i], _rows(ckv2[i * KC // 2:(i + 1) * KC // 2, :]))
            cxs.append([o[:, 128 * b:128 * (b + 1)] for b in range(4)])

        def ctx_block(i, b):
            kq = KC // 4
            k0 = i * KC
            return functools.reduce(jnp.add, [
                _dot(ps[i][:, kq * u:kq * (u + 1)],
                     _rows(ckv2[(k0 + kq * u) // 2:(k0 + kq * (u + 1)) // 2, 128 * b:128 * (b + 1)]))
                for u in range(4)])

        scs = [scores(0), scores(1)]
        soft(scs[0])
        for i in range(NC - NL):
            if i + 2 < NC:
                scs.append(scores(i + 2))
            ctx_all(i)
            soft(scs[i + 1])
        for i in range(NC - NL + 1, NC):
            soft(scs[i])
        tail = [[None] * 4 for _ in range(NL)]
        for b in range(4):
            for i in range(NL):
                tail[i][b] = ctx_block(NC - NL + i, b)
        cxs += tail
        mx = functools.reduce(jnp.maximum, ms)
        ws = [jnp.exp(m_ - mx) for m_ in ms]
        den = functools.reduce(jnp.add, [w_ * l_ for w_, l_ in zip(ws, ls)])
        inv = 1.0 / jnp.sum(den, axis=1, keepdims=True)
        cx = [functools.reduce(jnp.add, [w_ * c_[b] for w_, c_ in zip(ws, cxs)]) for b in range(4)]
        return cx, inv

    def value_mxu(cx, inv, hf, first):
        acc = jnp.zeros((16, 128), f32)
        for b in range(4):
            sb = cx[b][16 * hf:16 * hf + 16]
            for j0 in range(0, 16, T):
                lhs = jnp.concatenate(
                    [jnp.where(diag_nat, pltpu.roll(sb, 16 - j, 1, stride=1, stride_axis=0), 0.0)
                     for j in range(j0, j0 + T)], axis=1).astype(bf16)
                x0 = 8 * (16 * b + j0)
                if first:
                    w = wuv[x0:x0 + 8 * T, 16 * hf:16 * hf + 16, :].reshape(128 * T, 128)
                else:
                    w = _rows(wuv0[x0:x0 + 8 * T].reshape(64 * T, 128))
                acc = acc + _dot(lhs, w)
        return acc * inv[16 * hf:16 * hf + 16]

    def out_mxu(ctx, first):
        acc = jnp.zeros((16, M), f32)
        hc = 4
        for h0 in range(0, 16 * len(ctx), hc):
            lhs = jnp.concatenate(
                [jnp.broadcast_to(ctx[h // 16][h % 16:h % 16 + 1], (16, 128)) for h in range(h0, h0 + hc)],
                axis=1).astype(bf16)
            w = wo[128 * h0:128 * (h0 + hc), :] if first else _rows(wo0[64 * h0:64 * (h0 + hc), :])
            acc = acc + _dot(lhs, w)
        return acc[0:8]

    def after(x, gate):
        return lax.bitcast_convert_type(lax.bitcast_convert_type(x, u32) | gate, f32)

    def fence(v):
        return lax.bitcast_convert_type(jnp.broadcast_to(v, (8, 128)), u32) & zero_w

    def value_out_vpu(cx, inv):
        vacc = None
        gates = []
        for n, h in enumerate(range(15, -1, -1)):
            rows = [jnp.broadcast_to(cx[b][16 + h:17 + h], (8, 128)) for b in range(4)]
            if n >= HEAD_LAG:
                rows = [after(r_, gates[n - HEAD_LAG]) for r_ in rows]
            hacc = None
            for j in range(0, 16, 2):
                cols = []
                for jj in (j, j + 1):
                    w = wuvT[h, 8 * jj:8 * jj + 8, :]
                    s_ = functools.reduce(jnp.add, [w[:, 128 * b:128 * (b + 1)] * rows[b] for b in range(4)])
                    cols.append(jnp.sum(s_, axis=1, keepdims=True))
                r0 = 128 * h + 8 * j
                t = cols[0] * wof[r0:r0 + 8, :] + cols[1] * wof[r0 + 8:r0 + 16, :]
                hacc = t if hacc is None else hacc + t
            gates.append(fence(cols[0]))
            t = hacc * jnp.broadcast_to(inv[16 + h:17 + h], (8, 1))
            vacc = t if vacc is None else vacc + t
        return _subsum(vacc)

    def normalise_q(qacc, x, first):
        mean, rs = _stats(x, first)
        m16 = jnp.concatenate([mean, mean], axis=0)
        rs16 = jnp.concatenate([rs, rs], axis=0)
        return [(qacc[hf] + jnp.concatenate([rev8(qacc[2 + hf][8:16]), rev8(qacc[2 + hf][0:8])], axis=0)
                 - m16 * qsum[hf]) * rs16 for hf in range(2)]

    def ffn_parts(x, first):
        lhs = jnp.concatenate([x, jnp.ones((8, M), f32)], axis=0).astype(bf16)
        mean, rs = _stats(x, first)
        xn = (x - mean) * rs
        wr = jnp.broadcast_to(wrs[...].reshape(1, M).astype(f32), (8, M))
        sig = 0.5 + 0.5 * jnp.tanh(0.5 * jnp.sum(xn * wr, axis=1, keepdims=True))
        return lhs, mean, rs, xn, sig

    def act(g, u, mean, rs):
        g = (g[0:8] - mean * g[8:16]) * rs
        u = (u[0:8] - mean * u[8:16]) * rs
        return _dup_rows(_half_silu(0.5 * g) * u)

    def ffn_mxu_block(lhs, mean, rs, f0, n):
        return act(_dot(lhs, _rows(wgT[:, f0:f0 + n])), _dot(lhs, _rows(wuT[:, f0:f0 + n])), mean, rs)

    def wd_relayout(r0, n, c0, nc):
        if r0 == 0:
            for f0 in range(0, FV, 64):
                wdf[f0:f0 + 64, c0:c0 + nc] = wd[f0:f0 + 64, c0:c0 + nc].astype(f32)
        for f0 in range(max(r0, FV), r0 + n, 64):
            wdm[(f0 - FV) // 2:(f0 - FV) // 2 + 32, c0:c0 + nc] = _words(wd[f0:f0 + 64, c0:c0 + nc])

    @pl.when(step == 0)
    def _():
        for cp in copies + wd_copies:
            cp.start()
        cp_x.wait()
        cp_wr.wait()
        x = jnp.broadcast_to(xs[0].astype(f32), (8, M))
        z16 = jnp.zeros((16, 128), f32)
        cp_wq.wait()
        for m0 in range(0, M, 16):
            wq[m0:m0 + 16] = _words(wqb[m0:m0 + 16])
        for m_lo, m_hi in QV:
            for m0 in range(m_lo, m_hi, 16):
                wqf[QV_POS[m0]:QV_POS[m0] + 16] = wqb[m0:m0 + 16].astype(f32)
        qacc = q_partial(x, 0, M, [z16] * 4, True)
        cx, inv = attend(absorb(normalise_q(qacc, x, True), True), True)
        cp_wuv.wait()
        for c0 in range(0, C, 16):
            wuv0[c0:c0 + 16] = _words(wuv[c0:c0 + 16, 0:16, :])
        for bq in range(64):
            b, q = bq // 16, bq % 16
            c0 = 128 * b + 64 * (q % 2) + (q // 2 + 1) % 8
            v = jnp.stack([_words(wuv[c0 + 8 * i, 16:32, :]) for i in range(8)], axis=0)
            gat[:, 8 * bq:8 * bq + 8, :] = jnp.swapaxes(v, 0, 1)
        eye = eye128()
        for r in range(8):
            for b in range(4):
                w = gat[r, 128 * b:128 * (b + 1), :]
                for e, bits in enumerate((w << 16, w & hi)):
                    t = lax.bitcast_convert_type(bits, f32).astype(bf16)
                    wuvT[2 * r + e, :, 128 * b:128 * (b + 1)] = _dot_t(eye, t)
        ctx = [value_mxu(cx, inv, 0, True), value_mxu(cx, inv, 1, True)]
        cp_wo.wait()
        for r0 in range(0, 16 * D, 64):
            wof[r0:r0 + 64] = wo[16 * D + r0:16 * D + r0 + 64].astype(f32)
            wo0[r0 // 2:r0 // 2 + 32] = _words(wo[r0:r0 + 64])
        x = x + out_mxu(ctx, True)
        lhs, mean, rs, xn, sig = ffn_parts(x, True)
        eye = eye128()
        for cp, src, dst in ((cp_wg1, wg, wgT), (cp_wu1, wu, wuT)):
            cp.wait()
            for g in range(5):
                for f0 in range(0, FM, 512):
                    dst[64 * g:64 * (g + 1), f0:f0 + 512] = _words(_dot_t(
                        eye, src[FV + f0:FV + f0 + 512, 128 * g:128 * (g + 1)]).astype(bf16))
        hm = ffn_mxu_block(lhs, mean, rs, 0, FM)
        cp_wg0.wait()
        gv = _dot_t(lhs, wg[0:FV, :])
        for f0 in range(0, FV, 64):
            wgf[f0:f0 + 64] = wg[f0:f0 + 64].astype(f32) * 0.5
        cp_wu0.wait()
        hw = jnp.concatenate([act(gv, _dot_t(lhs, wu[0:FV, :]), mean, rs), hm], axis=1)
        for f0 in range(0, FV, 64):
            wuf[f0:f0 + 64] = wu[f0:f0 + 64].astype(f32)
        base = x + xn
        qacc = [z16] * 4
        ys = {}
        for cp, (r0, n, c0, nc) in zip(wd_copies[:-1], WD[:-1]):
            cp.wait()
            o = _dot(_rows(hw[:, r0:r0 + n]), wd[r0:r0 + n, c0:c0 + nc])[0:8]
            ys[c0] = o if c0 not in ys else ys[c0] + o
            if r0 + n == F:
                x2 = base[:, c0:c0 + nc] + ys[c0] * sig
                st_x[0, :, c0:c0 + nc] = x2
                xpad = jnp.concatenate([jnp.zeros((8, c0), f32), x2], axis=1) if c0 else x2
                qacc = q_partial(xpad, c0, c0 + nc, qacc, False)
            wd_relayout(r0, n, c0, nc)
        for i in range(4):
            st_q[i] = qacc[i]
        c0 = WD[-1][2]
        st_x[0, :, c0:M] = base[:, c0:M]
        st_x[1] = jnp.broadcast_to(sig, (8, M))
        st_h[...] = hw

    @pl.when(step == 1)
    def _():
        c0 = WD[-1][2]
        wd_copies[-1].wait()
        ylate = _dot(_rows(st_h[...]), wd[:, c0:M])[0:8]
        x = jnp.concatenate([st_x[0, :, 0:c0], st_x[0, :, c0:M] + ylate * st_x[1, :, c0:M]], axis=1)
        qacc = q_partial(x, c0, M, [st_q[i] for i in range(4)], False)
        wd_relayout(*WD[-1])
        cx, inv = attend(absorb(normalise_q(qacc, x, False), False), False)
        x = x + (out_mxu([value_mxu(cx, inv, 0, False)], False) + value_out_vpu(cx, inv))
        lhs, mean, rs, xn, sig = ffn_parts(x, False)
        hs = [ffn_mxu_block(lhs, mean, rs, f0, FB) for f0 in range(0, FM, FB)]
        ym = functools.reduce(jnp.add, [_dot(_rows(h_), _rows(wdm[FB // 2 * i:FB // 2 * (i + 1), :]))[0:8]
                                        for i, h_ in enumerate(hs)])
        yv = jnp.zeros((8, M), f32)
        xg = xn
        gates = []
        for i in range(FV // 8):
            if i % FFN_EVERY == 0 and i >= FFN_LAG:
                xg = jnp.concatenate([after(xn[:, 128 * k:128 * (k + 1)], gates[i - FFN_LAG]) for k in range(5)], axis=1)
            pg = wgf[8 * i:8 * i + 8, :] * xg
            pu = wuf[8 * i:8 * i + 8, :] * xg
            sg = (pg[:, 0:128] + pg[:, 128:256]) + (pg[:, 256:384] + pg[:, 384:512]) + pg[:, 512:640]
            su = (pu[:, 0:128] + pu[:, 128:256]) + (pu[:, 256:384] + pu[:, 384:512]) + pu[:, 512:640]
            hc = _half_silu(jnp.sum(sg, axis=1, keepdims=True)) * jnp.sum(su, axis=1, keepdims=True)
            gates.append(fence(hc))
            yv = yv + hc * wdf[8 * i:8 * i + 8, :]
        x = x + xn + (_subsum(yv) + ym) * sig
        out_ref[0] = x[0:1].astype(bf16)


_SCRATCH = [
    pltpu.VMEM((1, 1, M), bf16), pltpu.VMEM((M,), bf16),
    pltpu.VMEM((M, H, D), bf16), pltpu.VMEM((C, H, D), bf16), pltpu.VMEM((S, C), bf16),
    pltpu.VMEM((C, H, D), bf16), pltpu.VMEM((F, M), bf16), pltpu.VMEM((F, M), bf16),
    pltpu.VMEM((H * D, M), bf16), pltpu.VMEM((F, M), bf16),
    pltpu.VMEM((M, H // 2, D), u32), pltpu.VMEM((C, 8, D), u32), pltpu.VMEM((8 * D, M), u32),
    pltpu.VMEM((FM // 2, M), u32), pltpu.VMEM((4, D // 2, 32 * 128), u32),
    pltpu.VMEM((C // 2, S), u32), pltpu.VMEM((S // 2, C), u32),
    pltpu.VMEM((M // 2, FM), u32), pltpu.VMEM((M // 2, FM), u32),
    pltpu.VMEM((len(QV_ROWS), H, D), f32), pltpu.VMEM((NV, D, 128), f32), pltpu.VMEM((16, D, C), f32),
    pltpu.VMEM((16 * D, M), f32), pltpu.VMEM((FV, M), f32), pltpu.VMEM((FV, M), f32), pltpu.VMEM((FV, M), f32),
    pltpu.VMEM((8, C, D), u32), pltpu.VMEM((2, 16, 128), f32),
    pltpu.VMEM((2, 8, M), f32), pltpu.VMEM((8, F), u32), pltpu.VMEM((4, 16, 128), f32),
    pltpu.SemaphoreType.DMA((11 + len(WD),)),
]


@jax.jit
def pallas_interleave_layers__compressed_kv_cla__moe_arch_mod__decode_kernel(
        A_x, A_c_kv, A_w_q, A_w_uk, A_w_uv, A_w_o, B_x, B_w_r, B_w_gate, B_w_up, B_w_down):
    del B_x
    return pl.pallas_call(
        _kernel,
        out_shape=jax.ShapeDtypeStruct((1, 1, M), bf16),
        grid=(2,),
        in_specs=[pl.BlockSpec(memory_space=pl.ANY)] * 10,
        out_specs=pl.BlockSpec((1, 1, M), lambda i: (0, 0, 0)),
        scratch_shapes=_SCRATCH,
        compiler_params=pltpu.CompilerParams(vmem_limit_bytes=120 * 1024 * 1024,
                                             dimension_semantics=("arbitrary",)),
        name="fused_decode",
    )(A_x, B_w_r, A_w_q, A_w_uk, A_c_kv.reshape(S, C), A_w_uv, B_w_gate.T, B_w_up.T,
      A_w_o.reshape(H * D, M), B_w_down)
```
